```python
import jax
import jax.numpy as jnp

def _softmax(x, axis=-1):
    return jax.nn.softmax(x, axis=axis)

def _gelu(x):
    return jax.nn.gelu(x, approximate=True)

def _silu(x):
    return jax.nn.silu(x)

def _sigmoid(x):
    return jax.nn.sigmoid(x)

def _layernorm(x, axis=-1, eps=1e-05):
    m = jnp.mean(x, axis=axis, keepdims=True)
    v = jnp.var(x, axis=axis, keepdims=True)
    return (x - m) / jnp.sqrt(v + eps)

def _scatter_add(tgt, idx, src, axis=0):
    return tgt.at[idx].add(src)

def _segment_sum(src, seg, n):
    return jax.ops.segment_sum(src, seg, n)

class _Rng:

    def __init__(self, key):
        self._k = key

    def _next(self):
        self._k, sub = jax.random.split(self._k)
        return sub

    def normal(self, shape):
        return jax.random.normal(self._next(), shape, dtype=jnp.bfloat16)

    def randint(self, lo, hi, shape):
        return jax.random.randint(self._next(), shape, lo, hi, dtype=jnp.int32)

    def uniform(self, shape, lo=0.0, hi=1.0):
        return jax.random.uniform(self._next(), shape, jnp.bfloat16, lo, hi)

    def permutation(self, n):
        return jax.random.permutation(self._next(), n)
kernel_name = 'concat_heads__memory_aug_recurrent_mem_tr__spectral_gfnet__prompt'

def setup_inputs():
    _rng = _Rng(jax.random.key(int.from_bytes(__import__("os").urandom(4), "little")))
    _w = lambda a: (lambda t: t.astype(jnp.bfloat16) if jnp.issubdtype(t.dtype, jnp.floating) else t)(jnp.asarray(a))

    def _A_setup():
        B, S, Dm = (1, 2048, 1024)
        H, Dh = (32, 128)
        M, seg = (8, 32)
        seg = min(seg, S)
        S = S // seg * seg
        return {'x': _w((lambda *s: _rng.normal(s) * 0.05)(B, S, Dm)), 'mem0': _w((lambda *s: _rng.normal(s) * 0.05)(B, M, Dm)), 'Wq': _w((lambda *s: _rng.normal(s) * 0.05)(Dm, H, Dh) * Dm ** (-0.5)), 'Wk': _w((lambda *s: _rng.normal(s) * 0.05)(Dm, H, Dh) * Dm ** (-0.5)), 'Wv': _w((lambda *s: _rng.normal(s) * 0.05)(Dm, H, Dh) * Dm ** (-0.5)), 'Wo': _w((lambda *s: _rng.normal(s) * 0.05)(H, Dh, Dm) * (H * Dh) ** (-0.5)), 'seg_len': seg}
    _A_in = _A_setup()

    def _B_setup():
        B, S, D = (1, 2048, 1024)
        Df = D // 2 + 1
        return {'x': _w((lambda *s: _rng.normal(s) * 0.05)(B, S, D)), 'w_r': _w((lambda *s: _rng.normal(s) * 0.05)(S, Df) * 0.02), 'w_i': _w((lambda *s: _rng.normal(s) * 0.05)(S, Df) * 0.02)}
    _B_in = _B_setup()
    return {'A_x': _A_in['x'], 'A_mem0': _A_in['mem0'], 'A_Wq': _A_in['Wq'], 'A_Wk': _A_in['Wk'], 'A_Wv': _A_in['Wv'], 'A_Wo': _A_in['Wo'], 'A_seg_len': _A_in['seg_len'], 'B_x': _B_in['x'], 'B_w_r': _B_in['w_r'], 'B_w_i': _B_in['w_i']}

def reference(A_x, A_mem0, A_Wq, A_Wk, A_Wv, A_Wo, A_seg_len, B_x, B_w_r, B_w_i):

    def _A_ref(x, mem0, Wq, Wk, Wv, Wo, seg_len):
        B, S, Dm = x.shape
        H, Dh = (Wq.shape[1], Wq.shape[2])
        M = mem0.shape[1]
        scale = Dh ** (-0.5)
        n_seg = S // seg_len
        L = M + seg_len
        idx = jnp.arange(L)
        mask = (idx[:, None] < M) | (idx[:, None] >= idx[None, :])
        mem = mem0
        outs = []
        for s in range(n_seg):
            xs = x[:, s * seg_len:(s + 1) * seg_len, :].copy()
            h = jnp.concatenate([mem, xs], axis=1)
            q = jnp.einsum('btd,dhe->bhte', h, Wq)
            k = jnp.einsum('btd,dhe->bhte', h, Wk)
            v = jnp.einsum('btd,dhe->bhte', h, Wv)
            scores = jnp.einsum('bhqe,bhke->bhqk', q, k) * scale
            scores = jnp.where(mask[None, None], scores, -1000000000.0)
            p = _softmax(scores, axis=-1)
            o = jnp.einsum('bhqk,bhke->bhqe', p, v)
            o = jnp.einsum('bhte,hed->btd', o, Wo)
            mem = o[:, :M, :].copy()
            outs.append(o[:, M:, :])
        return jnp.concatenate(outs, axis=1)

    def _B_ref(x, w_r, w_i):
        B, S, D = x.shape
        X = (lambda x, axes=(-2, -1): jnp.fft.rfft2(x.astype(jnp.float32), axes=axes))(x, axes=(-2, -1))
        W = w_r + 1j * w_i
        X = X * W
        y = (lambda x, s, axes=(-2, -1): jnp.fft.irfft2(x, s=s, axes=axes).astype(jnp.bfloat16))(X, (S, D), axes=(-2, -1))
        return y
    a = _A_ref(A_x, A_mem0, A_Wq, A_Wk, A_Wv, A_Wo, A_seg_len)
    b = _B_ref(B_x, B_w_r, B_w_i)
    return jnp.concatenate([a, b], axis=-1)
```

```python
import numpy as np
import jax
import jax.numpy as jnp
from jax import lax
import jax.experimental.pallas as pl
import jax.experimental.pallas.tpu as pltpu

S, D, H, DH, M, SEG = 2048, 1024, 32, 128, 8, 32
L = M + SEG
NSEG = S // SEG
DF = D // 2 + 1
R1, R2 = 16, 128
NT = 5
f32, bf16, u32 = jnp.float32, jnp.bfloat16, jnp.uint32


def _dft_constants():
    d = np.arange(D)[:, None]
    k = np.arange(D // 2)[None, :]
    ang = 2.0 * np.pi * ((d * k) % D) / D
    fc, fs = np.cos(ang), -np.sin(ang)
    fs[:, 0] = 1.0 - 2.0 * (np.arange(D) % 2)
    fd = np.concatenate([fc, fs], axis=1)
    f1 = np.arange(R1)[:, None, None]
    f2 = np.arange(R2)[None, :, None]
    t2 = np.arange(R2)[None, None, :]
    a = -2.0 * np.pi * ((t2 * (f1 + R1 * f2)) % S) / S
    mr, mi = np.cos(a), np.sin(a)
    blk = np.concatenate([np.concatenate([mr, -mi], 2), np.concatenate([mi, mr], 2)], 1)
    return fd.astype(np.float32), blk.astype(np.float32)


_FD, _MBLK = _dft_constants()


def _dot(a, b):
    return lax.dot_general(a, b, (((1,), (0,)), ((), ())), preferred_element_type=f32)


def _dot_nt(a, b):
    return lax.dot_general(a, b, (((1,), (1,)), ((), ())), preferred_element_type=f32)


def _dot_tn(a, b):
    return lax.dot_general(a, b, (((0,), (0,)), ((), ())), preferred_element_type=f32)


def _cmul_const(x, e, n, sign):
    xr, xi = x
    e = e % n
    if e == 0:
        return x
    if 4 * e == n:
        return (_neg(xi), xr) if sign > 0 else (xi, _neg(xr))
    c = float(np.cos(2.0 * np.pi * e / n))
    s = float(sign * np.sin(2.0 * np.pi * e / n))
    if xi is None:
        return xr * c, xr * s
    if 8 * e == n or 8 * e == 3 * n:
        if c * s > 0:
            return (xr - xi) * c, (xr + xi) * c
        return (xr + xi) * c, (xi - xr) * c
    return xr * c - xi * s, xr * s + xi * c


def _neg(a):
    return None if a is None else -a


def _add(a, b):
    return b if a is None else a if b is None else a + b


def _sub(a, b):
    return _neg(b) if a is None else a if b is None else a - b


def _fft(xs, sign):
    n = len(xs)
    if n == 1:
        return xs
    ev, od = _fft(xs[0::2], sign), _fft(xs[1::2], sign)
    out = [None] * n
    for j in range(n // 2):
        e = ev[j]
        if 4 * j == n:
            orr, oi = od[j]
            if sign > 0:
                out[j] = (_sub(e[0], oi), _add(e[1], orr))
                out[j + n // 2] = (_add(e[0], oi), _sub(e[1], orr))
            else:
                out[j] = (_add(e[0], oi), _sub(e[1], orr))
                out[j + n // 2] = (_sub(e[0], oi), _add(e[1], orr))
            continue
        t = _cmul_const(od[j], j, n, sign)
        out[j] = (_add(e[0], t[0]), _add(e[1], t[1]))
        out[j + n // 2] = (_sub(e[0], t[0]), _sub(e[1], t[1]))
    return out


def _spectral_phase(xb, fd, mblk, wst, zb, yb):
    G = 16

    def fwd(g, _):
        r0 = pl.multiple_of(g * G, G)
        lane0 = lax.broadcasted_iota(jnp.int32, (R1 * G, 128), 1) == 0
        xg = jnp.concatenate([xb[pl.ds(t1 * R2 + r0, G), :] for t1 in range(R1)], axis=0)
        nyq = None
        for j in range(NT):
            if j < 4:
                zr = _dot(xg, fd[:, j * 128:(j + 1) * 128])
                zi = _dot(xg, fd[:, 512 + j * 128:512 + (j + 1) * 128])
                if j == 0:
                    nyq = jnp.where(lane0, zi, 0.0)
                    zi = jnp.where(lane0, 0.0, zi)
                xs = [(zr[t * G:(t + 1) * G], zi[t * G:(t + 1) * G]) for t in range(R1)]
            else:
                xs = [(nyq[t * G:(t + 1) * G], None) for t in range(R1)]
            ys = _fft(xs, -1)
            for f1 in range(R1):
                yr, yi = ys[f1]
                yi = jnp.zeros_like(yr) if yi is None else yi
                zb[f1, pl.ds(r0, G), j * 128:(j + 1) * 128] = yr.astype(bf16)
                zb[f1, pl.ds(R2 + r0, G), j * 128:(j + 1) * 128] = yi.astype(bf16)
        return 0

    lax.fori_loop(0, R2 // G, fwd, 0)

    def mid(g, _):
        lane = lax.broadcasted_iota(jnp.int32, (1, 128), 1)
        for half in range(2):
            f1 = 2 * g + half
            mb = mblk[f1]
            x = _dot(mb, zb[f1])
            ys = []
            for j in range(NT):
                wr = wst[0, j, pl.ds(g, R2, stride=R1 // 2), :]
                wi = wst[1, j, pl.ds(g, R2, stride=R1 // 2), :]
                if half == 0:
                    wr, wi = wr << 16, wi << 16
                else:
                    wr, wi = wr & u32(0xFFFF0000), wi & u32(0xFFFF0000)
                if j == 0:
                    sc = jnp.where(lane == 0, 1.0 / (S * D), 2.0 / (S * D))
                else:
                    sc = (1.0 if j == 4 else 2.0) / (S * D)
                wr = pltpu.bitcast(wr, f32) * sc
                wi = pltpu.bitcast(wi, f32) * sc
                xr = x[:R2, j * 128:(j + 1) * 128]
                xi = x[R2:, j * 128:(j + 1) * 128]
                ys.append(jnp.concatenate([xr * wr - xi * wi, xr * wi + xi * wr], axis=0).astype(bf16))
            yb[f1] = _dot_tn(mb, jnp.concatenate(ys, axis=1))
        return 0

    lax.fori_loop(0, R1 // 2, mid, 0)

    def inv(g, _):
        r0 = pl.multiple_of(g * G, G)
        lane0 = lax.broadcasted_iota(jnp.int32, (R1 * G, 128), 1) == 0

        def tile(j):
            xs = [(yb[f1, pl.ds(r0, G), j * 128:(j + 1) * 128],
                   yb[f1, pl.ds(R2 + r0, G), j * 128:(j + 1) * 128]) for f1 in range(R1)]
            ys = _fft(xs, +1)
            return (jnp.concatenate([y[0] for y in ys], axis=0),
                    jnp.concatenate([y[1] for y in ys], axis=0))

        nyq = tile(4)[0]
        acc = None
        for j in range(4):
            yr, yi = tile(j)
            if j == 0:
                yi = jnp.where(lane0, nyq, yi)
            p = (_dot_nt(yr.astype(bf16), fd[:, j * 128:(j + 1) * 128])
                 + _dot_nt(yi.astype(bf16), fd[:, 512 + j * 128:512 + (j + 1) * 128]))
            acc = p if acc is None else acc + p
        acc = acc.astype(bf16)
        for t1 in range(R1):
            xb[pl.ds(t1 * R2 + r0, G), :] = acc[t1 * G:(t1 + 1) * G]
        return 0

    lax.fori_loop(0, R2 // G, inv, 0)


def _attention_phase(xa, mem_ref, wqkv, wo, outa, store_rows):
    row = lax.broadcasted_iota(jnp.int32, (L, L), 0)
    col = lax.broadcasted_iota(jnp.int32, (L, L), 1)

    def step(s, mem):
        mask = (row < M) | (row >= col)
        rows = pl.ds(pl.multiple_of(s * SEG, SEG), SEG)
        h = jnp.concatenate([mem, xa[rows, :].astype(f32)], axis=0)
        st = {}

        def do_qkv(hd):
            qkv = _dot(h, pltpu.bitcast(wqkv[:, hd * 384:(hd + 1) * 384], bf16))
            st['q', hd] = qkv[:, :128] * (DH ** -0.5)
            st['k', hd] = qkv[:, 128:256].astype(bf16)
            st['v', hd] = qkv[:, 256:].astype(bf16)

        def do_qk(hd):
            sc = jnp.where(mask, _dot_nt(st['q', hd], st['k', hd]), -1e9)
            e = jnp.exp(sc - jnp.max(sc, axis=1, keepdims=True))
            st['e', hd] = e
            st['r', hd] = 1.0 / jnp.sum(e, axis=1, keepdims=True)

        def do_pv(hd):
            st['o', hd] = _dot(st['e', hd], st['v', hd]) * st['r', hd]

        def do_wo(g, ng=4):
            o = jnp.concatenate([st['o', hd] for hd in range(g * ng, (g + 1) * ng)], axis=1)
            for n in range(8):
                r = _dot(o, wo[n, g * ng * 128:(g + 1) * ng * 128, :])
                st['out', n] = r if g == 0 else st['out', n] + r

        for t in range(H):
            do_qkv(t)
            if t >= 1:
                do_qk(t - 1)
            if t >= 3:
                do_pv(t - 3)
        do_wo(0); do_qk(H - 1); do_pv(H - 3)
        do_wo(1); do_pv(H - 2)
        do_wo(2); do_pv(H - 1)
        for g in range(3, 8):
            do_wo(g)
        out = jnp.concatenate([st['out', n] for n in range(8)], axis=1)
        outa[rows, :] = out[M:].astype(bf16)
        store_rows(s)
        return out[:M].astype(bf16).astype(f32)

    lax.fori_loop(0, NSEG, step, mem_ref[...].astype(f32))


def _kernel(xa_hbm, mem_ref, wq_hbm, wk_hbm, wv_hbm, wo_hbm, xb_hbm, wr_hbm, wi_hbm, fd_hbm, mblk_hbm,
            out_hbm, raw, wqkv, wo, xa, xb, fd, mblk, wraw, wst, zb, yb, sems, osem):
    def copy(src, dst, i):
        c = pltpu.make_async_copy(src, dst, sems.at[i])
        c.start()
        return c

    c_xb = copy(xb_hbm, xb, 0)
    c_fd = copy(fd_hbm, fd, 1)
    c_wr = copy(wr_hbm, wraw.at[0], 2)
    c_wi = copy(wi_hbm, wraw.at[1], 3)
    c_mb = copy(mblk_hbm, mblk, 4)
    c_w = [copy(w, raw.at[j], 5 + j) for j, w in enumerate((wq_hbm, wk_hbm, wv_hbm))]
    c_wo = [copy(wo_hbm.at[:, n * 128:(n + 1) * 128], wo.at[n], 8 + n) for n in range(8)]
    c_xa = copy(xa_hbm, xa, 16)

    c_wr.wait()
    c_wi.wait()

    def prep(t, _):
        src = pl.ds(pl.multiple_of(t * 128, 128), 128)
        dst = pl.ds(pl.multiple_of(t * 64, 64), 64)
        for c in range(2):
            for j in range(4):
                wst[c, j, dst, :] = pltpu.bitcast(wraw[c, src, j * 128:(j + 1) * 128], u32)
            last = jnp.broadcast_to(wraw[c, src, 512:513].astype(f32), (128, 128))
            wst[c, 4, dst, :] = pltpu.bitcast(last.astype(bf16), u32)
        return 0

    lax.fori_loop(0, S // 128, prep, 0)

    c_xb.wait()
    c_fd.wait()
    c_mb.wait()
    _spectral_phase(xb, fd, mblk, wst, zb, yb)
    c_ob = copy(xb, out_hbm.at[:, D:], 17)

    for j in range(3):
        c_w[j].wait()
        pairs = raw.at[j].bitcast(u32)

        def relayout(t, _):
            blk = pairs.at[pl.ds(pl.multiple_of(t * 256, 256), 256), :]
            dst = pl.ds(pl.multiple_of(t * 8, 8), 8)
            for i in range(H // 2):
                a = blk[pl.ds(i, 8, stride=32), :]
                b = blk[pl.ds(16 + i, 8, stride=32), :]
                wqkv[dst, pl.ds((2 * i) * 384 + j * 128, 128)] = (a & u32(0xFFFF)) | (b << 16)
                wqkv[dst, pl.ds((2 * i + 1) * 384 + j * 128, 128)] = (a >> 16) | (b & u32(0xFFFF0000))
            return 0

        lax.fori_loop(0, D // 16, relayout, 0)
    for c in c_wo:
        c.wait()
    c_xa.wait()

    def out_copy(s):
        rows = pl.ds(pl.multiple_of(s * SEG, SEG), SEG)
        return pltpu.make_async_copy(xa.at[rows, :], out_hbm.at[rows, pl.ds(0, D)], osem.at[0])

    _attention_phase(xa, mem_ref, wqkv, wo, xa, lambda s: out_copy(s).start())

    def drain(s, _):
        out_copy(s).wait()
        return 0

    lax.fori_loop(0, NSEG, drain, 0)
    c_ob.wait()


@jax.jit
def pallas_concat_heads__memory_aug_recurrent_mem_tr__spectral_gfnet__prompt_kernel(
    A_x, A_mem0, A_Wq, A_Wk, A_Wv, A_Wo, A_seg_len, B_x, B_w_r, B_w_i,
):
    del A_seg_len
    hbm = pl.BlockSpec(memory_space=pl.ANY)
    out = pl.pallas_call(
        _kernel,
        out_shape=jax.ShapeDtypeStruct((S, 2 * D), bf16),
        in_specs=[hbm, pl.BlockSpec(memory_space=pltpu.VMEM)] + [hbm] * 9,
        out_specs=hbm,
        scratch_shapes=[
            pltpu.VMEM((3, D * H, DH), bf16),
            pltpu.VMEM((D // 2, H * 384), u32),
            pltpu.VMEM((8, H * DH, 128), bf16),
            pltpu.VMEM((S, D), bf16),
            pltpu.VMEM((S, D), bf16),
            pltpu.VMEM((D, D), bf16),
            pltpu.VMEM((R1, 2 * R2, 2 * R2), bf16),
            pltpu.VMEM((2, S, DF), bf16),
            pltpu.VMEM((2, NT, S // 2, 128), u32),
            pltpu.VMEM((R1, 2 * R2, NT * 128), bf16),
            pltpu.VMEM((R1, 2 * R2, NT * 128), f32),
            pltpu.SemaphoreType.DMA((18,)),
            pltpu.SemaphoreType.DMA((1,)),
        ],
        compiler_params=pltpu.CompilerParams(vmem_limit_bytes=120 * 2 ** 20),
    )(
        A_x.reshape(S, D), A_mem0.reshape(M, D),
        A_Wq.reshape(D * H, DH), A_Wk.reshape(D * H, DH), A_Wv.reshape(D * H, DH),
        A_Wo.reshape(H * DH, D),
        B_x.reshape(S, D), B_w_r, B_w_i,
        jnp.asarray(_FD, dtype=bf16), jnp.asarray(_MBLK, dtype=bf16),
    )
    return out.reshape(1, S, 2 * D)
```

```python
import numpy as np
import jax
import jax.numpy as jnp
from jax import lax
import jax.experimental.pallas as pl
import jax.experimental.pallas.tpu as pltpu

S, D, H, DH, M, SEG = 2048, 1024, 32, 128, 8, 32
L = M + SEG
NSEG = S // SEG
DF = D // 2 + 1
R1, R2 = 16, 128
G = 16
WC = 64
WP = 24
XA0 = 2
NT = 5
f32, bf16, u32 = jnp.float32, jnp.bfloat16, jnp.uint32


def _k1_pair(j):
    return j, (4 if j == 0 else 8 - j)


def _dft_constants():
    b = np.arange(128)[:, None]
    c = np.arange(64)[None, :]
    fd = np.zeros((4, 256, 256))
    for j in range(4):
        for half, k1 in enumerate(_k1_pair(j)):
            ang = 2.0 * np.pi * ((b * (k1 + 8 * c)) % D) / D
            co, si = np.cos(ang), np.sin(ang)
            re = slice(64 * half, 64 * half + 64)
            im = slice(128 + 64 * half, 128 + 64 * half + 64)
            if j == 0:
                rows = slice(128 * half, 128 * half + 128)
                fd[j, rows, re], fd[j, rows, im] = co, -si
            else:
                sg = 1.0 - 2.0 * half
                fd[j, :128, re], fd[j, :128, im] = co, -si
                fd[j, 128:, re], fd[j, 128:, im] = sg * si, sg * co
    fd[0, :128, 128] = 1.0 - 2.0 * (np.arange(128) % 2)
    f1 = np.arange(R1)[:, None, None]
    f2 = np.arange(R2)[None, :, None]
    t2 = np.arange(R2)[None, None, :]
    a = -2.0 * np.pi * ((t2 * (f1 + R1 * f2)) % S) / S
    mr, mi = np.cos(a), np.sin(a)
    blk = np.concatenate([np.concatenate([mr, -mi], 2), np.concatenate([mi, mr], 2)], 1)
    return fd.astype(np.float32), blk.astype(np.float32)


_FD, _MBLK = _dft_constants()
_RH = float(np.sqrt(0.5))


def _dot(a, b):
    return lax.dot_general(a, b, (((1,), (0,)), ((), ())), preferred_element_type=f32)


def _dot_nt(a, b):
    return lax.dot_general(a, b, (((1,), (1,)), ((), ())), preferred_element_type=f32)


def _dot_tn(a, b):
    return lax.dot_general(a, b, (((0,), (0,)), ((), ())), preferred_element_type=f32)


def _cmul_const(x, e, n, sign):
    xr, xi = x
    e = e % n
    if e == 0:
        return x
    if 4 * e == n:
        return (_neg(xi), xr) if sign > 0 else (xi, _neg(xr))
    c = float(np.cos(2.0 * np.pi * e / n))
    s = float(sign * np.sin(2.0 * np.pi * e / n))
    if xi is None:
        return xr * c, xr * s
    if 8 * e == n or 8 * e == 3 * n:
        if c * s > 0:
            return (xr - xi) * c, (xr + xi) * c
        return (xr + xi) * c, (xi - xr) * c
    return xr * c - xi * s, xr * s + xi * c


def _neg(a):
    return None if a is None else -a


def _add(a, b):
    return b if a is None else a if b is None else a + b


def _sub(a, b):
    return _neg(b) if a is None else a if b is None else a - b


def _fft(xs, sign):
    n = len(xs)
    if n == 1:
        return xs
    ev, od = _fft(xs[0::2], sign), _fft(xs[1::2], sign)
    out = [None] * n
    for j in range(n // 2):
        e = ev[j]
        if 4 * j == n:
            orr, oi = od[j]
            if sign > 0:
                out[j] = (_sub(e[0], oi), _add(e[1], orr))
                out[j + n // 2] = (_add(e[0], oi), _sub(e[1], orr))
            else:
                out[j] = (_add(e[0], oi), _sub(e[1], orr))
                out[j + n // 2] = (_sub(e[0], oi), _add(e[1], orr))
            continue
        t = _cmul_const(od[j], j, n, sign)
        out[j] = (_add(e[0], t[0]), _add(e[1], t[1]))
        out[j + n // 2] = (_sub(e[0], t[0]), _sub(e[1], t[1]))
    return out


def _rfft8(x):
    s04, d04, s26, d26 = x[0] + x[4], x[0] - x[4], x[2] + x[6], x[2] - x[6]
    s15, d15, s37, d37 = x[1] + x[5], x[1] - x[5], x[3] + x[7], x[3] - x[7]
    e, o = s04 + s26, s15 + s37
    p, q = (d15 - d37) * _RH, (d15 + d37) * _RH
    return [(e + o, e - o), (d04 + p, -(d26 + q)), (s04 - s26, s37 - s15), (d04 - p, d26 - q)]


def _rfft8_adjoint(g):
    (g0, g4), (r1, i1), (r2, i2), (r3, i3) = g
    e, o = g0 + g4, g0 - g4
    s04, s26, s15, s37 = e + r2, e - r2, o - i2, o + i2
    d04, d26 = r1 + r3, i3 - i1
    p, q = (r1 - r3) * _RH, (i1 + i3) * _RH
    d15, d37 = p - q, -(p + q)
    return [s04 + d04, s15 + d15, s26 + d26, s37 + d37, s04 - d04, s15 - d15, s26 - d26, s37 - d37]


def _spectral_phase(xb, fd, mblk, wst, zb, yb, wait_rows, before_mid, in_mid, before_inv, in_inv):
    def fwd(g, _):
        wait_rows(g)
        r0 = pl.multiple_of(g * G, G)
        lane0 = lax.broadcasted_iota(jnp.int32, (R1 * G, 128), 1) == 0
        xg = xb[g].reshape(R1 * G, D)
        us = _rfft8([xg[:, a * 128:(a + 1) * 128].astype(f32) for a in range(8)])
        nyq = None
        for j in range(NT):
            if j < 4:
                z = _dot(jnp.concatenate(us[j], axis=1).astype(bf16), fd[j])
                zr, zi = z[:, :128], z[:, 128:]
                if j == 0:
                    nyq = jnp.where(lane0, zi, 0.0)
                    zi = jnp.where(lane0, 0.0, zi)
                xs = [(zr[t * G:(t + 1) * G], zi[t * G:(t + 1) * G]) for t in range(R1)]
            else:
                xs = [(nyq[t * G:(t + 1) * G], None) for t in range(R1)]
            ys = _fft(xs, -1)
            for f1 in range(R1):
                yr, yi = ys[f1]
                yi = jnp.zeros_like(yr) if yi is None else yi
                zb[f1, pl.ds(r0, G), j * 128:(j + 1) * 128] = yr.astype(bf16)
                zb[f1, pl.ds(R2 + r0, G), j * 128:(j + 1) * 128] = yi.astype(bf16)
        return 0

    lax.fori_loop(0, R2 // G, fwd, 0)
    before_mid()

    def mid(g, _):
        side = in_mid(g, 4 * NT)
        lane = lax.broadcasted_iota(jnp.int32, (1, 128), 1)
        for half in range(2):
            f1 = 2 * g + half
            mb = mblk[f1]
            xs = []
            for j in range(NT):
                xs.append(_dot(mb, zb[f1, :, j * 128:(j + 1) * 128]))
                next(side)
            mbt = mb.T
            for j in range(NT):
                wr = wst[0, j, pl.ds(g, R2, stride=R1 // 2), :]
                wi = wst[1, j, pl.ds(g, R2, stride=R1 // 2), :]
                if half == 0:
                    wr, wi = wr << 16, wi << 16
                else:
                    wr, wi = wr & u32(0xFFFF0000), wi & u32(0xFFFF0000)
                if j == 0:
                    sc = jnp.where(lane == 0, 1.0 / (S * D), 2.0 / (S * D))
                else:
                    sc = (1.0 if j == 4 else 2.0) / (S * D)
                wr = pltpu.bitcast(wr, f32) * sc
                wi = pltpu.bitcast(wi, f32) * sc
                xr, xi = xs[j][:R2], xs[j][R2:]
                y = jnp.concatenate([xr * wr - xi * wi, xr * wi + xi * wr], axis=0).astype(bf16)
                yb[f1, :, j * 128:(j + 1) * 128] = _dot(mbt, y)
                next(side)
        return 0

    lax.fori_loop(0, R1 // 2, mid, 0)

    before_inv()

    def inv(g, _):
        side = in_inv(g, 5)
        r0 = pl.multiple_of(g * G, G)
        lane0 = lax.broadcasted_iota(jnp.int32, (R1 * G, 128), 1) == 0

        def tile(j):
            xs = [(yb[f1, pl.ds(r0, G), j * 128:(j + 1) * 128],
                   yb[f1, pl.ds(R2 + r0, G), j * 128:(j + 1) * 128]) for f1 in range(R1)]
            ys = _fft(xs, +1)
            return (jnp.concatenate([y[0] for y in ys], axis=0),
                    jnp.concatenate([y[1] for y in ys], axis=0))

        nyq = tile(4)[0]
        next(side)
        gs = []
        for j in range(4):
            yr, yi = tile(j)
            if j == 0:
                yi = jnp.where(lane0, nyq, yi)
            p = _dot_nt(jnp.concatenate([yr, yi], axis=1).astype(bf16), fd[j])
            gs.append((p[:, :128], p[:, 128:]))
            next(side)
        y = jnp.concatenate(_rfft8_adjoint(gs), axis=1).astype(bf16)
        xb[g] = y.reshape(R1, G, D)
        return 0

    lax.fori_loop(0, R2 // G, inv, 0)


def _attention_phase(xa, mem_ref, wqkv, wo, outa, before_step, store_rows):
    row = lax.broadcasted_iota(jnp.int32, (L, L), 0)
    col = lax.broadcasted_iota(jnp.int32, (L, L), 1)

    def step(s, mem):
        before_step(s)
        mask = (row < M) | (row >= col)
        rows = pl.ds(pl.multiple_of(s * SEG, SEG), SEG)
        h = jnp.concatenate([mem, xa[rows, :].astype(f32)], axis=0)
        st = {}

        def do_qkv(hd):
            qkv = _dot(h, pltpu.bitcast(wqkv[:, hd * 384:(hd + 1) * 384], bf16))
            st['q', hd] = qkv[:, :128] * (DH ** -0.5)
            st['k', hd] = qkv[:, 128:256].astype(bf16)
            st['v', hd] = qkv[:, 256:].astype(bf16)

        def do_qk(hd):
            sc = jnp.where(mask, _dot_nt(st['q', hd], st['k', hd]), -1e9)
            e = jnp.exp(sc - jnp.max(sc, axis=1, keepdims=True))
            st['e', hd] = e
            st['r', hd] = 1.0 / jnp.sum(e, axis=1, keepdims=True)

        def do_pv(hd):
            st['o', hd] = _dot(st['e', hd], st['v', hd]) * st['r', hd]

        def do_wo(g, ng=4):
            o = jnp.concatenate([st['o', hd] for hd in range(g * ng, (g + 1) * ng)], axis=1)
            for n in range(8):
                r = _dot(o, wo[n, g * ng * 128:(g + 1) * ng * 128, :])
                st['out', n] = r if g == 0 else st['out', n] + r

        for t in range(H):
            do_qkv(t)
            if t >= 1:
                do_qk(t - 1)
            if t >= 3:
                do_pv(t - 3)
        do_wo(0); do_qk(H - 1); do_pv(H - 3)
        do_wo(1); do_pv(H - 2)
        do_wo(2); do_pv(H - 1)
        for g in range(3, 8):
            do_wo(g)
        out = jnp.concatenate([st['out', n] for n in range(8)], axis=1)
        outa[rows, :] = out[M:].astype(bf16)
        store_rows(s)
        return out[:M].astype(bf16).astype(f32)

    lax.fori_loop(0, NSEG, step, mem_ref[...].astype(f32))


def _kernel(xa_hbm, mem_hbm, wq_hbm, wk_hbm, wv_hbm, wo_hbm, xb_hbm, wr_hbm, wi_hbm, fd_hbm, mblk_hbm,
            out_hbm, mem_ref, raw, wqkv, wo, xa, xb, fd, mblk, wraw, wnyq, wst, zb, yb,
            sems, xsem, wsem, osem):
    def copy(src, dst, i, priority=0):
        c = pltpu.make_async_copy(src, dst, sems.at[i])
        c.start(priority=priority)
        return c

    def xb_copy(g):
        return pltpu.make_async_copy(xb_hbm.at[:, pl.ds(pl.multiple_of(g * G, G), G), :], xb.at[g], xsem.at[g])

    def yb_copy(g):
        return pltpu.make_async_copy(
            xb.at[g], out_hbm.at[:, pl.ds(pl.multiple_of(g * G, G), G), pl.ds(D, D)], osem.at[1])

    def w_copies(c):
        rows = pl.ds(pl.multiple_of(c * WC, WC), WC)
        return [pltpu.make_async_copy(w.bitcast(u32).at[rows],
                                      raw.at[c, j].reshape(WC, WP, DH).at[:, pl.ds(0, H // 2), :], wsem.at[c])
                for j, w in enumerate((wq_hbm, wk_hbm, wv_hbm))]

    c_fd = copy(fd_hbm, fd, 0)
    for g in range(R2 // G):
        xb_copy(g).start()

    def filter_copies():
        cps = []
        for c, w in enumerate((wr_hbm, wi_hbm)):
            cps.append(pltpu.make_async_copy(w.at[pl.ds(D // 2, 1), :], wnyq.at[c], sems.at[1 + c]))
            cps += [pltpu.make_async_copy(w.at[pl.ds(0, D // 2), pl.ds(t * 128, 128)], wraw.at[c * R1 + t],
                                          sems.at[3]) for t in range(R1)]
        return cps

    def wait_rows(g):
        xb_copy(g).wait()

        @pl.when(g == 2)
        def _():
            for cp in filter_copies():
                cp.start()

    def relayout(c, pieces):
        for cp in w_copies(c):
            cp.wait()

        def unit(j, t, i):
            dst = pl.ds(pl.multiple_of(c * (WC // 2) + t * 8, 8), 8)
            w = jnp.concatenate([raw[c, j, pl.ds((t * 16 + r) * WP + i, 8, stride=WP), :] for r in (0, 8)], axis=0)
            for hd, bits in ((2 * i, w << 16), (2 * i + 1, w & u32(0xFFFF0000))):
                wqkv[dst, pl.ds(hd * 384 + j * 128, 128)] = pltpu.bitcast(
                    pltpu.bitcast(bits, f32).astype(bf16), u32)

        units = [(j, t, i) for j in range(3) for t in range(WC // 16) for i in range(H // 2)]
        for n in range(pieces):
            for u in units[n * len(units) // pieces:(n + 1) * len(units) // pieces]:
                unit(*u)
            yield

    started = {}

    def prepare_filter():
        c_mb = copy(mblk_hbm, mblk, 4)
        for c in filter_copies():
            c.wait()
        for c in range(D // WC):
            for cp in w_copies(c):
                cp.start()
        started['mem'] = copy(mem_hbm, mem_ref, 5)
        started['xa'] = copy(xa_hbm.at[pl.ds(0, XA0 * SEG), :], xa.at[pl.ds(0, XA0 * SEG), :], 6)
        pairs = wraw.bitcast(u32)

        def prep(t, _):
            dst = pl.ds(pl.multiple_of(t * 64, 64), 64)
            for c in range(2):
                res = []
                for m in range(4):
                    w = pairs[c * R1 + t, pl.ds(m, 64, stride=4), :]
                    res += [pltpu.bitcast(w << 16, f32), pltpu.bitcast(w & u32(0xFFFF0000), f32)]
                for j in range(4):
                    lo, hi = _k1_pair(j)
                    tile = jnp.concatenate([res[lo], res[hi]], axis=0).T
                    wst[c, j, dst, :] = pltpu.bitcast(tile.astype(bf16), u32)
                last = wnyq[c, :, pl.ds(pl.multiple_of(t * 128, 128), 128)].astype(f32)
                wst[c, 4, dst, :] = pltpu.bitcast(jnp.broadcast_to(last, (128, 128)).T.astype(bf16), u32)
            return 0

        lax.fori_loop(0, S // 128, prep, 0)
        c_mb.wait()

    late = []

    def before_inv():
        late.extend(copy(wo_hbm.at[:, n * 128:(n + 1) * 128], wo.at[n], 7) for n in range(8))
        rest = pl.ds(XA0 * SEG, S - XA0 * SEG)
        late.append(copy(xa_hbm.at[rest, :], xa.at[rest, :], 8))

    c_fd.wait()
    _spectral_phase(xb, fd, mblk, wst, zb, yb, wait_rows, prepare_filter,
                    relayout, before_inv, lambda g, n: relayout(R1 // 2 + g, n))
    for c in late[:-1]:
        c.wait()
    started['xa'].wait()
    started['mem'].wait()
    for g in range(R2 // G):
        yb_copy(g).start()

    def before_step(s):
        @pl.when(s == XA0)
        def _():
            late[-1].wait()

    def out_copy(s):
        rows = pl.ds(pl.multiple_of(s * SEG, SEG), SEG)
        dst = out_hbm.at[s // 4, pl.ds(pl.multiple_of((s % 4) * SEG, SEG), SEG), pl.ds(0, D)]
        return pltpu.make_async_copy(xa.at[rows, :], dst, osem.at[0])

    _attention_phase(xa, mem_ref, wqkv, wo, xa, before_step, lambda s: out_copy(s).start())

    def drain(s, _):
        out_copy(s).wait()
        return 0

    lax.fori_loop(0, NSEG, drain, 0)
    for g in range(R2 // G):
        yb_copy(g).wait()


@jax.jit
def pallas_concat_heads__memory_aug_recurrent_mem_tr__spectral_gfnet__prompt_kernel(
    A_x, A_mem0, A_Wq, A_Wk, A_Wv, A_Wo, A_seg_len, B_x, B_w_r, B_w_i,
):
    del A_seg_len
    hbm = pl.BlockSpec(memory_space=pl.ANY)
    out = pl.pallas_call(
        _kernel,
        out_shape=jax.ShapeDtypeStruct((R1, R2, 2 * D), bf16),
        in_specs=[hbm] * 11,
        out_specs=hbm,
        scratch_shapes=[
            pltpu.VMEM((M, D), bf16),
            pltpu.VMEM((D // WC, 3, WC * WP, DH), u32),
            pltpu.VMEM((D // 2, H * 384), u32),
            pltpu.VMEM((8, H * DH, 128), bf16),
            pltpu.VMEM((S, D), bf16),
            pltpu.VMEM((R2 // G, R1, G, D), bf16),
            pltpu.VMEM((4, 256, 256), bf16),
            pltpu.VMEM((R1, 2 * R2, 2 * R2), bf16),
            pltpu.VMEM((2 * R1, D // 2, 128), bf16),
            pltpu.VMEM((2, 1, S), bf16),
            pltpu.VMEM((2, NT, S // 2, 128), u32),
            pltpu.VMEM((R1, 2 * R2, NT * 128), bf16),
            pltpu.VMEM((R1, 2 * R2, NT * 128), f32),
            pltpu.SemaphoreType.DMA((9,)),
            pltpu.SemaphoreType.DMA((R2 // G,)),
            pltpu.SemaphoreType.DMA((D // WC,)),
            pltpu.SemaphoreType.DMA((2,)),
        ],
        compiler_params=pltpu.CompilerParams(vmem_limit_bytes=120 * 2 ** 20),
    )(
        A_x.reshape(S, D), A_mem0.reshape(M, D),
        A_Wq, A_Wk, A_Wv,
        A_Wo.reshape(H * DH, D),
        B_x.reshape(R1, R2, D), B_w_r.T, B_w_i.T,
        jnp.asarray(_FD, dtype=bf16), jnp.asarray(_MBLK, dtype=bf16),
    )
    return out.reshape(1, S, 2 * D)
```

```python
import numpy as np
import jax
import jax.numpy as jnp
from jax import lax
import jax.experimental.pallas as pl
import jax.experimental.pallas.tpu as pltpu

S, D, H, DH, M, SEG = 2048, 1024, 32, 128, 8, 32
L = M + SEG
NSEG = S // SEG
DF = D // 2 + 1
R1, R2 = 16, 128
G = 16
WC = 64
WP = 24
UNROLL = 2
XA0 = 2
NT = 5
f32, bf16, u32 = jnp.float32, jnp.bfloat16, jnp.uint32


def _k1_pair(j):
    return j, (4 if j == 0 else 8 - j)


def _dft_constants():
    b = np.arange(128)[:, None]
    c = np.arange(64)[None, :]
    fd = np.zeros((4, 256, 256))
    for j in range(4):
        for half, k1 in enumerate(_k1_pair(j)):
            ang = 2.0 * np.pi * ((b * (k1 + 8 * c)) % D) / D
            co, si = np.cos(ang), np.sin(ang)
            re = slice(64 * half, 64 * half + 64)
            im = slice(128 + 64 * half, 128 + 64 * half + 64)
            if j == 0:
                rows = slice(128 * half, 128 * half + 128)
                fd[j, rows, re], fd[j, rows, im] = co, -si
            else:
                sg = 1.0 - 2.0 * half
                fd[j, :128, re], fd[j, :128, im] = co, -si
                fd[j, 128:, re], fd[j, 128:, im] = sg * si, sg * co
    fd[0, :128, 128] = 1.0 - 2.0 * (np.arange(128) % 2)
    f1 = np.arange(R1)[:, None, None]
    f2 = np.arange(R2)[None, :, None]
    t2 = np.arange(R2)[None, None, :]
    a = -2.0 * np.pi * ((t2 * (f1 + R1 * f2)) % S) / S
    mr, mi = np.cos(a), np.sin(a)
    blk = np.concatenate([np.concatenate([mr, -mi], 2), np.concatenate([mi, mr], 2)], 1)
    return fd.astype(np.float32), blk.astype(np.float32)


_FD, _MBLK = _dft_constants()
_RH = float(np.sqrt(0.5))


def _dot(a, b):
    return lax.dot_general(a, b, (((1,), (0,)), ((), ())), preferred_element_type=f32)


def _dot_nt(a, b):
    return lax.dot_general(a, b, (((1,), (1,)), ((), ())), preferred_element_type=f32)


def _dot_tn(a, b):
    return lax.dot_general(a, b, (((0,), (0,)), ((), ())), preferred_element_type=f32)


def _cmul_const(x, e, n, sign):
    xr, xi = x
    e = e % n
    if e == 0:
        return x
    if 4 * e == n:
        return (_neg(xi), xr) if sign > 0 else (xi, _neg(xr))
    c = float(np.cos(2.0 * np.pi * e / n))
    s = float(sign * np.sin(2.0 * np.pi * e / n))
    if xi is None:
        return xr * c, xr * s
    if 8 * e == n or 8 * e == 3 * n:
        if c * s > 0:
            return (xr - xi) * c, (xr + xi) * c
        return (xr + xi) * c, (xi - xr) * c
    return xr * c - xi * s, xr * s + xi * c


def _neg(a):
    return None if a is None else -a


def _add(a, b):
    return b if a is None else a if b is None else a + b


def _sub(a, b):
    return _neg(b) if a is None else a if b is None else a - b


def _fft(xs, sign):
    n = len(xs)
    if n == 1:
        return xs
    ev, od = _fft(xs[0::2], sign), _fft(xs[1::2], sign)
    out = [None] * n
    for j in range(n // 2):
        e = ev[j]
        if 4 * j == n:
            orr, oi = od[j]
            if sign > 0:
                out[j] = (_sub(e[0], oi), _add(e[1], orr))
                out[j + n // 2] = (_add(e[0], oi), _sub(e[1], orr))
            else:
                out[j] = (_add(e[0], oi), _sub(e[1], orr))
                out[j + n // 2] = (_sub(e[0], oi), _add(e[1], orr))
            continue
        t = _cmul_const(od[j], j, n, sign)
        out[j] = (_add(e[0], t[0]), _add(e[1], t[1]))
        out[j + n // 2] = (_sub(e[0], t[0]), _sub(e[1], t[1]))
    return out


def _rfft8(x):
    s04, d04, s26, d26 = x[0] + x[4], x[0] - x[4], x[2] + x[6], x[2] - x[6]
    s15, d15, s37, d37 = x[1] + x[5], x[1] - x[5], x[3] + x[7], x[3] - x[7]
    e, o = s04 + s26, s15 + s37
    p, q = (d15 - d37) * _RH, (d15 + d37) * _RH
    return [(e + o, e - o), (d04 + p, -(d26 + q)), (s04 - s26, s37 - s15), (d04 - p, d26 - q)]


def _rfft8_adjoint(g):
    (g0, g4), (r1, i1), (r2, i2), (r3, i3) = g
    e, o = g0 + g4, g0 - g4
    s04, s26, s15, s37 = e + r2, e - r2, o - i2, o + i2
    d04, d26 = r1 + r3, i3 - i1
    p, q = (r1 - r3) * _RH, (i1 + i3) * _RH
    d15, d37 = p - q, -(p + q)
    return [s04 + d04, s15 + d15, s26 + d26, s37 + d37, s04 - d04, s15 - d15, s26 - d26, s37 - d37]


def _spectral_phase(xb, fd, mblk, wst, zb, yb, wait_rows, before_mid, in_mid, before_inv, in_inv):
    def fwd(g, _):
        wait_rows(g)
        r0 = pl.multiple_of(g * G, G)
        lane0 = lax.broadcasted_iota(jnp.int32, (R1 * G, 128), 1) == 0
        xg = xb[g].reshape(R1 * G, D)
        us = _rfft8([xg[:, a * 128:(a + 1) * 128].astype(f32) for a in range(8)])
        nyq = None
        for j in range(NT):
            if j < 4:
                z = _dot(jnp.concatenate(us[j], axis=1).astype(bf16), fd[j])
                zr, zi = z[:, :128], z[:, 128:]
                if j == 0:
                    nyq = jnp.where(lane0, zi, 0.0)
                    zi = jnp.where(lane0, 0.0, zi)
                xs = [(zr[t * G:(t + 1) * G], zi[t * G:(t + 1) * G]) for t in range(R1)]
            else:
                xs = [(nyq[t * G:(t + 1) * G], None) for t in range(R1)]
            ys = _fft(xs, -1)
            for f1 in range(R1):
                yr, yi = ys[f1]
                yi = jnp.zeros_like(yr) if yi is None else yi
                zb[f1, pl.ds(r0, G), j * 128:(j + 1) * 128] = yr.astype(bf16)
                zb[f1, pl.ds(R2 + r0, G), j * 128:(j + 1) * 128] = yi.astype(bf16)
        return 0

    lax.fori_loop(0, R2 // G, fwd, 0)
    before_mid()

    def mid(g, _):
        side = in_mid(g, 4 * NT)
        lane = lax.broadcasted_iota(jnp.int32, (1, 128), 1)
        for half in range(2):
            f1 = 2 * g + half
            mb = mblk[f1]
            xs = []
            for j in range(NT):
                xs.append(_dot(mb, zb[f1, :, j * 128:(j + 1) * 128]))
                next(side)
            mbt = mb.T
            for j in range(NT):
                wr = wst[0, j, pl.ds(g, R2, stride=R1 // 2), :]
                wi = wst[1, j, pl.ds(g, R2, stride=R1 // 2), :]
                if half == 0:
                    wr, wi = wr << 16, wi << 16
                else:
                    wr, wi = wr & u32(0xFFFF0000), wi & u32(0xFFFF0000)
                if j == 0:
                    sc = jnp.where(lane == 0, 1.0 / (S * D), 2.0 / (S * D))
                else:
                    sc = (1.0 if j == 4 else 2.0) / (S * D)
                wr = pltpu.bitcast(wr, f32) * sc
                wi = pltpu.bitcast(wi, f32) * sc
                xr, xi = xs[j][:R2], xs[j][R2:]
                y = jnp.concatenate([xr * wr - xi * wi, xr * wi + xi * wr], axis=0).astype(bf16)
                yb[f1, :, j * 128:(j + 1) * 128] = _dot(mbt, y)
                next(side)
        return 0

    lax.fori_loop(0, R1 // 2, mid, 0)

    before_inv()

    def inv(g, _):
        side = in_inv(g, 5)
        r0 = pl.multiple_of(g * G, G)
        lane0 = lax.broadcasted_iota(jnp.int32, (R1 * G, 128), 1) == 0

        def tile(j):
            xs = [(yb[f1, pl.ds(r0, G), j * 128:(j + 1) * 128],
                   yb[f1, pl.ds(R2 + r0, G), j * 128:(j + 1) * 128]) for f1 in range(R1)]
            ys = _fft(xs, +1)
            return (jnp.concatenate([y[0] for y in ys], axis=0),
                    jnp.concatenate([y[1] for y in ys], axis=0))

        nyq = tile(4)[0]
        next(side)
        gs = []
        for j in range(4):
            yr, yi = tile(j)
            if j == 0:
                yi = jnp.where(lane0, nyq, yi)
            p = _dot_nt(jnp.concatenate([yr, yi], axis=1).astype(bf16), fd[j])
            gs.append((p[:, :128], p[:, 128:]))
            next(side)
        y = jnp.concatenate(_rfft8_adjoint(gs), axis=1).astype(bf16)
        xb[g] = y.reshape(R1, G, D)
        return 0

    lax.fori_loop(0, R2 // G, inv, 0)


def _attention_phase(xa, mem_ref, wqkv, wo, outa, before_step, store_rows):
    row = lax.broadcasted_iota(jnp.int32, (L, L), 0)
    col = lax.broadcasted_iota(jnp.int32, (L, L), 1)

    def step(s, mem):
        mask = (row < M) | (row >= col)
        rows = pl.ds(pl.multiple_of(s * SEG, SEG), SEG)
        h = jnp.concatenate([mem, xa[rows, :].astype(f32)], axis=0)
        st = {}

        def project(hd, lo, hi):
            return _dot(h[:, lo:hi], pltpu.bitcast(wqkv[lo // 2:hi // 2, hd * 384:(hd + 1) * 384], bf16))

        for hd in range(2):
            st['early', hd] = project(hd, 0, D // 2)

        def do_qkv(hd):
            qkv = st['early', hd] + project(hd, D // 2, D) if ('early', hd) in st else project(hd, 0, D)
            st['q', hd] = qkv[:, :128] * (DH ** -0.5)
            st['k', hd] = qkv[:, 128:256].astype(bf16)
            st['v', hd] = qkv[:, 256:].astype(bf16)

        def do_qk(hd):
            sc = jnp.where(mask, _dot_nt(st['q', hd], st['k', hd]), -1e9)
            e = jnp.exp(sc - jnp.max(sc, axis=1, keepdims=True))
            st['e', hd] = e
            den = jnp.sum(e, axis=1, keepdims=True)
            r = pl.reciprocal(den, approx=True)
            st['r', hd] = r * (2.0 - den * r)

        def do_pv(hd):
            st['o', hd] = _dot(st['e', hd], st['v', hd]) * st['r', hd]

        def do_wo(g, ng=4):
            o = jnp.concatenate([st['o', hd] for hd in range(g * ng, (g + 1) * ng)], axis=1)
            for n in range(8):
                r = _dot(o, pltpu.bitcast(wo[g * ng * 64:(g + 1) * ng * 64, n * 128:(n + 1) * 128], bf16))
                st['out', n] = st['out', n] + r if ('out', n) in st else r

        for t in range(H):
            do_qkv(t)
            if t >= 1: do_qk(t - 1)
            if t >= 3: do_pv(t - 3)
        do_wo(0); do_pv(H - 3)
        do_wo(1); do_qk(H - 1); do_pv(H - 2)
        do_wo(2)
        do_wo(3); do_pv(H - 1)
        do_wo(4); do_wo(5); do_wo(3, 8)
        out = jnp.concatenate([st['out', n] for n in range(8)], axis=1)
        outa[rows, :] = out[M:].astype(bf16)
        return out[:M].astype(bf16).astype(f32)

    def steps(i, mem):
        before_step(i * UNROLL)
        for u in range(UNROLL):
            mem = step(i * UNROLL + u, mem)
        store_rows(i)
        return mem

    lax.fori_loop(0, NSEG // UNROLL, steps, mem_ref[...].astype(f32))


def _kernel(xa_hbm, mem_hbm, wq_hbm, wk_hbm, wv_hbm, wo_hbm, xb_hbm, wr_hbm, wi_hbm, fd_hbm, mblk_hbm,
            out_hbm, mem_ref, raw, wqkv, wo, xa, ya, xb, fd, mblk, wraw, wnyq, wst, zb, yb,
            sems, xsem, wsem, osem):
    def copy(src, dst, i, priority=0):
        c = pltpu.make_async_copy(src, dst, sems.at[i])
        c.start(priority=priority)
        return c

    def xb_copy(g):
        return pltpu.make_async_copy(xb_hbm.at[:, pl.ds(pl.multiple_of(g * G, G), G), :], xb.at[g], xsem.at[g])

    def yb_copy(g):
        return pltpu.make_async_copy(
            xb.at[g], out_hbm.at[:, pl.ds(pl.multiple_of(g * G, G), G), pl.ds(D, D)], osem.at[1])

    def w_copies(c):
        rows = pl.ds(pl.multiple_of(c * WC, WC), WC)
        return [pltpu.make_async_copy(w.bitcast(u32).at[rows],
                                      raw.at[c, j].reshape(WC, WP, DH).at[:, pl.ds(0, H // 2), :], wsem.at[c])
                for j, w in enumerate((wq_hbm, wk_hbm, wv_hbm))]

    c_fd = copy(fd_hbm, fd, 0)
    for g in range(R2 // G):
        xb_copy(g).start()

    def filter_copies():
        cps = []
        for c, w in enumerate((wr_hbm, wi_hbm)):
            cps.append(pltpu.make_async_copy(w.at[pl.ds(D // 2, 1), :], wnyq.at[c], sems.at[1 + c]))
            cps += [pltpu.make_async_copy(w.at[pl.ds(0, D // 2), pl.ds(t * 128, 128)], wraw.at[c * R1 + t],
                                          sems.at[3]) for t in range(R1)]
        return cps

    def wait_rows(g):
        xb_copy(g).wait()

        @pl.when(g == 2)
        def _():
            for cp in filter_copies():
                cp.start()

    def relayout(c, pieces):
        for cp in w_copies(c):
            cp.wait()

        def unit(j, t, i):
            dst = pl.ds(pl.multiple_of(c * (WC // 2) + t * 8, 8), 8)
            w = jnp.concatenate([raw[c, j, pl.ds((t * 16 + r) * WP + i, 8, stride=WP), :] for r in (0, 8)], axis=0)
            for hd, bits in ((2 * i, w << 16), (2 * i + 1, w & u32(0xFFFF0000))):
                wqkv[dst, pl.ds(hd * 384 + j * 128, 128)] = pltpu.bitcast(
                    pltpu.bitcast(bits, f32).astype(bf16), u32)

        units = [(j, t, i) for j in range(3) for t in range(WC // 16) for i in range(H // 2)]
        for n in range(pieces):
            for u in units[n * len(units) // pieces:(n + 1) * len(units) // pieces]:
                unit(*u)
            yield

    started = {}

    def prepare_filter():
        c_mb = copy(mblk_hbm, mblk, 4)
        for c in filter_copies():
            c.wait()
        for c in range(D // WC):
            for cp in w_copies(c):
                cp.start()
        started['mem'] = copy(mem_hbm, mem_ref, 5)
        started['xa'] = copy(xa_hbm.at[pl.ds(0, XA0 * SEG), :], xa.at[pl.ds(0, XA0 * SEG), :], 6)
        pairs = wraw.bitcast(u32)

        def prep(t, _):
            dst = pl.ds(pl.multiple_of(t * 64, 64), 64)
            for c in range(2):
                res = []
                for m in range(4):
                    w = pairs[c * R1 + t, pl.ds(m, 64, stride=4), :]
                    res += [pltpu.bitcast(w << 16, f32), pltpu.bitcast(w & u32(0xFFFF0000), f32)]
                for j in range(4):
                    lo, hi = _k1_pair(j)
                    tile = jnp.concatenate([res[lo], res[hi]], axis=0).T
                    wst[c, j, dst, :] = pltpu.bitcast(tile.astype(bf16), u32)
                last = wnyq[c, :, pl.ds(pl.multiple_of(t * 128, 128), 128)].astype(f32)
                wst[c, 4, dst, :] = pltpu.bitcast(jnp.broadcast_to(last, (128, 128)).T.astype(bf16), u32)
            return 0

        lax.fori_loop(0, S // 128, prep, 0)
        c_mb.wait()

    late = []

    def before_inv():
        late.append(copy(wo_hbm.bitcast(u32), wo, 7))
        rest = pl.ds(XA0 * SEG, S - XA0 * SEG)
        late.append(copy(xa_hbm.at[rest, :], xa.at[rest, :], 8))

    c_fd.wait()
    _spectral_phase(xb, fd, mblk, wst, zb, yb, wait_rows, prepare_filter,
                    relayout, before_inv, lambda g, n: relayout(R1 // 2 + g, n))
    for c in late[:-1]:
        c.wait()
    started['xa'].wait()
    started['mem'].wait()
    for g in range(R2 // G):
        yb_copy(g).start()

    def before_step(s):
        @pl.when(s == XA0)
        def _():
            late[-1].wait()

    def out_copy(i):
        n = UNROLL * SEG
        dst = out_hbm.at[i // (R2 // n), pl.ds(pl.multiple_of((i % (R2 // n)) * n, n), n), pl.ds(0, D)]
        return pltpu.make_async_copy(ya.at[pl.ds(pl.multiple_of(i * n, n), n), :], dst, osem.at[0])

    _attention_phase(xa, mem_ref, wqkv, wo, ya, before_step, lambda i: out_copy(i).start())

    def drain(i, _):
        out_copy(i).wait()
        return 0

    lax.fori_loop(0, NSEG // UNROLL, drain, 0)
    for g in range(R2 // G):
        yb_copy(g).wait()


@jax.jit
def pallas_concat_heads__memory_aug_recurrent_mem_tr__spectral_gfnet__prompt_kernel(
    A_x, A_mem0, A_Wq, A_Wk, A_Wv, A_Wo, A_seg_len, B_x, B_w_r, B_w_i,
):
    del A_seg_len
    hbm = pl.BlockSpec(memory_space=pl.ANY)
    out = pl.pallas_call(
        _kernel,
        out_shape=jax.ShapeDtypeStruct((R1, R2, 2 * D), bf16),
        in_specs=[hbm] * 11,
        out_specs=hbm,
        scratch_shapes=[
            pltpu.VMEM((M, D), bf16),
            pltpu.VMEM((D // WC, 3, WC * WP, DH), u32),
            pltpu.VMEM((D // 2, H * 384), u32),
            pltpu.VMEM((H * DH // 2, D), u32),
            pltpu.VMEM((S, D), bf16),
            pltpu.VMEM((S, D), bf16),
            pltpu.VMEM((R2 // G, R1, G, D), bf16),
            pltpu.VMEM((4, 256, 256), bf16),
            pltpu.VMEM((R1, 2 * R2, 2 * R2), bf16),
            pltpu.VMEM((2 * R1, D // 2, 128), bf16),
            pltpu.VMEM((2, 1, S), bf16),
            pltpu.VMEM((2, NT, S // 2, 128), u32),
            pltpu.VMEM((R1, 2 * R2, NT * 128), bf16),
            pltpu.VMEM((R1, 2 * R2, NT * 128), f32),
            pltpu.SemaphoreType.DMA((9,)),
            pltpu.SemaphoreType.DMA((R2 // G,)),
            pltpu.SemaphoreType.DMA((D // WC,)),
            pltpu.SemaphoreType.DMA((2,)),
        ],
        compiler_params=pltpu.CompilerParams(vmem_limit_bytes=120 * 2 ** 20),
    )(
        A_x.reshape(S, D), A_mem0.reshape(M, D),
        A_Wq, A_Wk, A_Wv,
        A_Wo.reshape(H * DH, D),
        B_x.reshape(R1, R2, D), B_w_r.T, B_w_i.T,
        jnp.asarray(_FD, dtype=bf16), jnp.asarray(_MBLK, dtype=bf16),
    )
    return out.reshape(1, S, 2 * D)
```

```python
import functools

import numpy as np
import jax
import jax.numpy as jnp
from jax import lax
import jax.experimental.pallas as pl
import jax.experimental.pallas.tpu as pltpu

S, D, H, DH, M, SEG = 2048, 1024, 32, 128, 8, 32
L = M + SEG
NSEG = S // SEG
DF = D // 2 + 1
R1, R2 = 16, 128
G = 16
HG = 16
UNROLL = 2
PRE = 22
NT = 5
f32, bf16, u32 = jnp.float32, jnp.bfloat16, jnp.uint32


def _k1_pair(j):
    return j, (4 if j == 0 else 8 - j)


def _dft_constants():
    b = np.arange(128)[:, None]
    c = np.arange(64)[None, :]
    fd = np.zeros((4, 256, 256))
    for j in range(4):
        for half, k1 in enumerate(_k1_pair(j)):
            ang = 2.0 * np.pi * ((b * (k1 + 8 * c)) % D) / D
            co, si = np.cos(ang), np.sin(ang)
            re = slice(64 * half, 64 * half + 64)
            im = slice(128 + 64 * half, 128 + 64 * half + 64)
            if j == 0:
                rows = slice(128 * half, 128 * half + 128)
                fd[j, rows, re], fd[j, rows, im] = co, -si
            else:
                sg = 1.0 - 2.0 * half
                fd[j, :128, re], fd[j, :128, im] = co, -si
                fd[j, 128:, re], fd[j, 128:, im] = sg * si, sg * co
    fd[0, :128, 128] = 1.0 - 2.0 * (np.arange(128) % 2)
    f1 = np.arange(R1)[:, None, None]
    f2 = np.arange(R2)[None, :, None]
    t2 = np.arange(R2)[None, None, :]
    a = -2.0 * np.pi * ((t2 * (f1 + R1 * f2)) % S) / S
    mr, mi = np.cos(a), np.sin(a)
    blk = np.concatenate([np.concatenate([mr, -mi], 2), np.concatenate([mi, mr], 2)], 1)
    return fd.astype(np.float32), blk.astype(np.float32)


_FD, _MBLK = _dft_constants()
_RH = float(np.sqrt(0.5))


def _dot(a, b):
    return lax.dot_general(a, b, (((1,), (0,)), ((), ())), preferred_element_type=f32)


def _dot_nt(a, b):
    return lax.dot_general(a, b, (((1,), (1,)), ((), ())), preferred_element_type=f32)


def _dot_tn(a, b):
    return lax.dot_general(a, b, (((0,), (0,)), ((), ())), preferred_element_type=f32)


def _cmul_const(x, e, n, sign):
    xr, xi = x
    e = e % n
    if e == 0:
        return x
    if 4 * e == n:
        return (_neg(xi), xr) if sign > 0 else (xi, _neg(xr))
    c = float(np.cos(2.0 * np.pi * e / n))
    s = float(sign * np.sin(2.0 * np.pi * e / n))
    if xi is None:
        return xr * c, xr * s
    if 8 * e == n or 8 * e == 3 * n:
        if c * s > 0:
            return (xr - xi) * c, (xr + xi) * c
        return (xr + xi) * c, (xi - xr) * c
    return xr * c - xi * s, xr * s + xi * c


def _neg(a):
    return None if a is None else -a


def _add(a, b):
    return b if a is None else a if b is None else a + b


def _sub(a, b):
    return _neg(b) if a is None else a if b is None else a - b


def _fft(xs, sign):
    n = len(xs)
    if n == 1:
        return xs
    ev, od = _fft(xs[0::2], sign), _fft(xs[1::2], sign)
    out = [None] * n
    for j in range(n // 2):
        e = ev[j]
        if 4 * j == n:
            orr, oi = od[j]
            if sign > 0:
                out[j] = (_sub(e[0], oi), _add(e[1], orr))
                out[j + n // 2] = (_add(e[0], oi), _sub(e[1], orr))
            else:
                out[j] = (_add(e[0], oi), _sub(e[1], orr))
                out[j + n // 2] = (_sub(e[0], oi), _add(e[1], orr))
            continue
        t = _cmul_const(od[j], j, n, sign)
        out[j] = (_add(e[0], t[0]), _add(e[1], t[1]))
        out[j + n // 2] = (_sub(e[0], t[0]), _sub(e[1], t[1]))
    return out


def _rfft8(x):
    s04, d04, s26, d26 = x[0] + x[4], x[0] - x[4], x[2] + x[6], x[2] - x[6]
    s15, d15, s37, d37 = x[1] + x[5], x[1] - x[5], x[3] + x[7], x[3] - x[7]
    e, o = s04 + s26, s15 + s37
    p, q = (d15 - d37) * _RH, (d15 + d37) * _RH
    return [(e + o, e - o), (d04 + p, -(d26 + q)), (s04 - s26, s37 - s15), (d04 - p, d26 - q)]


def _rfft8_adjoint(g):
    (g0, g4), (r1, i1), (r2, i2), (r3, i3) = g
    e, o = g0 + g4, g0 - g4
    s04, s26, s15, s37 = e + r2, e - r2, o - i2, o + i2
    d04, d26 = r1 + r3, i3 - i1
    p, q = (r1 - r3) * _RH, (i1 + i3) * _RH
    d15, d37 = p - q, -(p + q)
    return [s04 + d04, s15 + d15, s26 + d26, s37 + d37, s04 - d04, s15 - d15, s26 - d26, s37 - d37]


def _spectral_phase(xb, fd, mblk, wst, zb, yb, wait_rows, before_mid):
    def fwd(g, _):
        wait_rows(g)
        r0 = pl.multiple_of(g * G, G)
        lane0 = lax.broadcasted_iota(jnp.int32, (R1 * G, 128), 1) == 0
        xg = xb[g].reshape(R1 * G, D)
        us = _rfft8([xg[:, a * 128:(a + 1) * 128].astype(f32) for a in range(8)])
        nyq = None
        for j in range(NT):
            if j < 4:
                z = _dot(jnp.concatenate(us[j], axis=1).astype(bf16), fd[j])
                zr, zi = z[:, :128], z[:, 128:]
                if j == 0:
                    nyq = jnp.where(lane0, zi, 0.0)
                    zi = jnp.where(lane0, 0.0, zi)
                xs = [(zr[t * G:(t + 1) * G], zi[t * G:(t + 1) * G]) for t in range(R1)]
            else:
                xs = [(nyq[t * G:(t + 1) * G], None) for t in range(R1)]
            ys = _fft(xs, -1)
            for f1 in range(R1):
                yr, yi = ys[f1]
                yi = jnp.zeros_like(yr) if yi is None else yi
                zb[f1, pl.ds(r0, G), j * 128:(j + 1) * 128] = yr.astype(bf16)
                zb[f1, pl.ds(R2 + r0, G), j * 128:(j + 1) * 128] = yi.astype(bf16)
        return 0

    lax.fori_loop(0, R2 // G, fwd, 0)
    before_mid()

    def mid(g, _):
        lane = lax.broadcasted_iota(jnp.int32, (1, 128), 1)
        for half in range(2):
            f1 = 2 * g + half
            mb = mblk[f1]
            xs = []
            for j in range(NT):
                xs.append(_dot(mb, zb[f1, :, j * 128:(j + 1) * 128]))
            mbt = mb.T
            for j in range(NT):
                wr = wst[0, j, pl.ds(g, R2, stride=R1 // 2), :]
                wi = wst[1, j, pl.ds(g, R2, stride=R1 // 2), :]
                if half == 0:
                    wr, wi = wr << 16, wi << 16
                else:
                    wr, wi = wr & u32(0xFFFF0000), wi & u32(0xFFFF0000)
                if j == 0:
                    sc = jnp.where(lane == 0, 1.0 / (S * D), 2.0 / (S * D))
                else:
                    sc = (1.0 if j == 4 else 2.0) / (S * D)
                wr = pltpu.bitcast(wr, f32) * sc
                wi = pltpu.bitcast(wi, f32) * sc
                xr, xi = xs[j][:R2], xs[j][R2:]
                y = jnp.concatenate([xr * wr - xi * wi, xr * wi + xi * wr], axis=0).astype(bf16)
                yb[f1, :, j * 128:(j + 1) * 128] = _dot(mbt, y)
        return 0

    lax.fori_loop(0, R1 // 2, mid, 0)

    def inv(g, _):
        r0 = pl.multiple_of(g * G, G)
        lane0 = lax.broadcasted_iota(jnp.int32, (R1 * G, 128), 1) == 0

        def tile(j):
            xs = [(yb[f1, pl.ds(r0, G), j * 128:(j + 1) * 128],
                   yb[f1, pl.ds(R2 + r0, G), j * 128:(j + 1) * 128]) for f1 in range(R1)]
            ys = _fft(xs, +1)
            return (jnp.concatenate([y[0] for y in ys], axis=0),
                    jnp.concatenate([y[1] for y in ys], axis=0))

        nyq = tile(4)[0]
        gs = []
        for j in range(4):
            yr, yi = tile(j)
            if j == 0:
                yi = jnp.where(lane0, nyq, yi)
            p = _dot_nt(jnp.concatenate([yr, yi], axis=1).astype(bf16), fd[j])
            gs.append((p[:, :128], p[:, 128:]))
        y = jnp.concatenate(_rfft8_adjoint(gs), axis=1).astype(bf16)
        xb[g] = y.reshape(R1, G, D)
        return 0

    lax.fori_loop(0, R2 // G, inv, 0)


def _attention_phase(xa, mem_ref, wqkv, pre, wo, outa, before_rest, store_rows):
    row = lax.broadcasted_iota(jnp.int32, (L, L), 0)
    col = lax.broadcasted_iota(jnp.int32, (L, L), 1)

    def step(s, mem, ahead):
        mask = (row < M) | (row >= col)
        rows = pl.ds(pl.multiple_of(s * SEG, SEG), SEG)
        h = jnp.concatenate([mem, xa[rows, :].astype(f32)], axis=0)
        if ahead:
            h = h[:L - 8]
        st = {}

        def project(hd, lo, hi):
            w = jnp.concatenate([wqkv[hd, j, lo // 2:hi // 2, :] for j in range(3)], axis=1)
            return _dot(h[:, lo:hi], pltpu.bitcast(w, bf16))

        for hd in range(2):
            st['early', hd] = project(hd, 0, D // 2)

        def do_qkv(hd):
            qkv = st['early', hd] + project(hd, D // 2, D) if ('early', hd) in st else project(hd, 0, D)
            if ahead:
                r8 = pl.ds(pl.multiple_of(s * 8, 8), 8)
                qkv = jnp.concatenate(
                    [qkv, jnp.concatenate([pre[hd, j, r8, :] for j in range(3)], axis=1)], axis=0)
            st['q', hd] = qkv[:, :128] * (DH ** -0.5)
            st['k', hd] = qkv[:, 128:256].astype(bf16)
            st['v', hd] = qkv[:, 256:].astype(bf16)

        def do_qk(hd):
            sc = jnp.where(mask, _dot_nt(st['q', hd], st['k', hd]), -1e9)
            e = jnp.exp(sc - jnp.max(sc, axis=1, keepdims=True))
            st['e', hd] = e
            den = jnp.sum(e, axis=1, keepdims=True)
            r = pl.reciprocal(den, approx=True)
            st['r', hd] = r * (2.0 - den * r)

        def do_pv(hd):
            st['o', hd] = _dot(st['e', hd], st['v', hd]) * st['r', hd]

        def do_wo(g, ng=4):
            o = jnp.concatenate([st['o', hd] for hd in range(g * ng, (g + 1) * ng)], axis=1)
            for n in range(8):
                r = _dot(o, pltpu.bitcast(wo[g * ng * 64:(g + 1) * ng * 64, n * 128:(n + 1) * 128], bf16))
                st['out', n] = st['out', n] + r if ('out', n) in st else r

        for t in range(H):
            do_qkv(t)
            if t >= 1: do_qk(t - 1)
            if t >= 3: do_pv(t - 3)
        do_wo(0); do_pv(H - 3)
        do_wo(1); do_qk(H - 1); do_pv(H - 2)
        do_wo(2)
        do_wo(3); do_pv(H - 1)
        do_wo(4); do_wo(5); do_wo(3, 8)
        out = jnp.concatenate([st['out', n] for n in range(8)], axis=1)
        outa[rows, :] = out[M:].astype(bf16)
        return out[:M].astype(bf16).astype(f32)

    def steps(ahead, i, mem):
        for u in range(UNROLL):
            mem = step(i * UNROLL + u, mem, ahead)
        store_rows(i)
        return mem

    mem = lax.fori_loop(0, PRE // UNROLL, functools.partial(steps, True), mem_ref[...].astype(f32))
    before_rest()
    lax.fori_loop(PRE // UNROLL, NSEG // UNROLL, functools.partial(steps, False), mem)


def _kernel(xa_hbm, mem_hbm, wq_hbm, wk_hbm, wv_hbm, wo_hbm, xb_hbm, wr_hbm, wi_hbm, fd_hbm, mblk_hbm,
            out_hbm, mem_ref, raw, wqkv, xpre, pre, wo, xa, ya, xb, fd, mblk, wraw, wnyq, wst, zb, yb,
            sems, xsem, wsem, osem):
    def copy(src, dst, i, priority=0):
        c = pltpu.make_async_copy(src, dst, sems.at[i])
        c.start(priority=priority)
        return c

    def xb_copy(g):
        return pltpu.make_async_copy(xb_hbm.at[:, pl.ds(pl.multiple_of(g * G, G), G), :], xb.at[g], xsem.at[g])

    def yb_copy(g):
        return pltpu.make_async_copy(
            xb.at[g], out_hbm.at[:, pl.ds(pl.multiple_of(g * G, G), G), pl.ds(D, D)], osem.at[1])

    def w_copy(j, hg):
        src = (wq_hbm, wk_hbm, wv_hbm)[j].bitcast(u32).at[:, pl.ds(hg * (HG // 2), HG // 2), :]
        c = j * (H // HG) + hg
        return pltpu.make_async_copy(src, raw.at[c].reshape(D, HG // 2, DH), wsem.at[c])

    c_fd = copy(fd_hbm, fd, 0)
    xb_copy(0).start()
    c_fd.wait()
    for g in range(1, R2 // G):
        xb_copy(g).start()

    def filter_copies():
        cps = []
        for c, w in enumerate((wr_hbm, wi_hbm)):
            cps.append(pltpu.make_async_copy(w.at[pl.ds(D // 2, 1), :], wnyq.at[c], sems.at[1 + c]))
            cps += [pltpu.make_async_copy(w.at[pl.ds(0, D // 2), pl.ds(t * 128, 128)], wraw.at[c * R1 + t],
                                          sems.at[3]) for t in range(R1)]
        return cps

    def wait_rows(g):
        xb_copy(g).wait()

        @pl.when(g == 2)
        def _():
            for cp in filter_copies():
                cp.start()

    started = {}

    def prepare_filter():
        c_mb = copy(mblk_hbm, mblk, 4)
        started['mem'] = copy(mem_hbm, mem_ref, 5)
        started['xa'] = copy(xa_hbm.at[pl.ds(0, PRE * SEG), :], xa.at[pl.ds(0, PRE * SEG), :], 6)
        for c in filter_copies():
            c.wait()
        for j in range(3):
            for hg in range(H // HG):
                w_copy(j, hg).start()
        started['wo'] = copy(wo_hbm.bitcast(u32), wo, 7)
        pairs = wraw.bitcast(u32)

        def prep(t, _):
            dst = pl.ds(pl.multiple_of(t * 64, 64), 64)
            for c in range(2):
                res = []
                for m in range(4):
                    w = pairs[c * R1 + t, pl.ds(m, 64, stride=4), :]
                    res += [pltpu.bitcast(w << 16, f32), pltpu.bitcast(w & u32(0xFFFF0000), f32)]
                for j in range(4):
                    lo, hi = _k1_pair(j)
                    tile = jnp.concatenate([res[lo], res[hi]], axis=0).T
                    wst[c, j, dst, :] = pltpu.bitcast(tile.astype(bf16), u32)
                last = wnyq[c, :, pl.ds(pl.multiple_of(t * 128, 128), 128)].astype(f32)
                wst[c, 4, dst, :] = pltpu.bitcast(jnp.broadcast_to(last, (128, 128)).T.astype(bf16), u32)
            return 0

        lax.fori_loop(0, S // 128, prep, 0)
        c_mb.wait()

    _spectral_phase(xb, fd, mblk, wst, zb, yb, wait_rows, prepare_filter)

    started['xa'].wait()
    for s in range(PRE):
        xpre[s * 8:(s + 1) * 8, :] = xa[s * SEG + 16:(s + 1) * SEG, :].astype(f32)[8:]

    def relayout(c, _):
        pltpu.make_async_copy(raw.at[c], raw.at[c], wsem.at[c]).wait()
        j, h0 = c // (H // HG), (c % (H // HG)) * HG
        for i in range(HG // 2):
            w = raw[c, pl.ds(i, D, stride=HG // 2), :]
            for hd, bits in ((2 * i, w << 16), (2 * i + 1, w & u32(0xFFFF0000))):
                panel = pltpu.bitcast(bits, f32).astype(bf16)
                wqkv[h0 + hd, j] = pltpu.bitcast(panel, u32)
                pre[h0 + hd, j] = _dot(xpre[...], panel)
        return 0

    lax.fori_loop(0, 3 * H // HG, relayout, 0)
    started['mem'].wait()
    started['wo'].wait()
    rest = pl.ds(PRE * SEG, S - PRE * SEG)
    c_rest = copy(xa_hbm.at[rest, :], xa.at[rest, :], 8)
    for g in range(R2 // G):
        yb_copy(g).start()

    def out_copy(i):
        n = UNROLL * SEG
        dst = out_hbm.at[i // (R2 // n), pl.ds(pl.multiple_of((i % (R2 // n)) * n, n), n), pl.ds(0, D)]
        return pltpu.make_async_copy(ya.at[pl.ds(pl.multiple_of(i * n, n), n), :], dst, osem.at[0])

    _attention_phase(xa, mem_ref, wqkv, pre, wo, ya, c_rest.wait, lambda i: out_copy(i).start())

    def drain(i, _):
        out_copy(i).wait()
        return 0

    lax.fori_loop(0, NSEG // UNROLL, drain, 0)
    for g in range(R2 // G):
        yb_copy(g).wait()


@jax.jit
def pallas_concat_heads__memory_aug_recurrent_mem_tr__spectral_gfnet__prompt_kernel(
    A_x, A_mem0, A_Wq, A_Wk, A_Wv, A_Wo, A_seg_len, B_x, B_w_r, B_w_i,
):
    del A_seg_len
    hbm = pl.BlockSpec(memory_space=pl.ANY)
    out = pl.pallas_call(
        _kernel,
        out_shape=jax.ShapeDtypeStruct((R1, R2, 2 * D), bf16),
        in_specs=[hbm] * 11,
        out_specs=hbm,
        scratch_shapes=[
            pltpu.VMEM((M, D), bf16),
            pltpu.VMEM((3 * H // HG, D * HG // 2, DH), u32),
            pltpu.VMEM((H, 3, D // 2, DH), u32),
            pltpu.VMEM((PRE * 8, D), f32),
            pltpu.VMEM((H, 3, PRE * 8, DH), f32),
            pltpu.VMEM((H * DH // 2, D), u32),
            pltpu.VMEM((S, D), bf16),
            pltpu.VMEM((S, D), bf16),
            pltpu.VMEM((R2 // G, R1, G, D), bf16),
            pltpu.VMEM((4, 256, 256), bf16),
            pltpu.VMEM((R1, 2 * R2, 2 * R2), bf16),
            pltpu.VMEM((2 * R1, D // 2, 128), bf16),
            pltpu.VMEM((2, 1, S), bf16),
            pltpu.VMEM((2, NT, S // 2, 128), u32),
            pltpu.VMEM((R1, 2 * R2, NT * 128), bf16),
            pltpu.VMEM((R1, 2 * R2, NT * 128), f32),
            pltpu.SemaphoreType.DMA((9,)),
            pltpu.SemaphoreType.DMA((R2 // G,)),
            pltpu.SemaphoreType.DMA((3 * H // HG,)),
            pltpu.SemaphoreType.DMA((2,)),
        ],
        compiler_params=pltpu.CompilerParams(vmem_limit_bytes=120 * 2 ** 20),
    )(
        A_x.reshape(S, D), A_mem0.reshape(M, D),
        A_Wq, A_Wk, A_Wv,
        A_Wo.reshape(H * DH, D),
        B_x.reshape(R1, R2, D), B_w_r.T, B_w_i.T,
        jnp.asarray(_FD, dtype=bf16), jnp.asarray(_MBLK, dtype=bf16),
    )
    return out.reshape(1, S, 2 * D)
```

```python
import functools

import numpy as np
import jax
import jax.numpy as jnp
from jax import lax
import jax.experimental.pallas as pl
import jax.experimental.pallas.tpu as pltpu

S, D, H, DH, M, SEG = 2048, 1024, 32, 128, 8, 32
L = M + SEG
NSEG = S // SEG
DF = D // 2 + 1
R1, R2 = 16, 128
G = 16
HG = 16
UNROLL = 2
PRE = 30
XA0 = 4
NT = 5
f32, bf16, u32 = jnp.float32, jnp.bfloat16, jnp.uint32


def _k1_pair(j):
    return j, (4 if j == 0 else 8 - j)


def _dft_constants():
    b = np.arange(128)[:, None]
    c = np.arange(64)[None, :]
    fd = np.zeros((4, 256, 256))
    for j in range(4):
        for half, k1 in enumerate(_k1_pair(j)):
            ang = 2.0 * np.pi * ((b * (k1 + 8 * c)) % D) / D
            co, si = np.cos(ang), np.sin(ang)
            re = slice(64 * half, 64 * half + 64)
            im = slice(128 + 64 * half, 128 + 64 * half + 64)
            if j == 0:
                rows = slice(128 * half, 128 * half + 128)
                fd[j, rows, re], fd[j, rows, im] = co, -si
            else:
                sg = 1.0 - 2.0 * half
                fd[j, :128, re], fd[j, :128, im] = co, -si
                fd[j, 128:, re], fd[j, 128:, im] = sg * si, sg * co
    fd[0, :128, 128] = 1.0 - 2.0 * (np.arange(128) % 2)
    n = np.arange(R2)
    a = -2.0 * np.pi * np.concatenate([(n[:, None] * n[None, :]) % R2 / R2,
                                       np.arange(R1)[:, None] * n[None, :] / S], axis=0)
    return fd.astype(np.float32), np.stack([np.cos(a), np.sin(a)]).astype(np.float32)


_FD, _FS = _dft_constants()
_RH = float(np.sqrt(0.5))


def _dot(a, b):
    return lax.dot_general(a, b, (((1,), (0,)), ((), ())), preferred_element_type=f32)


def _dot_nt(a, b):
    return lax.dot_general(a, b, (((1,), (1,)), ((), ())), preferred_element_type=f32)


def _dot_tn(a, b):
    return lax.dot_general(a, b, (((0,), (0,)), ((), ())), preferred_element_type=f32)


def _cmul_const(x, e, n, sign):
    xr, xi = x
    e = e % n
    if e == 0:
        return x
    if 4 * e == n:
        return (_neg(xi), xr) if sign > 0 else (xi, _neg(xr))
    c = float(np.cos(2.0 * np.pi * e / n))
    s = float(sign * np.sin(2.0 * np.pi * e / n))
    if xi is None:
        return xr * c, xr * s
    if 8 * e == n or 8 * e == 3 * n:
        if c * s > 0:
            return (xr - xi) * c, (xr + xi) * c
        return (xr + xi) * c, (xi - xr) * c
    return xr * c - xi * s, xr * s + xi * c


def _neg(a):
    return None if a is None else -a


def _add(a, b):
    return b if a is None else a if b is None else a + b


def _sub(a, b):
    return _neg(b) if a is None else a if b is None else a - b


def _fft(xs, sign):
    n = len(xs)
    if n == 1:
        return xs
    ev, od = _fft(xs[0::2], sign), _fft(xs[1::2], sign)
    out = [None] * n
    for j in range(n // 2):
        e = ev[j]
        if 4 * j == n:
            orr, oi = od[j]
            if sign > 0:
                out[j] = (_sub(e[0], oi), _add(e[1], orr))
                out[j + n // 2] = (_add(e[0], oi), _sub(e[1], orr))
            else:
                out[j] = (_add(e[0], oi), _sub(e[1], orr))
                out[j + n // 2] = (_sub(e[0], oi), _add(e[1], orr))
            continue
        t = _cmul_const(od[j], j, n, sign)
        out[j] = (_add(e[0], t[0]), _add(e[1], t[1]))
        out[j + n // 2] = (_sub(e[0], t[0]), _sub(e[1], t[1]))
    return out


def _rfft8(x):
    s04, d04, s26, d26 = x[0] + x[4], x[0] - x[4], x[2] + x[6], x[2] - x[6]
    s15, d15, s37, d37 = x[1] + x[5], x[1] - x[5], x[3] + x[7], x[3] - x[7]
    e, o = s04 + s26, s15 + s37
    p, q = (d15 - d37) * _RH, (d15 + d37) * _RH
    return [(e + o, e - o), (d04 + p, -(d26 + q)), (s04 - s26, s37 - s15), (d04 - p, d26 - q)]


def _rfft8_adjoint(g):
    (g0, g4), (r1, i1), (r2, i2), (r3, i3) = g
    e, o = g0 + g4, g0 - g4
    s04, s26, s15, s37 = e + r2, e - r2, o - i2, o + i2
    d04, d26 = r1 + r3, i3 - i1
    p, q = (r1 - r3) * _RH, (i1 + i3) * _RH
    d15, d37 = p - q, -(p + q)
    return [s04 + d04, s15 + d15, s26 + d26, s37 + d37, s04 - d04, s15 - d15, s26 - d26, s37 - d37]


def _spectral_phase(xb, fd, fs, wst, zb, wait_rows, prepare_filter):
    groups = [(h, t1) for h in range(G // 8) for t1 in range(R1)]

    def fwd(g, _):
        wait_rows(g)
        r0 = pl.multiple_of(g * G, G)
        lane0 = lax.broadcasted_iota(jnp.int32, (R1 * G, 128), 1) == 0
        xg = [xb[g, t1].astype(f32) for t1 in range(R1)]
        xg = jnp.concatenate([xg[t1][h * 8:(h + 1) * 8] for h, t1 in groups], axis=0)
        us = _rfft8([xg[:, a * 128:(a + 1) * 128] for a in range(8)])
        us = [jnp.concatenate(u, axis=1).astype(bf16) for u in us]
        nyq = None
        for j in range(NT):
            if j < 4:
                z = _dot(us[j], fd[j])
                zr, zi = z[:, :128], z[:, 128:]
                if j == 0:
                    nyq = jnp.where(lane0, zi, 0.0)
                    zi = jnp.where(lane0, 0.0, zi)
                xs = [(zr[n * 8:(n + 1) * 8], zi[n * 8:(n + 1) * 8]) for n in range(len(groups))]
            else:
                xs = [(nyq[n * 8:(n + 1) * 8], None) for n in range(len(groups))]
            for h in range(G // 8):
                for f1, (yr, yi) in enumerate(_fft(xs[h * R1:(h + 1) * R1], -1)):
                    zb[f1, pl.ds(r0 + h * 8, 8), j * 128:(j + 1) * 128] = yr
                    zb[f1, pl.ds(R2 + r0 + h * 8, 8), j * 128:(j + 1) * 128] = (
                        jnp.zeros_like(yr) if yi is None else yi)
        return 0

    lax.fori_loop(0, R2 // G, fwd, 0)

    def dft_block(f1):
        cr, ci = fs[0, :R2, :], fs[1, :R2, :]
        tr, ti = fs[0, pl.ds(R2 + f1, 1), :], fs[1, pl.ds(R2 + f1, 1), :]
        mr, mi = cr * tr - ci * ti, cr * ti + ci * tr
        return jnp.concatenate([jnp.concatenate([mr, -mi], axis=1),
                                jnp.concatenate([mi, mr], axis=1)], axis=0).astype(bf16)

    def dft(g, _):
        side = prepare_filter(g)
        for f1 in (2 * g, 2 * g + 1):
            mb = dft_block(f1)
            for j in range(NT):
                cols = slice(j * 128, (j + 1) * 128)
                zb[f1, :, cols] = _dot(mb, zb[f1, :, cols].astype(bf16))
                next(side)
        return 0

    lax.fori_loop(0, R1 // 2, dft, 0)

    def idft(g, _):
        lane = lax.broadcasted_iota(jnp.int32, (1, 128), 1)
        for half in range(2):
            f1 = 2 * g + half
            mbt = dft_block(f1).T
            for j in range(NT):
                cols = slice(j * 128, (j + 1) * 128)
                wr = wst[0, j, pl.ds(g, R2, stride=R1 // 2), :]
                wi = wst[1, j, pl.ds(g, R2, stride=R1 // 2), :]
                if half == 0:
                    wr, wi = wr << 16, wi << 16
                else:
                    wr, wi = wr & u32(0xFFFF0000), wi & u32(0xFFFF0000)
                if j == 0:
                    sc = jnp.where(lane == 0, 1.0 / (S * D), 2.0 / (S * D))
                else:
                    sc = (1.0 if j == 4 else 2.0) / (S * D)
                wr = pltpu.bitcast(wr, f32) * sc
                wi = pltpu.bitcast(wi, f32) * sc
                xr, xi = zb[f1, :R2, cols], zb[f1, R2:, cols]
                y = jnp.concatenate([xr * wr - xi * wi, xr * wi + xi * wr], axis=0).astype(bf16)
                zb[f1, :, cols] = _dot(mbt, y)
        return 0

    lax.fori_loop(0, R1 // 2, idft, 0)

    def inv(g, _):
        r0 = pl.multiple_of(g * G, G)
        lane0 = lax.broadcasted_iota(jnp.int32, (R1 * G, 128), 1) == 0

        def tile(j):
            ys = []
            for h in range(G // 8):
                ys += _fft([(zb[f1, pl.ds(r0 + h * 8, 8), j * 128:(j + 1) * 128],
                             zb[f1, pl.ds(R2 + r0 + h * 8, 8), j * 128:(j + 1) * 128]) for f1 in range(R1)], +1)
            return (jnp.concatenate([y[0] for y in ys], axis=0),
                    jnp.concatenate([y[1] for y in ys], axis=0))

        nyq = tile(4)[0]
        gs = []
        for j in range(4):
            yr, yi = tile(j)
            if j == 0:
                yi = jnp.where(lane0, nyq, yi)
            p = _dot_nt(jnp.concatenate([yr, yi], axis=1).astype(bf16), fd[j])
            gs.append((p[:, :128], p[:, 128:]))
        y = jnp.concatenate(_rfft8_adjoint(gs), axis=1)
        for t1 in range(R1):
            xb[g, t1] = jnp.concatenate(
                [y[(h * R1 + t1) * 8:(h * R1 + t1 + 1) * 8] for h in range(G // 8)], axis=0).astype(bf16)
        return 0

    lax.fori_loop(0, R2 // G, inv, 0)


def _attention_phase(xa, mem_ref, wqkv, pre, wo, outa, before_steps, store_rows):
    row = lax.broadcasted_iota(jnp.int32, (L, L), 0)
    col = lax.broadcasted_iota(jnp.int32, (L, L), 1)

    def step(s, mem, ahead):
        mask = (row < M) | (row >= col)
        rows = pl.ds(pl.multiple_of(s * SEG, SEG), SEG)
        h = jnp.concatenate([mem, xa[rows, :].astype(f32)], axis=0)
        if ahead:
            h = h[:L - 8]
        st = {}

        def project(hd, lo, hi):
            w = jnp.concatenate([wqkv[hd, j, lo // 2:hi // 2, :] for j in range(3)], axis=1)
            return _dot(h[:, lo:hi], pltpu.bitcast(w, bf16))

        for hd in range(2):
            st['early', hd] = project(hd, 0, D // 2)

        def do_qkv(hd):
            qkv = st['early', hd] + project(hd, D // 2, D) if ('early', hd) in st else project(hd, 0, D)
            if ahead:
                r8 = pl.ds(pl.multiple_of(s * 8, 8), 8)
                qkv = jnp.concatenate(
                    [qkv, jnp.concatenate([pre[hd, j, r8, :] for j in range(3)], axis=1)], axis=0)
            st['q', hd] = qkv[:, :128] * (DH ** -0.5)
            st['k', hd] = qkv[:, 128:256].astype(bf16)
            st['v', hd] = qkv[:, 256:].astype(bf16)

        def do_qk(hd):
            sc = jnp.where(mask, _dot_nt(st['q', hd], st['k', hd]), -1e9)
            e = jnp.exp(sc - jnp.max(sc, axis=1, keepdims=True))
            st['e', hd] = e
            den = jnp.sum(e, axis=1, keepdims=True)
            r = pl.reciprocal(den, approx=True)
            st['r', hd] = r * (2.0 - den * r)

        def do_pv(hd):
            st['o', hd] = _dot(st['e', hd], st['v', hd]) * st['r', hd]

        def do_wo(g, ng=4):
            o = jnp.concatenate([st['o', hd] for hd in range(g * ng, (g + 1) * ng)], axis=1)
            for n in range(8):
                r = _dot(o, pltpu.bitcast(wo[g * ng * 64:(g + 1) * ng * 64, n * 128:(n + 1) * 128], bf16))
                st['out', n] = st['out', n] + r if ('out', n) in st else r

        for t in range(H):
            do_qkv(t)
            if t >= 1: do_qk(t - 1)
            if t >= 3: do_pv(t - 3)
        do_wo(0); do_pv(H - 3)
        do_wo(1); do_qk(H - 1); do_pv(H - 2)
        do_wo(2)
        do_wo(3); do_pv(H - 1)
        do_wo(4); do_wo(5); do_wo(3, 8)
        out = jnp.concatenate([st['out', n] for n in range(8)], axis=1)
        outa[rows, :] = out[M:].astype(bf16)
        return out[:M].astype(bf16).astype(f32)

    def steps(ahead, i, mem):
        if ahead:
            before_steps(i)
        for u in range(UNROLL):
            mem = step(i * UNROLL + u, mem, ahead)
        store_rows(i)
        return mem

    mem = lax.fori_loop(0, PRE // UNROLL, functools.partial(steps, True), mem_ref[...].astype(f32))
    lax.fori_loop(PRE // UNROLL, NSEG // UNROLL, functools.partial(steps, False), mem)


def _kernel(xa_hbm, xa3_hbm, mem_hbm, wq_hbm, wk_hbm, wv_hbm, wo_hbm, xb_hbm, wr_hbm, wi_hbm, fd_hbm, fs_hbm,
            out_hbm, mem_ref, raw, wqkv, xq, xpre, pre, wo, xa, ya, xb, fd, fs, wraw, wnyq, wst, zb,
            sems, xsem, fsem, wsem, osem):
    def copy(src, dst, i, priority=0):
        c = pltpu.make_async_copy(src, dst, sems.at[i])
        c.start(priority=priority)
        return c

    def xb_copy(g):
        return pltpu.make_async_copy(xb_hbm.at[:, pl.ds(pl.multiple_of(g * G, G), G), :], xb.at[g], xsem.at[g])

    def yb_copy(g):
        return pltpu.make_async_copy(
            xb.at[g], out_hbm.at[:, pl.ds(pl.multiple_of(g * G, G), G), pl.ds(D, D)], osem.at[1])

    def w_copy(j, hg):
        src = (wq_hbm, wk_hbm, wv_hbm)[j].bitcast(u32).at[:, pl.ds(hg * (HG // 2), HG // 2), :]
        c = j * (H // HG) + hg
        return pltpu.make_async_copy(src, raw.at[c].reshape(D, HG // 2, DH), wsem.at[c])

    small = [copy(fd_hbm, fd, 0), copy(fs_hbm, fs, 4), copy(mem_hbm, mem_ref, 5)]
    small += [copy(w.at[pl.ds(D // 2, 1), :], wnyq.at[c], 1 + c) for c, w in enumerate((wr_hbm, wi_hbm))]
    xb_copy(0).start()
    for c in small:
        c.wait()
    for g in range(1, R2 // G):
        xb_copy(g).start()

    def filter_copies(g):
        return [pltpu.make_async_copy(
            w.at[pl.ds(0, D // 2), pl.ds(pl.multiple_of(t * 128, 128), 128)], wraw.at[c * R1 + t], fsem.at[g])
            for t in (2 * g, 2 * g + 1) for c, w in enumerate((wr_hbm, wi_hbm))]

    def wait_rows(g):
        xb_copy(g).wait()

        @pl.when(g == 2)
        def _():
            for i in range(R1 // 2):
                for cp in filter_copies(i):
                    cp.start()
            x_ahead().start()

    def x_first():
        rows = pl.ds(0, XA0 * SEG)
        return pltpu.make_async_copy(xa_hbm.at[rows, :], xa.at[rows, :], sems.at[6])

    def x_ahead():
        return pltpu.make_async_copy(xa3_hbm.at[pl.ds(0, PRE), pl.ds(SEG - 8, 8), :], xq, sems.at[9])

    def wo_copy():
        return pltpu.make_async_copy(wo_hbm.bitcast(u32), wo, sems.at[7])

    def prepare_filter(g):
        for cp in filter_copies(g):
            cp.wait()

        @pl.when(g == R1 // 2 - 2)
        def _():
            for j in range(3):
                for hg in range(H // HG):
                    w_copy(j, hg).start()
            wo_copy().start()
            x_first().start()

        pairs = wraw.bitcast(u32)
        for t in (2 * g, 2 * g + 1):
            dst = pl.ds(pl.multiple_of(t * 64, 64), 64)
            for j in range(NT):
                for c in range(2):
                    if j < 4:
                        res = []
                        for k1 in _k1_pair(j):
                            w = pairs[c * R1 + t, pl.ds(k1 // 2, 64, stride=4), :]
                            res.append(pltpu.bitcast(w & u32(0xFFFF0000) if k1 % 2 else w << 16, f32))
                        tile = jnp.concatenate(res, axis=0)
                    else:
                        last = wnyq[c, :, pl.ds(pl.multiple_of(t * 128, 128), 128)].astype(f32)
                        tile = jnp.broadcast_to(last, (128, 128))
                    wst[c, j, dst, :] = pltpu.bitcast(tile.T.astype(bf16), u32)
                yield

    _spectral_phase(xb, fd, fs, wst, zb, wait_rows, prepare_filter)

    x_ahead().wait()
    for s in range(PRE):
        xpre[s * 8:(s + 1) * 8, :] = xq[s].astype(f32)

    def relayout(c, _):
        pltpu.make_async_copy(raw.at[c], raw.at[c], wsem.at[c]).wait()
        j, h0 = c // (H // HG), (c % (H // HG)) * HG
        for i in range(HG // 2):
            w = raw[c, pl.ds(i, D, stride=HG // 2), :]
            for hd, bits in ((2 * i, w << 16), (2 * i + 1, w & u32(0xFFFF0000))):
                panel = pltpu.bitcast(bits, f32).astype(bf16)
                wqkv[h0 + hd, j] = pltpu.bitcast(panel, u32)
                pre[h0 + hd, j] = _dot(xpre[...], panel)
        return 0

    lax.fori_loop(0, 3 * H // HG, relayout, 0)
    wo_copy().wait()
    x_first().wait()
    rest = pl.ds(XA0 * SEG, S - XA0 * SEG)
    c_rest = copy(xa_hbm.at[rest, :], xa.at[rest, :], 8)
    for g in range(R2 // G):
        yb_copy(g).start()

    def before_steps(i):
        @pl.when(i == XA0 // UNROLL)
        def _():
            c_rest.wait()

    def out_copy(i):
        n = UNROLL * SEG
        dst = out_hbm.at[i // (R2 // n), pl.ds(pl.multiple_of((i % (R2 // n)) * n, n), n), pl.ds(0, D)]
        return pltpu.make_async_copy(ya.at[pl.ds(pl.multiple_of(i * n, n), n), :], dst, osem.at[0])

    _attention_phase(xa, mem_ref, wqkv, pre, wo, ya, before_steps, lambda i: out_copy(i).start())

    def drain(i, _):
        out_copy(i).wait()
        return 0

    lax.fori_loop(0, NSEG // UNROLL, drain, 0)
    for g in range(R2 // G):
        yb_copy(g).wait()


@jax.jit
def pallas_concat_heads__memory_aug_recurrent_mem_tr__spectral_gfnet__prompt_kernel(
    A_x, A_mem0, A_Wq, A_Wk, A_Wv, A_Wo, A_seg_len, B_x, B_w_r, B_w_i,
):
    del A_seg_len
    hbm = pl.BlockSpec(memory_space=pl.ANY)
    out = pl.pallas_call(
        _kernel,
        out_shape=jax.ShapeDtypeStruct((R1, R2, 2 * D), bf16),
        in_specs=[hbm] * 12,
        out_specs=hbm,
        scratch_shapes=[
            pltpu.VMEM((M, D), bf16),
            pltpu.VMEM((3 * H // HG, D * HG // 2, DH), u32),
            pltpu.VMEM((H, 3, D // 2, DH), u32),
            pltpu.VMEM((PRE, 8, D), bf16),
            pltpu.VMEM((PRE * 8, D), f32),
            pltpu.VMEM((H, 3, PRE * 8, DH), f32),
            pltpu.VMEM((H * DH // 2, D), u32),
            pltpu.VMEM((S, D), bf16),
            pltpu.VMEM((S, D), bf16),
            pltpu.VMEM((R2 // G, R1, G, D), bf16),
            pltpu.VMEM((4, 256, 256), bf16),
            pltpu.VMEM((2, R2 + R1, R2), f32),
            pltpu.VMEM((2 * R1, D // 2, 128), bf16),
            pltpu.VMEM((2, 1, S), bf16),
            pltpu.VMEM((2, NT, S // 2, 128), u32),
            pltpu.VMEM((R1, 2 * R2, NT * 128), f32),
            pltpu.SemaphoreType.DMA((10,)),
            pltpu.SemaphoreType.DMA((R2 // G,)),
            pltpu.SemaphoreType.DMA((R1 // 2,)),
            pltpu.SemaphoreType.DMA((3 * H // HG,)),
            pltpu.SemaphoreType.DMA((2,)),
        ],
        compiler_params=pltpu.CompilerParams(vmem_limit_bytes=120 * 2 ** 20),
    )(
        A_x.reshape(S, D), A_x.reshape(NSEG, SEG, D), A_mem0.reshape(M, D),
        A_Wq, A_Wk, A_Wv,
        A_Wo.reshape(H * DH, D),
        B_x.reshape(R1, R2, D), B_w_r.T, B_w_i.T,
        jnp.asarray(_FD, dtype=bf16), jnp.asarray(_FS),
    )
    return out.reshape(1, S, 2 * D)
```

```python
import functools

import numpy as np
import jax
import jax.numpy as jnp
from jax import lax
import jax.experimental.pallas as pl
import jax.experimental.pallas.tpu as pltpu

S, D, H, DH, M, SEG = 2048, 1024, 32, 128, 8, 32
L = M + SEG
NSEG = S // SEG
DF = D // 2 + 1
R1, R2 = 16, 128
G = 16
HG = 16
UNROLL = 2
PRE = 30
XA0 = 4
NT = 5
f32, bf16, u32 = jnp.float32, jnp.bfloat16, jnp.uint32


def _k1_pair(j):
    return j, (4 if j == 0 else 8 - j)


def _dft_constants():
    b = np.arange(128)[:, None]
    c = np.arange(64)[None, :]
    fd = np.zeros((4, 256, 256))
    for j in range(4):
        for half, k1 in enumerate(_k1_pair(j)):
            ang = 2.0 * np.pi * ((b * (k1 + 8 * c)) % D) / D
            co, si = np.cos(ang), np.sin(ang)
            re = slice(64 * half, 64 * half + 64)
            im = slice(128 + 64 * half, 128 + 64 * half + 64)
            if j == 0:
                rows = slice(128 * half, 128 * half + 128)
                fd[j, rows, re], fd[j, rows, im] = co, -si
            else:
                sg = 1.0 - 2.0 * half
                fd[j, :128, re], fd[j, :128, im] = co, -si
                fd[j, 128:, re], fd[j, 128:, im] = sg * si, sg * co
    fd[0, :128, 128] = 1.0 - 2.0 * (np.arange(128) % 2)
    n = np.arange(R2)
    a = -2.0 * np.pi * np.concatenate([(n[:, None] * n[None, :]) % R2 / R2,
                                       np.arange(R1)[:, None] * n[None, :] / S], axis=0)
    return fd.astype(np.float32), np.stack([np.cos(a), np.sin(a)]).astype(np.float32)


_FD, _FS = _dft_constants()
_RH = float(np.sqrt(0.5))


def _dot(a, b):
    return lax.dot_general(a, b, (((1,), (0,)), ((), ())), preferred_element_type=f32)


def _dot_nt(a, b):
    return lax.dot_general(a, b, (((1,), (1,)), ((), ())), preferred_element_type=f32)


def _dot_tn(a, b):
    return lax.dot_general(a, b, (((0,), (0,)), ((), ())), preferred_element_type=f32)


def _cmul_const(x, e, n, sign):
    xr, xi = x
    e = e % n
    if e == 0:
        return x
    if 4 * e == n:
        return (_neg(xi), xr) if sign > 0 else (xi, _neg(xr))
    c = float(np.cos(2.0 * np.pi * e / n))
    s = float(sign * np.sin(2.0 * np.pi * e / n))
    if xi is None:
        return xr * c, xr * s
    if 8 * e == n or 8 * e == 3 * n:
        if c * s > 0:
            return (xr - xi) * c, (xr + xi) * c
        return (xr + xi) * c, (xi - xr) * c
    return xr * c - xi * s, xr * s + xi * c


def _neg(a):
    return None if a is None else -a


def _add(a, b):
    return b if a is None else a if b is None else a + b


def _sub(a, b):
    return _neg(b) if a is None else a if b is None else a - b


def _fft(xs, sign):
    n = len(xs)
    if n == 1:
        return xs
    ev, od = _fft(xs[0::2], sign), _fft(xs[1::2], sign)
    out = [None] * n
    for j in range(n // 2):
        e = ev[j]
        if 4 * j == n:
            orr, oi = od[j]
            if sign > 0:
                out[j] = (_sub(e[0], oi), _add(e[1], orr))
                out[j + n // 2] = (_add(e[0], oi), _sub(e[1], orr))
            else:
                out[j] = (_add(e[0], oi), _sub(e[1], orr))
                out[j + n // 2] = (_sub(e[0], oi), _add(e[1], orr))
            continue
        t = _cmul_const(od[j], j, n, sign)
        out[j] = (_add(e[0], t[0]), _add(e[1], t[1]))
        out[j + n // 2] = (_sub(e[0], t[0]), _sub(e[1], t[1]))
    return out


def _rfft8(x):
    s04, d04, s26, d26 = x[0] + x[4], x[0] - x[4], x[2] + x[6], x[2] - x[6]
    s15, d15, s37, d37 = x[1] + x[5], x[1] - x[5], x[3] + x[7], x[3] - x[7]
    e, o = s04 + s26, s15 + s37
    p, q = (d15 - d37) * _RH, (d15 + d37) * _RH
    return [(e + o, e - o), (d04 + p, -(d26 + q)), (s04 - s26, s37 - s15), (d04 - p, d26 - q)]


def _rfft8_adjoint(g):
    (g0, g4), (r1, i1), (r2, i2), (r3, i3) = g
    e, o = g0 + g4, g0 - g4
    s04, s26, s15, s37 = e + r2, e - r2, o - i2, o + i2
    d04, d26 = r1 + r3, i3 - i1
    p, q = (r1 - r3) * _RH, (i1 + i3) * _RH
    d15, d37 = p - q, -(p + q)
    return [s04 + d04, s15 + d15, s26 + d26, s37 + d37, s04 - d04, s15 - d15, s26 - d26, s37 - d37]


def _spectral_phase(xb, fd, fs, wst, zb, yb, wait_rows, prepare_filter):
    groups = [(h, t1) for h in range(G // 8) for t1 in range(R1)]

    def fwd(g, _):
        wait_rows(g)
        r0 = pl.multiple_of(g * G, G)
        lane0 = lax.broadcasted_iota(jnp.int32, (R1 * G, 128), 1) == 0
        xg = [xb[g, t1].astype(f32) for t1 in range(R1)]
        xg = jnp.concatenate([xg[t1][h * 8:(h + 1) * 8] for h, t1 in groups], axis=0)
        us = _rfft8([xg[:, a * 128:(a + 1) * 128] for a in range(8)])
        us = [jnp.concatenate(u, axis=1).astype(bf16) for u in us]
        nyq = None
        for j in range(NT):
            if j < 4:
                z = _dot(us[j], fd[j])
                zr, zi = z[:, :128], z[:, 128:]
                if j == 0:
                    nyq = jnp.where(lane0, zi, 0.0)
                    zi = jnp.where(lane0, 0.0, zi)
                xs = [(zr[n * 8:(n + 1) * 8], zi[n * 8:(n + 1) * 8]) for n in range(len(groups))]
            else:
                xs = [(nyq[n * 8:(n + 1) * 8], None) for n in range(len(groups))]
            for h in range(G // 8):
                for f1, (yr, yi) in enumerate(_fft(xs[h * R1:(h + 1) * R1], -1)):
                    zb[f1, pl.ds(r0 + h * 8, 8), j * 128:(j + 1) * 128] = yr
                    zb[f1, pl.ds(R2 + r0 + h * 8, 8), j * 128:(j + 1) * 128] = (
                        jnp.zeros_like(yr) if yi is None else yi)
        return 0

    lax.fori_loop(0, R2 // G, fwd, 0)

    def dft_block(f1):
        cr, ci = fs[0, :R2, :], fs[1, :R2, :]
        tr, ti = fs[0, pl.ds(R2 + f1, 1), :], fs[1, pl.ds(R2 + f1, 1), :]
        mr, mi = cr * tr - ci * ti, cr * ti + ci * tr
        return jnp.concatenate([jnp.concatenate([mr, -mi], axis=1),
                                jnp.concatenate([mi, mr], axis=1)], axis=0).astype(bf16)

    def dft(g, _):
        side = prepare_filter(g)
        for f1 in (2 * g, 2 * g + 1):
            mb = dft_block(f1)
            for j in range(NT):
                cols = slice(j * 128, (j + 1) * 128)
                next(side)
                yb[f1, :, cols] = _dot(mb, zb[f1, :, cols].astype(bf16))
        return 0

    lax.fori_loop(0, R1 // 2, dft, 0)

    def idft(g, _):
        lane = lax.broadcasted_iota(jnp.int32, (1, 128), 1)
        for half in range(2):
            f1 = g + half * (R1 // 2)
            mbt = dft_block(f1).T
            for j in range(NT):
                cols = slice(j * 128, (j + 1) * 128)
                wr = wst[0, j, pl.ds(g, R2, stride=R1 // 2), :]
                wi = wst[1, j, pl.ds(g, R2, stride=R1 // 2), :]
                if half == 0:
                    wr, wi = wr << 16, wi << 16
                else:
                    wr, wi = wr & u32(0xFFFF0000), wi & u32(0xFFFF0000)
                if j == 0:
                    sc = jnp.where(lane == 0, 1.0 / (S * D), 2.0 / (S * D))
                else:
                    sc = (1.0 if j == 4 else 2.0) / (S * D)
                wr = pltpu.bitcast(wr, f32) * sc
                wi = pltpu.bitcast(wi, f32) * sc
                xr, xi = yb[f1, :R2, cols], yb[f1, R2:, cols]
                y = jnp.concatenate([xr * wr - xi * wi, xr * wi + xi * wr], axis=0).astype(bf16)
                zb[f1, :, cols] = _dot(mbt, y)
        return 0

    lax.fori_loop(0, R1 // 2, idft, 0)

    def inv(g, _):
        r0 = pl.multiple_of(g * G, G)
        lane0 = lax.broadcasted_iota(jnp.int32, (R1 * G, 128), 1) == 0

        def tile(j):
            ys = []
            for h in range(G // 8):
                ys += _fft([(zb[f1, pl.ds(r0 + h * 8, 8), j * 128:(j + 1) * 128],
                             zb[f1, pl.ds(R2 + r0 + h * 8, 8), j * 128:(j + 1) * 128]) for f1 in range(R1)], +1)
            return (jnp.concatenate([y[0] for y in ys], axis=0),
                    jnp.concatenate([y[1] for y in ys], axis=0))

        nyq = tile(4)[0]
        gs = []
        for j in range(4):
            yr, yi = tile(j)
            if j == 0:
                yi = jnp.where(lane0, nyq, yi)
            p = _dot_nt(jnp.concatenate([yr, yi], axis=1).astype(bf16), fd[j])
            gs.append((p[:, :128], p[:, 128:]))
        y = jnp.concatenate(_rfft8_adjoint(gs), axis=1)
        for t1 in range(R1):
            xb[g, t1] = jnp.concatenate(
                [y[(h * R1 + t1) * 8:(h * R1 + t1 + 1) * 8] for h in range(G // 8)], axis=0).astype(bf16)
        return 0

    lax.fori_loop(0, R2 // G, inv, 0)


def _attention_phase(xa, mem_ref, wqkv, pre, wo, outa, before_steps, store_rows):
    row = lax.broadcasted_iota(jnp.int32, (L, L), 0)
    col = lax.broadcasted_iota(jnp.int32, (L, L), 1)

    def step(s, mem, ahead):
        mask = (row < M) | (row >= col)
        rows = pl.ds(pl.multiple_of(s * SEG, SEG), SEG)
        h = jnp.concatenate([mem, xa[rows, :].astype(f32)], axis=0)
        if ahead:
            h = h[:L - 8]
        st = {}

        def project(hd, lo, hi):
            w = jnp.concatenate([wqkv[hd, j, lo // 2:hi // 2, :] for j in range(3)], axis=1)
            return _dot(h[:, lo:hi], pltpu.bitcast(w, bf16))

        for hd in range(2):
            st['early', hd] = project(hd, 0, D // 2)

        def do_qkv(hd):
            qkv = st['early', hd] + project(hd, D // 2, D) if ('early', hd) in st else project(hd, 0, D)
            if ahead:
                r8 = pl.ds(pl.multiple_of(s * 8, 8), 8)
                qkv = jnp.concatenate(
                    [qkv, jnp.concatenate([pre[hd, j, r8, :] for j in range(3)], axis=1)], axis=0)
            st['q', hd] = qkv[:, :128] * (DH ** -0.5)
            st['k', hd] = qkv[:, 128:256].astype(bf16)
            st['v', hd] = qkv[:, 256:].astype(bf16)

        def do_qk(hd):
            sc = jnp.where(mask, _dot_nt(st['q', hd], st['k', hd]), -1e9)
            e = jnp.exp(sc - jnp.max(sc, axis=1, keepdims=True))
            st['e', hd] = e
            den = jnp.sum(e, axis=1, keepdims=True)
            r = pl.reciprocal(den, approx=True)
            st['r', hd] = r * (2.0 - den * r)

        def do_pv(hd):
            st['o', hd] = _dot(st['e', hd], st['v', hd]) * st['r', hd]

        def do_wo(g, ng=4):
            o = jnp.concatenate([st['o', hd] for hd in range(g * ng, (g + 1) * ng)], axis=1)
            for n in range(8):
                r = _dot(o, pltpu.bitcast(wo[g * ng * 64:(g + 1) * ng * 64, n * 128:(n + 1) * 128], bf16))
                st['out', n] = st['out', n] + r if ('out', n) in st else r

        for t in range(H):
            do_qkv(t)
            if t >= 1: do_qk(t - 1)
            if t >= 3: do_pv(t - 3)
        do_wo(0); do_pv(H - 3)
        do_wo(1); do_qk(H - 1); do_pv(H - 2)
        do_wo(2)
        do_wo(3); do_pv(H - 1)
        do_wo(4); do_wo(5); do_wo(3, 8)
        out = jnp.concatenate([st['out', n] for n in range(8)], axis=1)
        outa[rows, :] = out[M:].astype(bf16)
        return out[:M].astype(bf16).astype(f32)

    def steps(ahead, i, mem):
        if ahead:
            before_steps(i)
        for u in range(UNROLL):
            mem = step(i * UNROLL + u, mem, ahead)
        store_rows(i)
        return mem

    mem = lax.fori_loop(0, PRE // UNROLL, functools.partial(steps, True), mem_ref[...].astype(f32))
    lax.fori_loop(PRE // UNROLL, NSEG // UNROLL, functools.partial(steps, False), mem)


def _kernel(xa_hbm, xa3_hbm, mem_hbm, wq_hbm, wk_hbm, wv_hbm, wo_hbm, xb_hbm, wr_hbm, wi_hbm, fd_hbm, fs_hbm,
            out_hbm, mem_ref, raw, wqkv, xq, xpre, pre, wo, xa, ya, xb, fd, fs, wraw, wnyq, wst, zb, yb,
            sems, xsem, fsem, wsem, osem):
    def copy(src, dst, i, priority=0):
        c = pltpu.make_async_copy(src, dst, sems.at[i])
        c.start(priority=priority)
        return c

    def xb_copy(g):
        return pltpu.make_async_copy(xb_hbm.at[:, pl.ds(pl.multiple_of(g * G, G), G), :], xb.at[g], xsem.at[g])

    def yb_copy(g):
        return pltpu.make_async_copy(
            xb.at[g], out_hbm.at[:, pl.ds(pl.multiple_of(g * G, G), G), pl.ds(D, D)], osem.at[1])

    def w_copy(j, hg):
        src = (wq_hbm, wk_hbm, wv_hbm)[j].bitcast(u32).at[:, pl.ds(hg * (HG // 2), HG // 2), :]
        c = j * (H // HG) + hg
        return pltpu.make_async_copy(src, raw.at[c].reshape(D, HG // 2, DH), wsem.at[c])

    small = [copy(fd_hbm, fd, 0), copy(fs_hbm, fs, 4), copy(mem_hbm, mem_ref, 5)]
    small += [copy(w.at[pl.ds(D // 2, 1), :], wnyq.at[c], 1 + c) for c, w in enumerate((wr_hbm, wi_hbm))]
    xb_copy(0).start()
    for c in small:
        c.wait()
    for g in range(1, R2 // G):
        xb_copy(g).start()

    def filter_copies(g):
        return [pltpu.make_async_copy(
            w.at[pl.ds(0, D // 2), pl.ds(pl.multiple_of(t * 128, 128), 128)], wraw.at[c * R1 + t], fsem.at[g])
            for t in (2 * g, 2 * g + 1) for c, w in enumerate((wr_hbm, wi_hbm))]

    def wait_rows(g):
        xb_copy(g).wait()

        @pl.when(g == 2)
        def _():
            for i in range(R1 // 2):
                for cp in filter_copies(i):
                    cp.start()
            x_ahead().start()

    def x_first():
        rows = pl.ds(0, XA0 * SEG)
        return pltpu.make_async_copy(xa_hbm.at[rows, :], xa.at[rows, :], sems.at[6])

    def x_ahead():
        return pltpu.make_async_copy(xa3_hbm.at[pl.ds(0, PRE), pl.ds(SEG - 8, 8), :], xq, sems.at[9])

    def wo_copy():
        return pltpu.make_async_copy(wo_hbm.bitcast(u32), wo, sems.at[7])

    def prepare_filter(g):
        for cp in filter_copies(g):
            cp.wait()

        @pl.when(g == R1 // 2 - 2)
        def _():
            for j in range(3):
                for hg in range(H // HG):
                    w_copy(j, hg).start()
            wo_copy().start()
            x_first().start()

        pairs = wraw.bitcast(u32)
        for t in (2 * g, 2 * g + 1):
            dst = pl.ds(pl.multiple_of(t * 64, 64), 64)
            for j in range(NT):
                for c in range(2):
                    if j < 4:
                        res = []
                        for k1 in _k1_pair(j):
                            w = pairs[c * R1 + t, pl.ds(k1 // 2, 64, stride=4), :]
                            res.append(pltpu.bitcast(w & u32(0xFFFF0000) if k1 % 2 else w << 16, f32))
                        tile = jnp.concatenate(res, axis=0)
                    else:
                        last = wnyq[c, :, pl.ds(pl.multiple_of(t * 128, 128), 128)].astype(f32)
                        tile = jnp.broadcast_to(last, (128, 128))
                    tile = pltpu.bitcast(tile.T, u32)
                    wst[c, j, dst, :] = jnp.concatenate(
                        [(tile[r:r + 8] >> 16) | tile[r + 8:r + 16] for r in range(0, 128, 16)], axis=0)
                yield

    _spectral_phase(xb, fd, fs, wst, zb, yb, wait_rows, prepare_filter)

    x_ahead().wait()
    for s in range(PRE):
        xpre[s * 8:(s + 1) * 8, :] = xq[s].astype(f32)

    def relayout(c, _):
        pltpu.make_async_copy(raw.at[c], raw.at[c], wsem.at[c]).wait()
        j, h0 = c // (H // HG), (c % (H // HG)) * HG
        for i in range(HG // 2):
            w = raw[c, pl.ds(i, D, stride=HG // 2), :]
            for hd, bits in ((2 * i, w << 16), (2 * i + 1, w & u32(0xFFFF0000))):
                panel = pltpu.bitcast(bits, f32).astype(bf16)
                wqkv[h0 + hd, j] = pltpu.bitcast(panel, u32)
                pre[h0 + hd, j] = _dot(xpre[...], panel)
        return 0

    lax.fori_loop(0, 3 * H // HG, relayout, 0)
    wo_copy().wait()
    x_first().wait()
    rest = pl.ds(XA0 * SEG, S - XA0 * SEG)
    c_rest = copy(xa_hbm.at[rest, :], xa.at[rest, :], 8)
    for g in range(R2 // G):
        yb_copy(g).start()

    def before_steps(i):
        @pl.when(i == XA0 // UNROLL)
        def _():
            c_rest.wait()

    def out_copy(i):
        n = UNROLL * SEG
        dst = out_hbm.at[i // (R2 // n), pl.ds(pl.multiple_of((i % (R2 // n)) * n, n), n), pl.ds(0, D)]
        return pltpu.make_async_copy(ya.at[pl.ds(pl.multiple_of(i * n, n), n), :], dst, osem.at[0])

    _attention_phase(xa, mem_ref, wqkv, pre, wo, ya, before_steps, lambda i: out_copy(i).start())

    def drain(i, _):
        out_copy(i).wait()
        return 0

    lax.fori_loop(0, NSEG // UNROLL, drain, 0)
    for g in range(R2 // G):
        yb_copy(g).wait()


@jax.jit
def pallas_concat_heads__memory_aug_recurrent_mem_tr__spectral_gfnet__prompt_kernel(
    A_x, A_mem0, A_Wq, A_Wk, A_Wv, A_Wo, A_seg_len, B_x, B_w_r, B_w_i,
):
    del A_seg_len
    hbm = pl.BlockSpec(memory_space=pl.ANY)
    out = pl.pallas_call(
        _kernel,
        out_shape=jax.ShapeDtypeStruct((R1, R2, 2 * D), bf16),
        in_specs=[hbm] * 12,
        out_specs=hbm,
        scratch_shapes=[
            pltpu.VMEM((M, D), bf16),
            pltpu.VMEM((3 * H // HG, D * HG // 2, DH), u32),
            pltpu.VMEM((H, 3, D // 2, DH), u32),
            pltpu.VMEM((PRE, 8, D), bf16),
            pltpu.VMEM((PRE * 8, D), f32),
            pltpu.VMEM((H, 3, PRE * 8, DH), f32),
            pltpu.VMEM((H * DH // 2, D), u32),
            pltpu.VMEM((S, D), bf16),
            pltpu.VMEM((S, D), bf16),
            pltpu.VMEM((R2 // G, R1, G, D), bf16),
            pltpu.VMEM((4, 256, 256), bf16),
            pltpu.VMEM((2, R2 + R1, R2), f32),
            pltpu.VMEM((2 * R1, D // 2, 128), bf16),
            pltpu.VMEM((2, 1, S), bf16),
            pltpu.VMEM((2, NT, S // 2, 128), u32),
            pltpu.VMEM((R1, 2 * R2, NT * 128), f32),
            pltpu.VMEM((R1, 2 * R2, NT * 128), f32),
            pltpu.SemaphoreType.DMA((10,)),
            pltpu.SemaphoreType.DMA((R2 // G,)),
            pltpu.SemaphoreType.DMA((R1 // 2,)),
            pltpu.SemaphoreType.DMA((3 * H // HG,)),
            pltpu.SemaphoreType.DMA((2,)),
        ],
        compiler_params=pltpu.CompilerParams(vmem_limit_bytes=120 * 2 ** 20),
    )(
        A_x.reshape(S, D), A_x.reshape(NSEG, SEG, D), A_mem0.reshape(M, D),
        A_Wq, A_Wk, A_Wv,
        A_Wo.reshape(H * DH, D),
        B_x.reshape(R1, R2, D), B_w_r.T, B_w_i.T,
        jnp.asarray(_FD, dtype=bf16), jnp.asarray(_FS),
    )
    return out.reshape(1, S, 2 * D)
```

```python
import functools

import numpy as np
import jax
import jax.numpy as jnp
from jax import lax
import jax.experimental.pallas as pl
import jax.experimental.pallas.tpu as pltpu

S, D, H, DH, M, SEG = 2048, 1024, 32, 128, 8, 32
L = M + SEG
NSEG = S // SEG
DF = D // 2 + 1
R1, R2 = 16, 128
G = 16
HG = 16
UNROLL = 2
PRE = 26
XA0 = 4
NT = 5
f32, bf16, u32 = jnp.float32, jnp.bfloat16, jnp.uint32


def _k1_pair(j):
    return j, (4 if j == 0 else 8 - j)


def _dft_constants():
    b = np.arange(128)[:, None]
    c = np.arange(64)[None, :]
    fd = np.zeros((4, 256, 256))
    for j in range(4):
        for half, k1 in enumerate(_k1_pair(j)):
            ang = 2.0 * np.pi * ((b * (k1 + 8 * c)) % D) / D
            co, si = np.cos(ang), np.sin(ang)
            re = slice(64 * half, 64 * half + 64)
            im = slice(128 + 64 * half, 128 + 64 * half + 64)
            if j == 0:
                rows = slice(128 * half, 128 * half + 128)
                fd[j, rows, re], fd[j, rows, im] = co, -si
            else:
                sg = 1.0 - 2.0 * half
                fd[j, :128, re], fd[j, :128, im] = co, -si
                fd[j, 128:, re], fd[j, 128:, im] = sg * si, sg * co
    fd[0, :128, 128] = 1.0 - 2.0 * (np.arange(128) % 2)
    n = np.arange(R2)
    a = -2.0 * np.pi * np.concatenate([(n[:, None] * n[None, :]) % R2 / R2,
                                       np.arange(R1)[:, None] * n[None, :] / S], axis=0)
    return fd.astype(np.float32), np.stack([np.cos(a), np.sin(a)]).astype(np.float32)


_FD, _FS = _dft_constants()
_RH = float(np.sqrt(0.5))


def _dot(a, b):
    return lax.dot_general(a, b, (((1,), (0,)), ((), ())), preferred_element_type=f32)


def _dot_nt(a, b):
    return lax.dot_general(a, b, (((1,), (1,)), ((), ())), preferred_element_type=f32)


def _dot_tn(a, b):
    return lax.dot_general(a, b, (((0,), (0,)), ((), ())), preferred_element_type=f32)


def _cmul_const(x, e, n, sign):
    xr, xi = x
    e = e % n
    if e == 0:
        return x
    if 4 * e == n:
        return (_neg(xi), xr) if sign > 0 else (xi, _neg(xr))
    c = float(np.cos(2.0 * np.pi * e / n))
    s = float(sign * np.sin(2.0 * np.pi * e / n))
    if xi is None:
        return xr * c, xr * s
    if 8 * e == n or 8 * e == 3 * n:
        if c * s > 0:
            return (xr - xi) * c, (xr + xi) * c
        return (xr + xi) * c, (xi - xr) * c
    return xr * c - xi * s, xr * s + xi * c


def _neg(a):
    return None if a is None else -a


def _add(a, b):
    return b if a is None else a if b is None else a + b


def _sub(a, b):
    return _neg(b) if a is None else a if b is None else a - b


def _fft(xs, sign):
    n = len(xs)
    if n == 1:
        return xs
    ev, od = _fft(xs[0::2], sign), _fft(xs[1::2], sign)
    out = [None] * n
    for j in range(n // 2):
        e = ev[j]
        if 4 * j == n:
            orr, oi = od[j]
            if sign > 0:
                out[j] = (_sub(e[0], oi), _add(e[1], orr))
                out[j + n // 2] = (_add(e[0], oi), _sub(e[1], orr))
            else:
                out[j] = (_add(e[0], oi), _sub(e[1], orr))
                out[j + n // 2] = (_sub(e[0], oi), _add(e[1], orr))
            continue
        t = _cmul_const(od[j], j, n, sign)
        out[j] = (_add(e[0], t[0]), _add(e[1], t[1]))
        out[j + n // 2] = (_sub(e[0], t[0]), _sub(e[1], t[1]))
    return out


def _rfft8(x):
    s04, d04, s26, d26 = x[0] + x[4], x[0] - x[4], x[2] + x[6], x[2] - x[6]
    s15, d15, s37, d37 = x[1] + x[5], x[1] - x[5], x[3] + x[7], x[3] - x[7]
    e, o = s04 + s26, s15 + s37
    p, q = (d15 - d37) * _RH, (d15 + d37) * _RH
    return [(e + o, e - o), (d04 + p, -(d26 + q)), (s04 - s26, s37 - s15), (d04 - p, d26 - q)]


def _rfft8_adjoint(g):
    (g0, g4), (r1, i1), (r2, i2), (r3, i3) = g
    e, o = g0 + g4, g0 - g4
    s04, s26, s15, s37 = e + r2, e - r2, o - i2, o + i2
    d04, d26 = r1 + r3, i3 - i1
    p, q = (r1 - r3) * _RH, (i1 + i3) * _RH
    d15, d37 = p - q, -(p + q)
    return [s04 + d04, s15 + d15, s26 + d26, s37 + d37, s04 - d04, s15 - d15, s26 - d26, s37 - d37]


def _spectral_phase(xb, fd, fs, wst, zb, yb, wait_rows, prepare_filter):
    groups = [(h, t1) for h in range(G // 8) for t1 in range(R1)]

    def fwd(g, _):
        wait_rows(g)
        r0 = pl.multiple_of(g * G, G)
        lane0 = lax.broadcasted_iota(jnp.int32, (R1 * G, 128), 1) == 0
        xg = [xb[g, t1].astype(f32) for t1 in range(R1)]
        xg = jnp.concatenate([xg[t1][h * 8:(h + 1) * 8] for h, t1 in groups], axis=0)
        us = _rfft8([xg[:, a * 128:(a + 1) * 128] for a in range(8)])
        us = [jnp.concatenate(u, axis=1).astype(bf16) for u in us]
        nyq = None
        for j in range(NT):
            if j < 4:
                z = _dot(us[j], fd[j])
                zr, zi = z[:, :128], z[:, 128:]
                if j == 0:
                    nyq = jnp.where(lane0, zi, 0.0)
                    zi = jnp.where(lane0, 0.0, zi)
                xs = [(zr[n * 8:(n + 1) * 8], zi[n * 8:(n + 1) * 8]) for n in range(len(groups))]
            else:
                xs = [(nyq[n * 8:(n + 1) * 8], None) for n in range(len(groups))]
            for h in range(G // 8):
                for f1, (yr, yi) in enumerate(_fft(xs[h * R1:(h + 1) * R1], -1)):
                    zb[f1, pl.ds(r0 + h * 8, 8), j * 128:(j + 1) * 128] = yr
                    zb[f1, pl.ds(R2 + r0 + h * 8, 8), j * 128:(j + 1) * 128] = (
                        jnp.zeros_like(yr) if yi is None else yi)
        return 0

    lax.fori_loop(0, R2 // G, fwd, 0)

    def dft_block(f1, inverse):
        cr, ci = fs[0, :R2, :], fs[1, :R2, :]
        tr, ti = fs[0, pl.ds(R2 + f1, 1), :], fs[1, pl.ds(R2 + f1, 1), :]
        if inverse:
            tr, ti = tr * (2.0 / (S * D)), ti * (2.0 / (S * D))
        mr, mi = cr * tr - ci * ti, cr * ti + ci * tr
        if inverse:
            return [m.astype(bf16).T for m in (mr, -mi - mr, mr - mi)]
        return [m.astype(bf16) for m in (mr, mi - mr, mr + mi)]

    def cmatmul(m, xr, xi):
        k = _dot(m[0], (xr + xi).astype(bf16))
        return k - _dot(m[2], xi.astype(bf16)), k + _dot(m[1], xr.astype(bf16))

    def dft(g, _):
        side = prepare_filter(g)
        for f1 in (2 * g, 2 * g + 1):
            mb = dft_block(f1, False)
            for j in range(NT):
                cols = slice(j * 128, (j + 1) * 128)
                next(side)
                yb[f1, :R2, cols], yb[f1, R2:, cols] = cmatmul(mb, zb[f1, :R2, cols], zb[f1, R2:, cols])
        return 0

    lax.fori_loop(0, R1 // 2, dft, 0)

    def idft(g, _):
        for half in range(2):
            f1 = g + half * (R1 // 2)
            mbt = dft_block(f1, True)
            for j in range(NT):
                cols = slice(j * 128, (j + 1) * 128)
                wr = wst[0, j, pl.ds(g, R2, stride=R1 // 2), :]
                wi = wst[1, j, pl.ds(g, R2, stride=R1 // 2), :]
                if half == 0:
                    wr, wi = wr << 16, wi << 16
                else:
                    wr, wi = wr & u32(0xFFFF0000), wi & u32(0xFFFF0000)
                wr, wi = pltpu.bitcast(wr, f32), pltpu.bitcast(wi, f32)
                xr, xi = yb[f1, :R2, cols], yb[f1, R2:, cols]
                zb[f1, :R2, cols], zb[f1, R2:, cols] = cmatmul(mbt, xr * wr - xi * wi, xr * wi + xi * wr)
        return 0

    lax.fori_loop(0, R1 // 2, idft, 0)

    def inv(g, _):
        r0 = pl.multiple_of(g * G, G)
        lane0 = lax.broadcasted_iota(jnp.int32, (R1 * G, 128), 1) == 0

        def tile(j):
            ys = []
            for h in range(G // 8):
                ys += _fft([(zb[f1, pl.ds(r0 + h * 8, 8), j * 128:(j + 1) * 128],
                             zb[f1, pl.ds(R2 + r0 + h * 8, 8), j * 128:(j + 1) * 128]) for f1 in range(R1)], +1)
            return (jnp.concatenate([y[0] for y in ys], axis=0),
                    jnp.concatenate([y[1] for y in ys], axis=0))

        nyq = tile(4)[0]
        gs = []
        for j in range(4):
            yr, yi = tile(j)
            if j == 0:
                yi = jnp.where(lane0, nyq, yi)
            p = _dot_nt(jnp.concatenate([yr, yi], axis=1).astype(bf16), fd[j])
            gs.append((p[:, :128], p[:, 128:]))
        y = jnp.concatenate(_rfft8_adjoint(gs), axis=1)
        for t1 in range(R1):
            xb[g, t1] = jnp.concatenate(
                [y[(h * R1 + t1) * 8:(h * R1 + t1 + 1) * 8] for h in range(G // 8)], axis=0).astype(bf16)
        return 0

    lax.fori_loop(0, R2 // G, inv, 0)


def _attention_phase(xa, mem_ref, wqkv, pre, wo, outa, before_steps, store_rows):
    row = lax.broadcasted_iota(jnp.int32, (L, L), 0)
    col = lax.broadcasted_iota(jnp.int32, (L, L), 1)

    def step(s, mem, ahead):
        mask = (row < M) | (row >= col)
        rows = pl.ds(pl.multiple_of(s * SEG, SEG), SEG)
        h = jnp.concatenate([mem, xa[rows, :].astype(f32)], axis=0)
        if ahead:
            h = h[:L - 8]
        st = {}

        def project(hd, lo, hi):
            w = jnp.concatenate([wqkv[hd, j, lo // 2:hi // 2, :] for j in range(3)], axis=1)
            return _dot(h[:, lo:hi], pltpu.bitcast(w, bf16))

        n_early, split = (2, D // 2) if ahead else (4, D // 4)
        for hd in range(n_early):
            st['early', hd] = project(hd, 0, split)

        def do_qkv(hd):
            qkv = st['early', hd] + project(hd, split, D) if ('early', hd) in st else project(hd, 0, D)
            if ahead:
                r8 = pl.ds(pl.multiple_of(s * 8, 8), 8)
                qkv = jnp.concatenate(
                    [qkv, jnp.concatenate([pre[hd, j, r8, :] for j in range(3)], axis=1)], axis=0)
            st['q', hd] = qkv[:, :128] * (DH ** -0.5)
            st['k', hd] = qkv[:, 128:256].astype(bf16)
            st['v', hd] = qkv[:, 256:].astype(bf16)

        def do_qk(hd):
            sc = jnp.where(mask, _dot_nt(st['q', hd], st['k', hd]), -1e9)
            e = jnp.exp(sc - jnp.max(sc, axis=1, keepdims=True))
            st['e', hd] = e
            den = jnp.sum(e, axis=1, keepdims=True)
            r = pl.reciprocal(den, approx=True)
            st['r', hd] = r * (2.0 - den * r)

        def do_pv(hd):
            st['o', hd] = _dot(st['e', hd], st['v', hd]) * st['r', hd]

        def do_wo(g, ng=4):
            o = jnp.concatenate([st['o', hd] for hd in range(g * ng, (g + 1) * ng)], axis=1)
            for n in range(8):
                r = _dot(o, pltpu.bitcast(wo[g * ng * 64:(g + 1) * ng * 64, n * 128:(n + 1) * 128], bf16))
                st['out', n] = st['out', n] + r if ('out', n) in st else r

        for t in range(H):
            do_qkv(t)
            if t >= 1: do_qk(t - 1)
            if t >= 3: do_pv(t - 3)
        do_wo(0); do_pv(H - 3)
        do_wo(1); do_qk(H - 1); do_pv(H - 2)
        do_wo(2)
        do_wo(3); do_pv(H - 1)
        do_wo(1, 16)
        out = jnp.concatenate([st['out', n] for n in range(8)], axis=1)
        outa[rows, :] = out[M:].astype(bf16)
        return out[:M].astype(bf16).astype(f32)

    def steps(ahead, i, mem):
        if ahead:
            before_steps(i)
        for u in range(UNROLL):
            mem = step(i * UNROLL + u, mem, ahead)
        store_rows(i)
        return mem

    mem = lax.fori_loop(0, PRE // UNROLL, functools.partial(steps, True), mem_ref[...].astype(f32))
    lax.fori_loop(PRE // UNROLL, NSEG // UNROLL, functools.partial(steps, False), mem)


def _kernel(xa_hbm, xa3_hbm, mem_hbm, wq_hbm, wk_hbm, wv_hbm, wo_hbm, xb_hbm, wr_hbm, wi_hbm, fd_hbm, fs_hbm,
            out_hbm, mem_ref, raw, wqkv, xq, xpre, pre, wo, xa, ya, xb, fd, fs, wraw, wnyq, wst, zb, yb,
            sems, xsem, fsem, wsem, osem):
    def copy(src, dst, i, priority=0):
        c = pltpu.make_async_copy(src, dst, sems.at[i])
        c.start(priority=priority)
        return c

    def xb_copy(g):
        return pltpu.make_async_copy(xb_hbm.at[:, pl.ds(pl.multiple_of(g * G, G), G), :], xb.at[g], xsem.at[g])

    def yb_copy(g):
        return pltpu.make_async_copy(
            xb.at[g], out_hbm.at[:, pl.ds(pl.multiple_of(g * G, G), G), pl.ds(D, D)], osem.at[1])

    def w_copy(j, hg):
        src = (wq_hbm, wk_hbm, wv_hbm)[j].bitcast(u32).at[:, pl.ds(hg * (HG // 2), HG // 2), :]
        c = j * (H // HG) + hg
        return pltpu.make_async_copy(src, raw.at[c].reshape(D, HG // 2, DH), wsem.at[c])

    small = [copy(fd_hbm, fd, 0), copy(fs_hbm, fs, 4), copy(mem_hbm, mem_ref, 5)]
    small += [copy(w.at[pl.ds(D // 2, 1), :], wnyq.at[c], 1 + c) for c, w in enumerate((wr_hbm, wi_hbm))]
    xb_copy(0).start()
    for c in small:
        c.wait()
    for g in range(1, R2 // G):
        xb_copy(g).start()

    def filter_copies(g):
        return [pltpu.make_async_copy(
            w.at[pl.ds(0, D // 2), pl.ds(pl.multiple_of(t * 128, 128), 128)], wraw.at[c * R1 + t], fsem.at[g])
            for t in (2 * g, 2 * g + 1) for c, w in enumerate((wr_hbm, wi_hbm))]

    def wait_rows(g):
        xb_copy(g).wait()

        @pl.when(g == 2)
        def _():
            for i in range(R1 // 2):
                for cp in filter_copies(i):
                    cp.start()
            x_ahead().start()

    def x_first():
        rows = pl.ds(0, XA0 * SEG)
        return pltpu.make_async_copy(xa_hbm.at[rows, :], xa.at[rows, :], sems.at[6])

    def x_ahead():
        return pltpu.make_async_copy(xa3_hbm.at[pl.ds(0, PRE), pl.ds(SEG - 8, 8), :], xq, sems.at[9])

    def wo_copy():
        return pltpu.make_async_copy(wo_hbm.bitcast(u32), wo, sems.at[7])

    def prepare_filter(g):
        for cp in filter_copies(g):
            cp.wait()

        @pl.when(g == R1 // 2 - 2)
        def _():
            for j in range(3):
                for hg in range(H // HG):
                    w_copy(j, hg).start()
            wo_copy().start()
            x_first().start()

        pairs = wraw.bitcast(u32)
        for t in (2 * g, 2 * g + 1):
            dst = pl.ds(pl.multiple_of(t * 64, 64), 64)
            for j in range(NT):
                for c in range(2):
                    if j < 4:
                        res = []
                        for k1 in _k1_pair(j):
                            w = pairs[c * R1 + t, pl.ds(k1 // 2, 64, stride=4), :]
                            res.append(pltpu.bitcast(w & u32(0xFFFF0000) if k1 % 2 else w << 16, f32))
                        if j == 0:
                            dc = lax.broadcasted_iota(jnp.int32, (8, 128), 0) == 0
                            res[:1] = [jnp.where(dc, 0.5 * res[0][:8], res[0][:8]), res[0][8:]]
                        tile = jnp.concatenate(res, axis=0)
                    else:
                        last = wnyq[c, :, pl.ds(pl.multiple_of(t * 128, 128), 128)].astype(f32)
                        tile = jnp.broadcast_to(0.5 * last, (128, 128))
                    tile = pltpu.bitcast(tile.T, u32)
                    wst[c, j, dst, :] = jnp.concatenate(
                        [(tile[r:r + 8] >> 16) | tile[r + 8:r + 16] for r in range(0, 128, 16)], axis=0)
                yield

    _spectral_phase(xb, fd, fs, wst, zb, yb, wait_rows, prepare_filter)

    x_ahead().wait()
    for s in range(PRE):
        xpre[s * 8:(s + 1) * 8, :] = xq[s].astype(f32)

    def relayout(c, _):
        pltpu.make_async_copy(raw.at[c], raw.at[c], wsem.at[c]).wait()
        j, h0 = c // (H // HG), (c % (H // HG)) * HG
        for i in range(HG // 2):
            w = raw[c, pl.ds(i, D, stride=HG // 2), :]
            for hd, bits in ((2 * i, w << 16), (2 * i + 1, w & u32(0xFFFF0000))):
                panel = pltpu.bitcast(bits, f32).astype(bf16)
                wqkv[h0 + hd, j] = pltpu.bitcast(panel, u32)
                pre[h0 + hd, j] = _dot(xpre[...], panel)
        return 0

    lax.fori_loop(0, 3 * H // HG, relayout, 0)
    wo_copy().wait()
    x_first().wait()
    rest = pl.ds(XA0 * SEG, S - XA0 * SEG)
    c_rest = copy(xa_hbm.at[rest, :], xa.at[rest, :], 8)
    for g in range(R2 // G):
        yb_copy(g).start()

    def before_steps(i):
        @pl.when(i == XA0 // UNROLL)
        def _():
            c_rest.wait()

    def out_copy(i):
        n = UNROLL * SEG
        dst = out_hbm.at[i // (R2 // n), pl.ds(pl.multiple_of((i % (R2 // n)) * n, n), n), pl.ds(0, D)]
        return pltpu.make_async_copy(ya.at[pl.ds(pl.multiple_of(i * n, n), n), :], dst, osem.at[0])

    _attention_phase(xa, mem_ref, wqkv, pre, wo, ya, before_steps, lambda i: out_copy(i).start())

    def drain(i, _):
        out_copy(i).wait()
        return 0

    lax.fori_loop(0, NSEG // UNROLL, drain, 0)
    for g in range(R2 // G):
        yb_copy(g).wait()


@jax.jit
def pallas_concat_heads__memory_aug_recurrent_mem_tr__spectral_gfnet__prompt_kernel(
    A_x, A_mem0, A_Wq, A_Wk, A_Wv, A_Wo, A_seg_len, B_x, B_w_r, B_w_i,
):
    del A_seg_len
    hbm = pl.BlockSpec(memory_space=pl.ANY)
    out = pl.pallas_call(
        _kernel,
        out_shape=jax.ShapeDtypeStruct((R1, R2, 2 * D), bf16),
        in_specs=[hbm] * 12,
        out_specs=hbm,
        scratch_shapes=[
            pltpu.VMEM((M, D), bf16),
            pltpu.VMEM((3 * H // HG, D * HG // 2, DH), u32),
            pltpu.VMEM((H, 3, D // 2, DH), u32),
            pltpu.VMEM((PRE, 8, D), bf16),
            pltpu.VMEM((PRE * 8, D), f32),
            pltpu.VMEM((H, 3, PRE * 8, DH), f32),
            pltpu.VMEM((H * DH // 2, D), u32),
            pltpu.VMEM((S, D), bf16),
            pltpu.VMEM((S, D), bf16),
            pltpu.VMEM((R2 // G, R1, G, D), bf16),
            pltpu.VMEM((4, 256, 256), bf16),
            pltpu.VMEM((2, R2 + R1, R2), f32),
            pltpu.VMEM((2 * R1, D // 2, 128), bf16),
            pltpu.VMEM((2, 1, S), bf16),
            pltpu.VMEM((2, NT, S // 2, 128), u32),
            pltpu.VMEM((R1, 2 * R2, NT * 128), f32),
            pltpu.VMEM((R1, 2 * R2, NT * 128), f32),
            pltpu.SemaphoreType.DMA((10,)),
            pltpu.SemaphoreType.DMA((R2 // G,)),
            pltpu.SemaphoreType.DMA((R1 // 2,)),
            pltpu.SemaphoreType.DMA((3 * H // HG,)),
            pltpu.SemaphoreType.DMA((2,)),
        ],
        compiler_params=pltpu.CompilerParams(vmem_limit_bytes=120 * 2 ** 20),
    )(
        A_x.reshape(S, D), A_x.reshape(NSEG, SEG, D), A_mem0.reshape(M, D),
        A_Wq, A_Wk, A_Wv,
        A_Wo.reshape(H * DH, D),
        B_x.reshape(R1, R2, D), B_w_r.T, B_w_i.T,
        jnp.asarray(_FD, dtype=bf16), jnp.asarray(_FS),
    )
    return out.reshape(1, S, 2 * D)
```

```python
import functools

import numpy as np
import jax
import jax.numpy as jnp
from jax import lax
import jax.experimental.pallas as pl
import jax.experimental.pallas.tpu as pltpu

S, D, H, DH, M, SEG = 2048, 1024, 32, 128, 8, 32
L = M + SEG
NSEG = S // SEG
DF = D // 2 + 1
R1, R2 = 16, 128
G = 16
HG = 16
UNROLL = 2
PRE = 28
XA0 = 4
UB = (1, 2, 2, 2, 2)
NT = 5
f32, bf16, u32 = jnp.float32, jnp.bfloat16, jnp.uint32


def _k1_pair(j):
    return j, (4 if j == 0 else 8 - j)


def _dft_constants():
    b = np.arange(128)[:, None]
    c = np.arange(64)[None, :]
    fd = np.zeros((4, 256, 256))
    for j in range(4):
        for half, k1 in enumerate(_k1_pair(j)):
            ang = 2.0 * np.pi * ((b * (k1 + 8 * c)) % D) / D
            co, si = np.cos(ang), np.sin(ang)
            re = slice(64 * half, 64 * half + 64)
            im = slice(128 + 64 * half, 128 + 64 * half + 64)
            if j == 0:
                rows = slice(128 * half, 128 * half + 128)
                fd[j, rows, re], fd[j, rows, im] = co, -si
            else:
                sg = 1.0 - 2.0 * half
                fd[j, :128, re], fd[j, :128, im] = co, -si
                fd[j, 128:, re], fd[j, 128:, im] = sg * si, sg * co
    fd[0, :128, 128] = 1.0 - 2.0 * (np.arange(128) % 2)
    n = np.arange(R2)
    a = -2.0 * np.pi * np.concatenate([(n[:, None] * n[None, :]) % R2 / R2,
                                       np.arange(R1)[:, None] * n[None, :] / S], axis=0)
    return fd.astype(np.float32), np.stack([np.cos(a), np.sin(a)]).astype(np.float32)


_FD, _FS = _dft_constants()
_RH = float(np.sqrt(0.5))


def _dot(a, b):
    return lax.dot_general(a, b, (((1,), (0,)), ((), ())), preferred_element_type=f32)


def _dot_nt(a, b):
    return lax.dot_general(a, b, (((1,), (1,)), ((), ())), preferred_element_type=f32)


def _dot_tn(a, b):
    return lax.dot_general(a, b, (((0,), (0,)), ((), ())), preferred_element_type=f32)


def _cmul_const(x, e, n, sign):
    xr, xi = x
    e = e % n
    if e == 0:
        return x
    if 4 * e == n:
        return (_neg(xi), xr) if sign > 0 else (xi, _neg(xr))
    c = float(np.cos(2.0 * np.pi * e / n))
    s = float(sign * np.sin(2.0 * np.pi * e / n))
    if xi is None:
        return xr * c, xr * s
    if 8 * e == n or 8 * e == 3 * n:
        if c * s > 0:
            return (xr - xi) * c, (xr + xi) * c
        return (xr + xi) * c, (xi - xr) * c
    return xr * c - xi * s, xr * s + xi * c


def _neg(a):
    return None if a is None else -a


def _add(a, b):
    return b if a is None else a if b is None else a + b


def _sub(a, b):
    return _neg(b) if a is None else a if b is None else a - b


def _fft(xs, sign):
    n = len(xs)
    if n == 1:
        return xs
    ev, od = _fft(xs[0::2], sign), _fft(xs[1::2], sign)
    out = [None] * n
    for j in range(n // 2):
        e = ev[j]
        if 4 * j == n:
            orr, oi = od[j]
            if sign > 0:
                out[j] = (_sub(e[0], oi), _add(e[1], orr))
                out[j + n // 2] = (_add(e[0], oi), _sub(e[1], orr))
            else:
                out[j] = (_add(e[0], oi), _sub(e[1], orr))
                out[j + n // 2] = (_sub(e[0], oi), _add(e[1], orr))
            continue
        t = _cmul_const(od[j], j, n, sign)
        out[j] = (_add(e[0], t[0]), _add(e[1], t[1]))
        out[j + n // 2] = (_sub(e[0], t[0]), _sub(e[1], t[1]))
    return out


def _rfft8(x):
    s04, d04, s26, d26 = x[0] + x[4], x[0] - x[4], x[2] + x[6], x[2] - x[6]
    s15, d15, s37, d37 = x[1] + x[5], x[1] - x[5], x[3] + x[7], x[3] - x[7]
    e, o = s04 + s26, s15 + s37
    p, q = (d15 - d37) * _RH, (d15 + d37) * _RH
    return [(e + o, e - o), (d04 + p, -(d26 + q)), (s04 - s26, s37 - s15), (d04 - p, d26 - q)]


def _rfft8_adjoint(g):
    (g0, g4), (r1, i1), (r2, i2), (r3, i3) = g
    e, o = g0 + g4, g0 - g4
    s04, s26, s15, s37 = e + r2, e - r2, o - i2, o + i2
    d04, d26 = r1 + r3, i3 - i1
    p, q = (r1 - r3) * _RH, (i1 + i3) * _RH
    d15, d37 = p - q, -(p + q)
    return [s04 + d04, s15 + d15, s26 + d26, s37 + d37, s04 - d04, s15 - d15, s26 - d26, s37 - d37]


def _loop(n, unroll, body, before=None):
    def group(i, _):
        if before is not None:
            for u in range(unroll):
                before(i * unroll + u)
        for u in range(unroll):
            body(i * unroll + u)
        return 0

    lax.fori_loop(0, n // unroll, group, 0)


def _spectral_phase(xb, fd, fs, wst, zb, yb, wait_rows, wait_filter, prepare_filter):
    groups = [(h, t1) for h in range(G // 8) for t1 in range(R1)]

    def fwd(g):
        r0 = pl.multiple_of(g * G, G)
        lane0 = lax.broadcasted_iota(jnp.int32, (R1 * G, 128), 1) == 0
        xg = [xb[g, t1].astype(f32) for t1 in range(R1)]
        xg = jnp.concatenate([xg[t1][h * 8:(h + 1) * 8] for h, t1 in groups], axis=0)
        us = _rfft8([xg[:, a * 128:(a + 1) * 128] for a in range(8)])
        us = [jnp.concatenate(u, axis=1).astype(bf16) for u in us]
        nyq = None
        for j in range(NT):
            if j < 4:
                z = _dot(us[j], fd[j])
                zr, zi = z[:, :128], z[:, 128:]
                if j == 0:
                    nyq = jnp.where(lane0, zi, 0.0)
                    zi = jnp.where(lane0, 0.0, zi)
                xs = [(zr[n * 8:(n + 1) * 8], zi[n * 8:(n + 1) * 8]) for n in range(len(groups))]
            else:
                xs = [(nyq[n * 8:(n + 1) * 8], None) for n in range(len(groups))]
            for h in range(G // 8):
                for f1, (yr, yi) in enumerate(_fft(xs[h * R1:(h + 1) * R1], -1)):
                    zb[f1, pl.ds(r0 + h * 8, 8), j * 128:(j + 1) * 128] = yr
                    zb[f1, pl.ds(R2 + r0 + h * 8, 8), j * 128:(j + 1) * 128] = (
                        jnp.zeros_like(yr) if yi is None else yi)

    _loop(R2 // G, UB[0], fwd, wait_rows)

    def dft_block(f1, inverse):
        cr, ci = fs[0, :R2, :], fs[1, :R2, :]
        tr, ti = fs[0, pl.ds(R2 + f1, 1), :], fs[1, pl.ds(R2 + f1, 1), :]
        if inverse:
            tr, ti = tr * (2.0 / (S * D)), ti * (2.0 / (S * D))
        mr, mi = cr * tr - ci * ti, cr * ti + ci * tr
        if inverse:
            return [m.astype(bf16).T for m in (mr, -mi - mr, mr - mi)]
        return [m.astype(bf16) for m in (mr, mi - mr, mr + mi)]

    def cmatmul(m, xr, xi):
        k = _dot(m[0], (xr + xi).astype(bf16))
        return k - _dot(m[2], xi.astype(bf16)), k + _dot(m[1], xr.astype(bf16))

    def dft(g):
        side = prepare_filter(g)
        for f1 in (2 * g, 2 * g + 1):
            mb = dft_block(f1, False)
            for j in range(NT):
                cols = slice(j * 128, (j + 1) * 128)
                next(side)
                yb[f1, :R2, cols], yb[f1, R2:, cols] = cmatmul(mb, zb[f1, :R2, cols], zb[f1, R2:, cols])

    _loop(R1 // 2, UB[1], dft, wait_filter)

    def idft(g):
        for half in range(2):
            f1 = g + half * (R1 // 2)
            mbt = dft_block(f1, True)
            for j in range(NT):
                cols = slice(j * 128, (j + 1) * 128)
                wr = wst[0, j, pl.ds(g, R2, stride=R1 // 2), :]
                wi = wst[1, j, pl.ds(g, R2, stride=R1 // 2), :]
                if half == 0:
                    wr, wi = wr << 16, wi << 16
                else:
                    wr, wi = wr & u32(0xFFFF0000), wi & u32(0xFFFF0000)
                wr, wi = pltpu.bitcast(wr, f32), pltpu.bitcast(wi, f32)
                xr, xi = yb[f1, :R2, cols], yb[f1, R2:, cols]
                zb[f1, :R2, cols], zb[f1, R2:, cols] = cmatmul(mbt, xr * wr - xi * wi, xr * wi + xi * wr)

    _loop(R1 // 2, UB[2], idft)

    def inv(g):
        r0 = pl.multiple_of(g * G, G)
        lane0 = lax.broadcasted_iota(jnp.int32, (R1 * G, 128), 1) == 0

        def tile(j):
            ys = []
            for h in range(G // 8):
                ys += _fft([(zb[f1, pl.ds(r0 + h * 8, 8), j * 128:(j + 1) * 128],
                             zb[f1, pl.ds(R2 + r0 + h * 8, 8), j * 128:(j + 1) * 128]) for f1 in range(R1)], +1)
            return (jnp.concatenate([y[0] for y in ys], axis=0),
                    jnp.concatenate([y[1] for y in ys], axis=0))

        nyq = tile(4)[0]
        gs = []
        for j in range(4):
            yr, yi = tile(j)
            if j == 0:
                yi = jnp.where(lane0, nyq, yi)
            p = _dot_nt(jnp.concatenate([yr, yi], axis=1).astype(bf16), fd[j])
            gs.append((p[:, :128], p[:, 128:]))
        y = jnp.concatenate(_rfft8_adjoint(gs), axis=1)
        for t1 in range(R1):
            xb[g, t1] = jnp.concatenate(
                [y[(h * R1 + t1) * 8:(h * R1 + t1 + 1) * 8] for h in range(G // 8)], axis=0).astype(bf16)

    _loop(R2 // G, UB[3], inv)


def _attention_phase(xa, mem_ref, wqkv, pre, wo, outa, before_steps, store_rows):
    row = lax.broadcasted_iota(jnp.int32, (L, L), 0)
    col = lax.broadcasted_iota(jnp.int32, (L, L), 1)

    def step(s, mem, ahead):
        mask = (row < M) | (row >= col)
        rows = pl.ds(pl.multiple_of(s * SEG, SEG), SEG)
        h = jnp.concatenate([mem, xa[rows, :].astype(f32)], axis=0)
        if ahead:
            h = h[:L - 8]
        st = {}

        def project(hd, lo, hi):
            w = jnp.concatenate([wqkv[hd, j, lo // 2:hi // 2, :] for j in range(3)], axis=1)
            return _dot(h[:, lo:hi], pltpu.bitcast(w, bf16))

        n_early, split = (2, D // 2) if ahead else (4, D // 4)
        for hd in range(n_early):
            st['early', hd] = project(hd, 0, split)

        def do_qkv(hd):
            qkv = st['early', hd] + project(hd, split, D) if ('early', hd) in st else project(hd, 0, D)
            if ahead:
                r8 = pl.ds(pl.multiple_of(s * 8, 8), 8)
                qkv = jnp.concatenate(
                    [qkv, jnp.concatenate([pre[hd, j, r8, :] for j in range(3)], axis=1)], axis=0)
            st['q', hd] = qkv[:, :128] * (DH ** -0.5)
            st['k', hd] = qkv[:, 128:256].astype(bf16)
            st['v', hd] = qkv[:, 256:].astype(bf16)

        def do_qk(hd):
            sc = jnp.where(mask, _dot_nt(st['q', hd], st['k', hd]), -1e9)
            e = jnp.exp(sc - jnp.max(sc, axis=1, keepdims=True))
            st['e', hd] = e
            den = jnp.sum(e, axis=1, keepdims=True)
            r = pl.reciprocal(den, approx=True)
            st['r', hd] = r * (2.0 - den * r)

        def do_pv(hd):
            st['o', hd] = _dot(st['e', hd], st['v', hd]) * st['r', hd]

        def do_wo(g, ng=4):
            o = jnp.concatenate([st['o', hd] for hd in range(g * ng, (g + 1) * ng)], axis=1)
            for n in range(8):
                r = _dot(o, pltpu.bitcast(wo[g * ng * 64:(g + 1) * ng * 64, n * 128:(n + 1) * 128], bf16))
                st['out', n] = st['out', n] + r if ('out', n) in st else r

        for t in range(H):
            do_qkv(t)
            if t >= 1: do_qk(t - 1)
            if t >= 3: do_pv(t - 3)
        do_wo(0); do_pv(H - 3)
        do_wo(1); do_qk(H - 1); do_pv(H - 2)
        do_wo(2)
        do_wo(3); do_pv(H - 1)
        do_wo(1, 16)
        out = jnp.concatenate([st['out', n] for n in range(8)], axis=1)
        outa[rows, :] = out[M:].astype(bf16)
        return out[:M].astype(bf16).astype(f32)

    def steps(ahead, i, mem):
        if ahead:
            before_steps(i)
        for u in range(UNROLL):
            mem = step(i * UNROLL + u, mem, ahead)
        store_rows(i)
        return mem

    mem = lax.fori_loop(0, PRE // UNROLL, functools.partial(steps, True), mem_ref[...].astype(f32))
    lax.fori_loop(PRE // UNROLL, NSEG // UNROLL, functools.partial(steps, False), mem)


def _kernel(xa_hbm, xa3_hbm, mem_hbm, wq_hbm, wk_hbm, wv_hbm, wo_hbm, xb_hbm, wr_hbm, wi_hbm, fd_hbm, fs_hbm,
            out_hbm, mem_ref, raw, wqkv, xq, xpre, pre, wo, xa, ya, xb, fd, fs, wraw, wnyq, wst, zb, yb,
            sems, xsem, fsem, wsem, osem):
    def copy(src, dst, i, priority=0):
        c = pltpu.make_async_copy(src, dst, sems.at[i])
        c.start(priority=priority)
        return c

    def xb_copy(g):
        return pltpu.make_async_copy(xb_hbm.at[:, pl.ds(pl.multiple_of(g * G, G), G), :], xb.at[g], xsem.at[g])

    def yb_copy(g):
        return pltpu.make_async_copy(
            xb.at[g], out_hbm.at[:, pl.ds(pl.multiple_of(g * G, G), G), pl.ds(D, D)], osem.at[1])

    def raw_chunk(c):
        return raw.at[c, pl.ds(0, D * HG // 2), :]

    def w_copy(j, hg):
        src = (wq_hbm, wk_hbm, wv_hbm)[j].bitcast(u32).at[:, pl.ds(hg * (HG // 2), HG // 2), :]
        c = j * (H // HG) + hg
        return pltpu.make_async_copy(src, raw_chunk(c).reshape(D, HG // 2, DH), wsem.at[c])

    small = [copy(fd_hbm, fd, 0), copy(fs_hbm, fs, 4), copy(mem_hbm, mem_ref, 5)]
    small += [copy(w.at[pl.ds(D // 2, 1), :], wnyq.at[c], 1 + c) for c, w in enumerate((wr_hbm, wi_hbm))]
    xb_copy(0).start()
    for c in small:
        c.wait()
    for g in range(1, R2 // G):
        xb_copy(g).start()

    def filter_copies(g):
        return [pltpu.make_async_copy(
            w.at[pl.ds(0, D // 2), pl.ds(pl.multiple_of(t * 128, 128), 128)], wraw.at[c * R1 + t, pl.ds(0, D // 2), :], fsem.at[g])
            for t in (2 * g, 2 * g + 1) for c, w in enumerate((wr_hbm, wi_hbm))]

    def wait_rows(g):
        xb_copy(g).wait()

        @pl.when(g == 2)
        def _():
            for i in range(R1 // 2):
                for cp in filter_copies(i):
                    cp.start()
            x_ahead().start()

    def x_first():
        rows = pl.ds(0, XA0 * SEG)
        return pltpu.make_async_copy(xa_hbm.at[rows, :], xa.at[rows, :], sems.at[6])

    def x_ahead():
        return pltpu.make_async_copy(xa3_hbm.at[pl.ds(0, PRE), pl.ds(SEG - 8, 8), :], xq, sems.at[9])

    def wo_copy():
        return pltpu.make_async_copy(wo_hbm.bitcast(u32), wo, sems.at[7])

    def wait_filter(g):
        for cp in filter_copies(g):
            cp.wait()

        @pl.when(g == R1 // 2 - 2)
        def _():
            for j in range(3):
                for hg in range(H // HG):
                    w_copy(j, hg).start()
            wo_copy().start()
            x_first().start()

    def prepare_filter(g):
        pairs = wraw.bitcast(u32)
        for t in (2 * g, 2 * g + 1):
            dst = pl.ds(pl.multiple_of(t * 64, 64), 64)
            for j in range(NT):
                for c in range(2):
                    if j < 4:
                        res = []
                        for k1 in _k1_pair(j):
                            w = pairs[c * R1 + t, pl.ds(k1 // 2, 64, stride=4), :]
                            res.append(pltpu.bitcast(w & u32(0xFFFF0000) if k1 % 2 else w << 16, f32))
                        if j == 0:
                            dc = lax.broadcasted_iota(jnp.int32, (8, 128), 0) == 0
                            res[:1] = [jnp.where(dc, 0.5 * res[0][:8], res[0][:8]), res[0][8:]]
                        tile = jnp.concatenate(res, axis=0)
                    else:
                        last = wnyq[c, :, pl.ds(pl.multiple_of(t * 128, 128), 128)].astype(f32)
                        tile = jnp.broadcast_to(0.5 * last, (128, 128))
                    tile = pltpu.bitcast(tile.T, u32)
                    wst[c, j, dst, :] = jnp.concatenate(
                        [(tile[r:r + 8] >> 16) | tile[r + 8:r + 16] for r in range(0, 128, 16)], axis=0)
                yield

    _spectral_phase(xb, fd, fs, wst, zb, yb, wait_rows, wait_filter, prepare_filter)

    x_ahead().wait()
    for s in range(PRE):
        xpre[s * 8:(s + 1) * 8, :] = xq[s].astype(f32)

    def relayout(c):
        j, h0 = c // (H // HG), (c % (H // HG)) * HG
        for i in range(HG // 2):
            w = raw[c, pl.ds(i, D, stride=HG // 2), :]
            for hd, bits in ((2 * i, w << 16), (2 * i + 1, w & u32(0xFFFF0000))):
                panel = pltpu.bitcast(bits, f32).astype(bf16)
                wqkv[h0 + hd, j] = pltpu.bitcast(panel, u32)
                pre[h0 + hd, j] = _dot(xpre[...], panel)

    _loop(3 * H // HG, UB[4], relayout,
          lambda c: pltpu.make_async_copy(raw_chunk(c), raw_chunk(c), wsem.at[c]).wait())
    wo_copy().wait()
    x_first().wait()
    rest = pl.ds(XA0 * SEG, S - XA0 * SEG)
    c_rest = copy(xa_hbm.at[rest, :], xa.at[rest, :], 8)
    for g in range(R2 // G):
        yb_copy(g).start()

    def before_steps(i):
        @pl.when(i == XA0 // UNROLL)
        def _():
            c_rest.wait()

    def out_copy(i):
        n = UNROLL * SEG
        dst = out_hbm.at[i // (R2 // n), pl.ds(pl.multiple_of((i % (R2 // n)) * n, n), n), pl.ds(0, D)]
        return pltpu.make_async_copy(ya.at[pl.ds(pl.multiple_of(i * n, n), n), :], dst, osem.at[0])

    _attention_phase(xa, mem_ref, wqkv, pre, wo, ya, before_steps, lambda i: out_copy(i).start())

    def drain(i, _):
        out_copy(i).wait()
        return 0

    lax.fori_loop(0, NSEG // UNROLL, drain, 0)
    for g in range(R2 // G):
        yb_copy(g).wait()


@jax.jit
def pallas_concat_heads__memory_aug_recurrent_mem_tr__spectral_gfnet__prompt_kernel(
    A_x, A_mem0, A_Wq, A_Wk, A_Wv, A_Wo, A_seg_len, B_x, B_w_r, B_w_i,
):
    del A_seg_len
    hbm = pl.BlockSpec(memory_space=pl.ANY)
    out = pl.pallas_call(
        _kernel,
        out_shape=jax.ShapeDtypeStruct((R1, R2, 2 * D), bf16),
        in_specs=[hbm] * 12,
        out_specs=hbm,
        scratch_shapes=[
            pltpu.VMEM((M, D), bf16),
            pltpu.VMEM((3 * H // HG, D * HG // 2 + 8, DH), u32),
            pltpu.VMEM((H, 3, D // 2, DH), u32),
            pltpu.VMEM((PRE, 8, D), bf16),
            pltpu.VMEM((PRE * 8, D), f32),
            pltpu.VMEM((H, 3, PRE * 8, DH), f32),
            pltpu.VMEM((H * DH // 2, D), u32),
            pltpu.VMEM((S, D), bf16),
            pltpu.VMEM((S, D), bf16),
            pltpu.VMEM((R2 // G, R1, G, D), bf16),
            pltpu.VMEM((4, 256, 256), bf16),
            pltpu.VMEM((2, R2 + R1, R2), f32),
            pltpu.VMEM((2 * R1, D // 2 + 16, 128), bf16),
            pltpu.VMEM((2, 1, S), bf16),
            pltpu.VMEM((2, NT, S // 2 + 8, 128), u32),
            pltpu.VMEM((R1, 2 * R2, NT * 128), f32),
            pltpu.VMEM((R1, 2 * R2, NT * 128), f32),
            pltpu.SemaphoreType.DMA((10,)),
            pltpu.SemaphoreType.DMA((R2 // G,)),
            pltpu.SemaphoreType.DMA((R1 // 2,)),
            pltpu.SemaphoreType.DMA((3 * H // HG,)),
            pltpu.SemaphoreType.DMA((2,)),
        ],
        compiler_params=pltpu.CompilerParams(vmem_limit_bytes=120 * 2 ** 20),
    )(
        A_x.reshape(S, D), A_x.reshape(NSEG, SEG, D), A_mem0.reshape(M, D),
        A_Wq, A_Wk, A_Wv,
        A_Wo.reshape(H * DH, D),
        B_x.reshape(R1, R2, D), B_w_r.T, B_w_i.T,
        jnp.asarray(_FD, dtype=bf16), jnp.asarray(_FS),
    )
    return out.reshape(1, S, 2 * D)
```

```python
import functools

import numpy as np
import jax
import jax.numpy as jnp
from jax import lax
import jax.experimental.pallas as pl
import jax.experimental.pallas.tpu as pltpu

S, D, H, DH, M, SEG = 2048, 1024, 32, 128, 8, 32
L = M + SEG
NSEG = S // SEG
DF = D // 2 + 1
R1, R2 = 16, 128
G = 16
HG = 16
UNROLL = 2
PRE = 30
XA0 = 4
UB = (1, 2, 2, 2, 2)
NT = 4
f32, bf16, u32 = jnp.float32, jnp.bfloat16, jnp.uint32


def _k1_pair(j):
    return j, (4 if j == 0 else 8 - j)


def _dft_constants():
    b = np.arange(128)[:, None]
    c = np.arange(64)[None, :]
    fd = np.zeros((4, 256, 256))
    for j in range(4):
        for half, k1 in enumerate(_k1_pair(j)):
            ang = 2.0 * np.pi * ((b * (k1 + 8 * c)) % D) / D
            co, si = np.cos(ang), np.sin(ang)
            re = slice(64 * half, 64 * half + 64)
            im = slice(128 + 64 * half, 128 + 64 * half + 64)
            if j == 0:
                rows = slice(128 * half, 128 * half + 128)
                fd[j, rows, re], fd[j, rows, im] = co, -si
            else:
                sg = 1.0 - 2.0 * half
                fd[j, :128, re], fd[j, :128, im] = co, -si
                fd[j, 128:, re], fd[j, 128:, im] = sg * si, sg * co
    fd[0, :128, 128] = 1.0 - 2.0 * (np.arange(128) % 2)
    n = np.arange(R2)
    a = -2.0 * np.pi * np.concatenate([(n[:, None] * n[None, :]) % R2 / R2,
                                       np.arange(R1)[:, None] * n[None, :] / S,
                                       n[:, None] * n[None, :] / S], axis=0)
    return fd.astype(np.float32), np.stack([np.cos(a), np.sin(a)]).astype(np.float32)


_FD, _FS = _dft_constants()
_RH = float(np.sqrt(0.5))


def _dot(a, b):
    return lax.dot_general(a, b, (((1,), (0,)), ((), ())), preferred_element_type=f32)


def _dot_nt(a, b):
    return lax.dot_general(a, b, (((1,), (1,)), ((), ())), preferred_element_type=f32)


def _dot_tn(a, b):
    return lax.dot_general(a, b, (((0,), (0,)), ((), ())), preferred_element_type=f32)


def _cmul_const(x, e, n, sign):
    xr, xi = x
    e = e % n
    if e == 0:
        return x
    if 4 * e == n:
        return (_neg(xi), xr) if sign > 0 else (xi, _neg(xr))
    c = float(np.cos(2.0 * np.pi * e / n))
    s = float(sign * np.sin(2.0 * np.pi * e / n))
    if xi is None:
        return xr * c, xr * s
    if 8 * e == n or 8 * e == 3 * n:
        if c * s > 0:
            return (xr - xi) * c, (xr + xi) * c
        return (xr + xi) * c, (xi - xr) * c
    return xr * c - xi * s, xr * s + xi * c


def _neg(a):
    return None if a is None else -a


def _add(a, b):
    return b if a is None else a if b is None else a + b


def _sub(a, b):
    return _neg(b) if a is None else a if b is None else a - b


def _fft(xs, sign):
    n = len(xs)
    if n == 1:
        return xs
    ev, od = _fft(xs[0::2], sign), _fft(xs[1::2], sign)
    out = [None] * n
    for j in range(n // 2):
        e = ev[j]
        if 4 * j == n:
            orr, oi = od[j]
            if sign > 0:
                out[j] = (_sub(e[0], oi), _add(e[1], orr))
                out[j + n // 2] = (_add(e[0], oi), _sub(e[1], orr))
            else:
                out[j] = (_add(e[0], oi), _sub(e[1], orr))
                out[j + n // 2] = (_sub(e[0], oi), _add(e[1], orr))
            continue
        t = _cmul_const(od[j], j, n, sign)
        out[j] = (_add(e[0], t[0]), _add(e[1], t[1]))
        out[j + n // 2] = (_sub(e[0], t[0]), _sub(e[1], t[1]))
    return out


def _rfft8(x):
    s04, d04, s26, d26 = x[0] + x[4], x[0] - x[4], x[2] + x[6], x[2] - x[6]
    s15, d15, s37, d37 = x[1] + x[5], x[1] - x[5], x[3] + x[7], x[3] - x[7]
    e, o = s04 + s26, s15 + s37
    p, q = (d15 - d37) * _RH, (d15 + d37) * _RH
    return [(e + o, e - o), (d04 + p, -(d26 + q)), (s04 - s26, s37 - s15), (d04 - p, d26 - q)]


def _rfft8_adjoint(g):
    (g0, g4), (r1, i1), (r2, i2), (r3, i3) = g
    e, o = g0 + g4, g0 - g4
    s04, s26, s15, s37 = e + r2, e - r2, o - i2, o + i2
    d04, d26 = r1 + r3, i3 - i1
    p, q = (r1 - r3) * _RH, (i1 + i3) * _RH
    d15, d37 = p - q, -(p + q)
    return [s04 + d04, s15 + d15, s26 + d26, s37 + d37, s04 - d04, s15 - d15, s26 - d26, s37 - d37]


def _loop(n, unroll, body, before=None):
    def group(i, _):
        if before is not None:
            for u in range(unroll):
                before(i * unroll + u)
        for u in range(unroll):
            body(i * unroll + u)
        return 0

    lax.fori_loop(0, n // unroll, group, 0)


def _spectral_phase(xb, fd, fs, wst, wnyq, zb, yb, zn, wait_rows, wait_filter, prepare_filter):
    groups = [(h, t1) for h in range(G // 8) for t1 in range(R1)]

    def fwd(g):
        r0 = pl.multiple_of(g * G, G)
        lane0 = lax.broadcasted_iota(jnp.int32, (R1 * G, 128), 1) == 0
        xg = [xb[g, t1].astype(f32) for t1 in range(R1)]
        xg = jnp.concatenate([xg[t1][h * 8:(h + 1) * 8] for h, t1 in groups], axis=0)
        us = _rfft8([xg[:, a * 128:(a + 1) * 128] for a in range(8)])
        us = [jnp.concatenate(u, axis=1).astype(bf16) for u in us]
        for j in range(NT):
            z = _dot(us[j], fd[j])
            zr, zi = z[:, :128], z[:, 128:]
            if j == 0:
                for h in range(G // 8):
                    ys = _fft([(jnp.where(lane0[:8], zi[n * 8:(n + 1) * 8], 0.0), None)
                               for n in range(h * R1, (h + 1) * R1)], -1)
                    for c in range(2):
                        parts = [pltpu.roll(y[c], f1, 1) if f1 else y[c]
                                 for f1, y in enumerate(ys) if y[c] is not None]
                        zn[c, pl.ds(r0 + h * 8, 8), :] = functools.reduce(jnp.add, parts)
                zi = jnp.where(lane0, 0.0, zi)
            xs = [(zr[n * 8:(n + 1) * 8], zi[n * 8:(n + 1) * 8]) for n in range(len(groups))]
            for h in range(G // 8):
                for f1, (yr, yi) in enumerate(_fft(xs[h * R1:(h + 1) * R1], -1)):
                    zb[f1, pl.ds(r0 + h * 8, 8), j * 128:(j + 1) * 128] = yr
                    zb[f1, pl.ds(R2 + r0 + h * 8, 8), j * 128:(j + 1) * 128] = yi

    _loop(R2 // G, UB[0], fwd, wait_rows)

    def dft_block(f1, inverse):
        cr, ci = fs[0, :R2, :], fs[1, :R2, :]
        tr, ti = fs[0, pl.ds(R2 + f1, 1), :], fs[1, pl.ds(R2 + f1, 1), :]
        if inverse:
            tr, ti = tr * (2.0 / (S * D)), ti * (2.0 / (S * D))
        mr, mi = cr * tr - ci * ti, cr * ti + ci * tr
        if inverse:
            return [m.astype(bf16).T for m in (mr, -mi - mr, mr - mi)]
        return [m.astype(bf16) for m in (mr, mi - mr, mr + mi)]

    def cmatmul(m, xr, xi):
        k = _dot(m[0], (xr + xi).astype(bf16))
        return k - _dot(m[2], xi.astype(bf16)), k + _dot(m[1], xr.astype(bf16))

    tr, ti = fs[0, R2 + R1:, :], fs[1, R2 + R1:, :]
    xr, xi = cmatmul(dft_block(0, False), zn[0] * tr - zn[1] * ti, zn[0] * ti + zn[1] * tr)

    def nyquist_filter(c):
        w = jnp.concatenate([jnp.broadcast_to(wnyq[c, :, t * 128:(t + 1) * 128].astype(f32), (8, 128))
                             for t in range(S // 128)], axis=0)
        f2 = lax.broadcasted_iota(jnp.int32, w.shape, 0)
        for bit in (1, 2, 4):
            w = jnp.where((f2 & bit) != 0, pltpu.roll(w, 128 - bit * R1, 1), w)
        return 0.5 * w

    wr, wi = nyquist_filter(0), nyquist_filter(1)
    yr, yi = cmatmul(dft_block(0, True), xr * wr - xi * wi, xr * wi + xi * wr)
    zn[0], zn[1] = yr * tr + yi * ti, yi * tr - yr * ti

    def dft(g):
        side = prepare_filter(g)
        for f1 in (2 * g, 2 * g + 1):
            mb = dft_block(f1, False)
            for j in range(NT):
                cols = slice(j * 128, (j + 1) * 128)
                next(side)
                yb[f1, :R2, cols], yb[f1, R2:, cols] = cmatmul(mb, zb[f1, :R2, cols], zb[f1, R2:, cols])

    _loop(R1 // 2, UB[1], dft, wait_filter)

    def idft(g):
        for half in range(2):
            f1 = g + half * (R1 // 2)
            mbt = dft_block(f1, True)
            for j in range(NT):
                cols = slice(j * 128, (j + 1) * 128)
                wr = wst[0, j, pl.ds(g, R2, stride=R1 // 2), :]
                wi = wst[1, j, pl.ds(g, R2, stride=R1 // 2), :]
                if half == 0:
                    wr, wi = wr << 16, wi << 16
                else:
                    wr, wi = wr & u32(0xFFFF0000), wi & u32(0xFFFF0000)
                wr, wi = pltpu.bitcast(wr, f32), pltpu.bitcast(wi, f32)
                xr, xi = yb[f1, :R2, cols], yb[f1, R2:, cols]
                zb[f1, :R2, cols], zb[f1, R2:, cols] = cmatmul(mbt, xr * wr - xi * wi, xr * wi + xi * wr)

    _loop(R1 // 2, UB[2], idft)

    def inv(g):
        r0 = pl.multiple_of(g * G, G)
        lane0 = lax.broadcasted_iota(jnp.int32, (R1 * G, 128), 1) == 0

        def tile(load):
            ys = []
            for h in range(G // 8):
                ys += _fft([load(f1, r0 + h * 8) for f1 in range(R1)], +1)
            return (jnp.concatenate([y[0] for y in ys], axis=0),
                    jnp.concatenate([y[1] for y in ys], axis=0))

        nyq = tile(lambda f1, r: tuple(pltpu.roll(zn[c, pl.ds(r, 8), :], 128 - f1, 1) if f1
                                       else zn[c, pl.ds(r, 8), :] for c in range(2)))[0]
        gs = []
        for j in range(4):
            yr, yi = tile(lambda f1, r: (zb[f1, pl.ds(r, 8), j * 128:(j + 1) * 128],
                                         zb[f1, pl.ds(R2 + r, 8), j * 128:(j + 1) * 128]))
            if j == 0:
                yi = jnp.where(lane0, nyq, yi)
            p = _dot_nt(jnp.concatenate([yr, yi], axis=1).astype(bf16), fd[j])
            gs.append((p[:, :128], p[:, 128:]))
        y = jnp.concatenate(_rfft8_adjoint(gs), axis=1)
        for t1 in range(R1):
            xb[g, t1] = jnp.concatenate(
                [y[(h * R1 + t1) * 8:(h * R1 + t1 + 1) * 8] for h in range(G // 8)], axis=0).astype(bf16)

    _loop(R2 // G, UB[3], inv)


def _attention_phase(xa, mem_ref, wqkv, pre, wo, outa, before_steps, store_rows):
    row = lax.broadcasted_iota(jnp.int32, (L, L), 0)
    col = lax.broadcasted_iota(jnp.int32, (L, L), 1)

    def step(s, mem, ahead):
        mask = (row < M) | (row >= col)
        rows = pl.ds(pl.multiple_of(s * SEG, SEG), SEG)
        h = jnp.concatenate([mem, xa[rows, :].astype(f32)], axis=0)
        if ahead:
            h = h[:L - 8]
        st = {}

        def project(hd, lo, hi):
            w = jnp.concatenate([wqkv[hd, j, lo // 2:hi // 2, :] for j in range(3)], axis=1)
            return _dot(h[:, lo:hi], pltpu.bitcast(w, bf16))

        n_early, split = (2, D // 2) if ahead else (4, D // 4)
        for hd in range(n_early):
            st['early', hd] = project(hd, 0, split)

        def do_qkv(hd):
            qkv = st['early', hd] + project(hd, split, D) if ('early', hd) in st else project(hd, 0, D)
            if ahead:
                r8 = pl.ds(pl.multiple_of(s * 8, 8), 8)
                qkv = jnp.concatenate(
                    [qkv, jnp.concatenate([pre[hd, j, r8, :] for j in range(3)], axis=1)], axis=0)
            st['q', hd] = qkv[:, :128] * (DH ** -0.5)
            st['k', hd] = qkv[:, 128:256].astype(bf16)
            st['v', hd] = qkv[:, 256:].astype(bf16)

        def do_qk(hd):
            sc = jnp.where(mask, _dot_nt(st['q', hd], st['k', hd]), -1e9)
            e = jnp.exp(sc - jnp.max(sc, axis=1, keepdims=True))
            st['e', hd] = e
            den = jnp.sum(e, axis=1, keepdims=True)
            r = pl.reciprocal(den, approx=True)
            st['r', hd] = r * (2.0 - den * r)

        def do_pv(hd):
            st['o', hd] = _dot(st['e', hd], st['v', hd]) * st['r', hd]

        def do_wo(g, ng=4):
            o = jnp.concatenate([st['o', hd] for hd in range(g * ng, (g + 1) * ng)], axis=1)
            for n in range(8):
                r = _dot(o, pltpu.bitcast(wo[g * ng * 64:(g + 1) * ng * 64, n * 128:(n + 1) * 128], bf16))
                st['out', n] = st['out', n] + r if ('out', n) in st else r

        for t in range(H):
            do_qkv(t)
            if t >= 1: do_qk(t - 1)
            if t >= 3: do_pv(t - 3)
        do_wo(0); do_pv(H - 3)
        do_wo(1); do_qk(H - 1); do_pv(H - 2)
        do_wo(2)
        do_wo(3); do_pv(H - 1)
        do_wo(1, 16)
        out = jnp.concatenate([st['out', n] for n in range(8)], axis=1)
        outa[rows, :] = out[M:].astype(bf16)
        return out[:M].astype(bf16).astype(f32)

    def steps(ahead, i, mem):
        if ahead:
            before_steps(i)
        for u in range(UNROLL):
            mem = step(i * UNROLL + u, mem, ahead)
        store_rows(i)
        return mem

    mem = lax.fori_loop(0, PRE // UNROLL, functools.partial(steps, True), mem_ref[...].astype(f32))
    lax.fori_loop(PRE // UNROLL, NSEG // UNROLL, functools.partial(steps, False), mem)


def _kernel(xa_hbm, xa3_hbm, mem_hbm, wq_hbm, wk_hbm, wv_hbm, wo_hbm, xb_hbm, wr_hbm, wi_hbm, fd_hbm, fs_hbm,
            out_hbm, mem_ref, raw, wqkv, xq, xpre, pre, wo, xa, ya, xb, fd, fs, wraw, wnyq, wst, zb, yb, zn,
            sems, xsem, fsem, wsem, osem):
    def copy(src, dst, i, priority=0):
        c = pltpu.make_async_copy(src, dst, sems.at[i])
        c.start(priority=priority)
        return c

    def xb_copy(g):
        return pltpu.make_async_copy(xb_hbm.at[:, pl.ds(pl.multiple_of(g * G, G), G), :], xb.at[g], xsem.at[g])

    def yb_copy(g):
        return pltpu.make_async_copy(
            xb.at[g], out_hbm.at[:, pl.ds(pl.multiple_of(g * G, G), G), pl.ds(D, D)], osem.at[1])

    def raw_chunk(c):
        return raw.at[c, pl.ds(0, D * HG // 2), :]

    def w_copy(j, hg):
        src = (wq_hbm, wk_hbm, wv_hbm)[j].bitcast(u32).at[:, pl.ds(hg * (HG // 2), HG // 2), :]
        c = j * (H // HG) + hg
        return pltpu.make_async_copy(src, raw_chunk(c).reshape(D, HG // 2, DH), wsem.at[c])

    small = [copy(fd_hbm, fd, 0), copy(fs_hbm, fs, 4), copy(mem_hbm, mem_ref, 5)]
    small += [copy(w.at[pl.ds(D // 2, 1), :], wnyq.at[c], 1 + c) for c, w in enumerate((wr_hbm, wi_hbm))]
    xb_copy(0).start()
    for c in small:
        c.wait()
    for g in range(1, R2 // G):
        xb_copy(g).start()

    def filter_copies(g):
        return [pltpu.make_async_copy(
            w.at[pl.ds(0, D // 2), pl.ds(pl.multiple_of(t * 128, 128), 128)], wraw.at[c * R1 + t, pl.ds(0, D // 2), :], fsem.at[g])
            for t in (2 * g, 2 * g + 1) for c, w in enumerate((wr_hbm, wi_hbm))]

    def wait_rows(g):
        xb_copy(g).wait()

        @pl.when(g == 2)
        def _():
            for i in range(R1 // 2):
                for cp in filter_copies(i):
                    cp.start()
            x_ahead().start()

    def x_first():
        rows = pl.ds(0, XA0 * SEG)
        return pltpu.make_async_copy(xa_hbm.at[rows, :], xa.at[rows, :], sems.at[6])

    def x_ahead():
        return pltpu.make_async_copy(xa3_hbm.at[pl.ds(0, PRE), pl.ds(SEG - 8, 8), :], xq, sems.at[9])

    def wo_copy():
        return pltpu.make_async_copy(wo_hbm.bitcast(u32), wo, sems.at[7])

    def wait_filter(g):
        for cp in filter_copies(g):
            cp.wait()

        @pl.when(g == R1 // 2 - 2)
        def _():
            for j in range(3):
                for hg in range(H // HG):
                    w_copy(j, hg).start()
            wo_copy().start()
            x_first().start()

    def prepare_filter(g):
        pairs = wraw.bitcast(u32)
        for t in (2 * g, 2 * g + 1):
            dst = pl.ds(pl.multiple_of(t * 64, 64), 64)
            for j in range(NT):
                for c in range(2):
                    res = []
                    for k1 in _k1_pair(j):
                        w = pairs[c * R1 + t, pl.ds(k1 // 2, 64, stride=4), :]
                        res.append(pltpu.bitcast(w & u32(0xFFFF0000) if k1 % 2 else w << 16, f32))
                    if j == 0:
                        dc = lax.broadcasted_iota(jnp.int32, (8, 128), 0) == 0
                        res[:1] = [jnp.where(dc, 0.5 * res[0][:8], res[0][:8]), res[0][8:]]
                    tile = jnp.concatenate(res, axis=0)
                    tile = pltpu.bitcast(tile.T, u32)
                    wst[c, j, dst, :] = jnp.concatenate(
                        [(tile[r:r + 8] >> 16) | tile[r + 8:r + 16] for r in range(0, 128, 16)], axis=0)
                yield

    _spectral_phase(xb, fd, fs, wst, wnyq, zb, yb, zn, wait_rows, wait_filter, prepare_filter)

    x_ahead().wait()
    for s in range(PRE):
        xpre[s * 8:(s + 1) * 8, :] = xq[s].astype(f32)

    def relayout(c):
        j, h0 = c // (H // HG), (c % (H // HG)) * HG
        for i in range(HG // 2):
            w = raw[c, pl.ds(i, D, stride=HG // 2), :]
            for hd, bits in ((2 * i, w << 16), (2 * i + 1, w & u32(0xFFFF0000))):
                panel = pltpu.bitcast(bits, f32).astype(bf16)
                wqkv[h0 + hd, j] = pltpu.bitcast(panel, u32)
                pre[h0 + hd, j] = _dot(xpre[...], panel)

    _loop(3 * H // HG, UB[4], relayout,
          lambda c: pltpu.make_async_copy(raw_chunk(c), raw_chunk(c), wsem.at[c]).wait())
    wo_copy().wait()
    x_first().wait()
    rest = pl.ds(XA0 * SEG, S - XA0 * SEG)
    c_rest = copy(xa_hbm.at[rest, :], xa.at[rest, :], 8)
    for g in range(R2 // G):
        yb_copy(g).start()

    def before_steps(i):
        @pl.when(i == XA0 // UNROLL)
        def _():
            c_rest.wait()

    def out_copy(i):
        n = UNROLL * SEG
        dst = out_hbm.at[i // (R2 // n), pl.ds(pl.multiple_of((i % (R2 // n)) * n, n), n), pl.ds(0, D)]
        return pltpu.make_async_copy(ya.at[pl.ds(pl.multiple_of(i * n, n), n), :], dst, osem.at[0])

    _attention_phase(xa, mem_ref, wqkv, pre, wo, ya, before_steps, lambda i: out_copy(i).start())

    def drain(i, _):
        out_copy(i).wait()
        return 0

    lax.fori_loop(0, NSEG // UNROLL, drain, 0)
    for g in range(R2 // G):
        yb_copy(g).wait()


@jax.jit
def pallas_concat_heads__memory_aug_recurrent_mem_tr__spectral_gfnet__prompt_kernel(
    A_x, A_mem0, A_Wq, A_Wk, A_Wv, A_Wo, A_seg_len, B_x, B_w_r, B_w_i,
):
    del A_seg_len
    hbm = pl.BlockSpec(memory_space=pl.ANY)
    out = pl.pallas_call(
        _kernel,
        out_shape=jax.ShapeDtypeStruct((R1, R2, 2 * D), bf16),
        in_specs=[hbm] * 12,
        out_specs=hbm,
        scratch_shapes=[
            pltpu.VMEM((M, D), bf16),
            pltpu.VMEM((3 * H // HG, D * HG // 2 + 8, DH), u32),
            pltpu.VMEM((H, 3, D // 2, DH), u32),
            pltpu.VMEM((PRE, 8, D), bf16),
            pltpu.VMEM((PRE * 8, D), f32),
            pltpu.VMEM((H, 3, PRE * 8, DH), f32),
            pltpu.VMEM((H * DH // 2, D), u32),
            pltpu.VMEM((S, D), bf16),
            pltpu.VMEM((S, D), bf16),
            pltpu.VMEM((R2 // G, R1, G, D), bf16),
            pltpu.VMEM((4, 256, 256), bf16),
            pltpu.VMEM((2, 2 * R2 + R1, R2), f32),
            pltpu.VMEM((2 * R1, D // 2 + 16, 128), bf16),
            pltpu.VMEM((2, 1, S), bf16),
            pltpu.VMEM((2, NT, S // 2 + 8, 128), u32),
            pltpu.VMEM((R1, 2 * R2, NT * 128), f32),
            pltpu.VMEM((R1, 2 * R2, NT * 128), f32),
            pltpu.VMEM((2, R2, 128), f32),
            pltpu.SemaphoreType.DMA((10,)),
            pltpu.SemaphoreType.DMA((R2 // G,)),
            pltpu.SemaphoreType.DMA((R1 // 2,)),
            pltpu.SemaphoreType.DMA((3 * H // HG,)),
            pltpu.SemaphoreType.DMA((2,)),
        ],
        compiler_params=pltpu.CompilerParams(vmem_limit_bytes=120 * 2 ** 20),
    )(
        A_x.reshape(S, D), A_x.reshape(NSEG, SEG, D), A_mem0.reshape(M, D),
        A_Wq, A_Wk, A_Wv,
        A_Wo.reshape(H * DH, D),
        B_x.reshape(R1, R2, D), B_w_r.T, B_w_i.T,
        jnp.asarray(_FD, dtype=bf16), jnp.asarray(_FS),
    )
    return out.reshape(1, S, 2 * D)
```

```python
import functools

import numpy as np
import jax
import jax.numpy as jnp
from jax import lax
import jax.experimental.pallas as pl
import jax.experimental.pallas.tpu as pltpu

S, D, H, DH, M, SEG = 2048, 1024, 32, 128, 8, 32
L = M + SEG
NSEG = S // SEG
DF = D // 2 + 1
R1, R2 = 16, 128
G = 16
HG = 16
UNROLL = 2
PRE = 30
XA0 = 4
UB = (1, 2, 2, 2, 2)
NT = 4
f32, bf16, u32 = jnp.float32, jnp.bfloat16, jnp.uint32


def _k1_pair(j):
    return j, (4 if j == 0 else 8 - j)


def _dft_constants():
    b = np.arange(128)[:, None]
    c = np.arange(64)[None, :]
    fd = np.zeros((4, 256, 256))
    for j in range(4):
        for half, k1 in enumerate(_k1_pair(j)):
            ang = 2.0 * np.pi * ((b * (k1 + 8 * c)) % D) / D
            co, si = np.cos(ang), np.sin(ang)
            re = slice(64 * half, 64 * half + 64)
            im = slice(128 + 64 * half, 128 + 64 * half + 64)
            if j == 0:
                rows = slice(128 * half, 128 * half + 128)
                fd[j, rows, re], fd[j, rows, im] = co, -si
            else:
                sg = 1.0 - 2.0 * half
                fd[j, :128, re], fd[j, :128, im] = co, -si
                fd[j, 128:, re], fd[j, 128:, im] = sg * si, sg * co
    fd[0, :128, 128] = 1.0 - 2.0 * (np.arange(128) % 2)
    n = np.arange(R2)
    a = -2.0 * np.pi * np.concatenate([(n[:, None] * n[None, :]) % R2 / R2,
                                       np.arange(R1)[:, None] * n[None, :] / S,
                                       n[:, None] * n[None, :] / S], axis=0)
    return fd.astype(np.float32), np.stack([np.cos(a), np.sin(a)]).astype(np.float32)


_FD, _FS = _dft_constants()
_RH = float(np.sqrt(0.5))


def _dot(a, b):
    return lax.dot_general(a, b, (((1,), (0,)), ((), ())), preferred_element_type=f32)


def _dot_nt(a, b):
    return lax.dot_general(a, b, (((1,), (1,)), ((), ())), preferred_element_type=f32)


def _dot_tn(a, b):
    return lax.dot_general(a, b, (((0,), (0,)), ((), ())), preferred_element_type=f32)


def _cmul_const(x, e, n, sign):
    xr, xi = x
    e = e % n
    if e == 0:
        return x
    if 4 * e == n:
        return (_neg(xi), xr) if sign > 0 else (xi, _neg(xr))
    c = float(np.cos(2.0 * np.pi * e / n))
    s = float(sign * np.sin(2.0 * np.pi * e / n))
    if xi is None:
        return xr * c, xr * s
    if 8 * e == n or 8 * e == 3 * n:
        if c * s > 0:
            return (xr - xi) * c, (xr + xi) * c
        return (xr + xi) * c, (xi - xr) * c
    return xr * c - xi * s, xr * s + xi * c


def _neg(a):
    return None if a is None else -a


def _add(a, b):
    return b if a is None else a if b is None else a + b


def _sub(a, b):
    return _neg(b) if a is None else a if b is None else a - b


def _fft(xs, sign):
    n = len(xs)
    if n == 1:
        return xs
    ev, od = _fft(xs[0::2], sign), _fft(xs[1::2], sign)
    out = [None] * n
    for j in range(n // 2):
        e = ev[j]
        if 4 * j == n:
            orr, oi = od[j]
            if sign > 0:
                out[j] = (_sub(e[0], oi), _add(e[1], orr))
                out[j + n // 2] = (_add(e[0], oi), _sub(e[1], orr))
            else:
                out[j] = (_add(e[0], oi), _sub(e[1], orr))
                out[j + n // 2] = (_sub(e[0], oi), _add(e[1], orr))
            continue
        t = _cmul_const(od[j], j, n, sign)
        out[j] = (_add(e[0], t[0]), _add(e[1], t[1]))
        out[j + n // 2] = (_sub(e[0], t[0]), _sub(e[1], t[1]))
    return out


def _rfft8(x):
    s04, d04, s26, d26 = x[0] + x[4], x[0] - x[4], x[2] + x[6], x[2] - x[6]
    s15, d15, s37, d37 = x[1] + x[5], x[1] - x[5], x[3] + x[7], x[3] - x[7]
    e, o = s04 + s26, s15 + s37
    p, q = (d15 - d37) * _RH, (d15 + d37) * _RH
    return [(e + o, e - o), (d04 + p, -(d26 + q)), (s04 - s26, s37 - s15), (d04 - p, d26 - q)]


def _rfft8_adjoint(g):
    (g0, g4), (r1, i1), (r2, i2), (r3, i3) = g
    e, o = g0 + g4, g0 - g4
    s04, s26, s15, s37 = e + r2, e - r2, o - i2, o + i2
    d04, d26 = r1 + r3, i3 - i1
    p, q = (r1 - r3) * _RH, (i1 + i3) * _RH
    d15, d37 = p - q, -(p + q)
    return [s04 + d04, s15 + d15, s26 + d26, s37 + d37, s04 - d04, s15 - d15, s26 - d26, s37 - d37]


def _loop(n, unroll, body, before=None):
    def group(i, _):
        if before is not None:
            for u in range(unroll):
                before(i * unroll + u)
        for u in range(unroll):
            body(i * unroll + u)
        return 0

    lax.fori_loop(0, n // unroll, group, 0)


def _spectral_phase(xb, fd, fs, wst, wnyq, zb, yb, zn, wait_rows, wait_filter, prepare_filter):
    groups = [(h, t1) for h in range(G // 8) for t1 in range(R1)]

    def fwd(g):
        r0 = pl.multiple_of(g * G, G)
        lane0 = lax.broadcasted_iota(jnp.int32, (R1 * G, 128), 1) == 0
        xg = [xb[g, t1].astype(f32) for t1 in range(R1)]
        xg = jnp.concatenate([xg[t1][h * 8:(h + 1) * 8] for h, t1 in groups], axis=0)
        us = _rfft8([xg[:, a * 128:(a + 1) * 128] for a in range(8)])
        us = [jnp.concatenate(u, axis=1).astype(bf16) for u in us]
        for j in range(NT):
            z = _dot(us[j], fd[j])
            zr, zi = z[:, :128], z[:, 128:]
            if j == 0:
                for h in range(G // 8):
                    ys = _fft([(jnp.where(lane0[:8], zi[n * 8:(n + 1) * 8], 0.0), None)
                               for n in range(h * R1, (h + 1) * R1)], -1)
                    for c in range(2):
                        parts = [pltpu.roll(y[c], f1, 1) if f1 else y[c]
                                 for f1, y in enumerate(ys) if y[c] is not None]
                        zn[c, pl.ds(r0 + h * 8, 8), :] = functools.reduce(jnp.add, parts)
                zi = jnp.where(lane0, 0.0, zi)
            xs = [(zr[n * 8:(n + 1) * 8], zi[n * 8:(n + 1) * 8]) for n in range(len(groups))]
            for h in range(G // 8):
                for f1, (yr, yi) in enumerate(_fft(xs[h * R1:(h + 1) * R1], -1)):
                    zb[f1, pl.ds(r0 + h * 8, 8), j * 128:(j + 1) * 128] = yr
                    zb[f1, pl.ds(R2 + r0 + h * 8, 8), j * 128:(j + 1) * 128] = yi

    _loop(R2 // G, UB[0], fwd, wait_rows)

    def dft_block(f1, inverse):
        cr, ci = fs[0, :R2, :], fs[1, :R2, :]
        tr, ti = fs[0, pl.ds(R2 + f1, 1), :], fs[1, pl.ds(R2 + f1, 1), :]
        if inverse:
            tr, ti = tr * (2.0 / (S * D)), ti * (2.0 / (S * D))
        mr, mi = cr * tr - ci * ti, cr * ti + ci * tr
        if inverse:
            return [m.astype(bf16).T for m in (mr, -mi - mr, mr - mi)]
        return [m.astype(bf16) for m in (mr, mi - mr, mr + mi)]

    def cmatmul(m, xr, xi):
        k = _dot(m[0], (xr + xi).astype(bf16))
        return k - _dot(m[2], xi.astype(bf16)), k + _dot(m[1], xr.astype(bf16))

    tr, ti = fs[0, R2 + R1:, :], fs[1, R2 + R1:, :]
    xr, xi = cmatmul(dft_block(0, False), zn[0] * tr - zn[1] * ti, zn[0] * ti + zn[1] * tr)

    def nyquist_filter(c):
        w = jnp.concatenate([jnp.broadcast_to(wnyq[c, :, t * 128:(t + 1) * 128].astype(f32), (8, 128))
                             for t in range(S // 128)], axis=0)
        f2 = lax.broadcasted_iota(jnp.int32, w.shape, 0)
        for bit in (1, 2, 4):
            w = jnp.where((f2 & bit) != 0, pltpu.roll(w, 128 - bit * R1, 1), w)
        return 0.5 * w

    wr, wi = nyquist_filter(0), nyquist_filter(1)
    yr, yi = cmatmul(dft_block(0, True), xr * wr - xi * wi, xr * wi + xi * wr)
    zn[0], zn[1] = yr * tr + yi * ti, yi * tr - yr * ti

    def dft(g):
        side = prepare_filter(g)
        for f1 in (2 * g, 2 * g + 1):
            mb = dft_block(f1, False)
            for j in range(NT):
                cols = slice(j * 128, (j + 1) * 128)
                next(side)
                yb[f1, :R2, cols], yb[f1, R2:, cols] = cmatmul(mb, zb[f1, :R2, cols], zb[f1, R2:, cols])

    _loop(R1 // 2, UB[1], dft, wait_filter)

    def idft(g):
        for half in range(2):
            f1 = g + half * (R1 // 2)
            mbt = dft_block(f1, True)
            for j in range(NT):
                cols = slice(j * 128, (j + 1) * 128)
                wr = wst[0, j, pl.ds(g, R2, stride=R1 // 2), :]
                wi = wst[1, j, pl.ds(g, R2, stride=R1 // 2), :]
                if half == 0:
                    wr, wi = wr << 16, wi << 16
                else:
                    wr, wi = wr & u32(0xFFFF0000), wi & u32(0xFFFF0000)
                wr, wi = pltpu.bitcast(wr, f32), pltpu.bitcast(wi, f32)
                xr, xi = yb[f1, :R2, cols], yb[f1, R2:, cols]
                zb[f1, :R2, cols], zb[f1, R2:, cols] = cmatmul(mbt, xr * wr - xi * wi, xr * wi + xi * wr)

    _loop(R1 // 2, UB[2], idft)

    def inv(g):
        r0 = pl.multiple_of(g * G, G)
        lane0 = lax.broadcasted_iota(jnp.int32, (R1 * G, 128), 1) == 0

        def tile(load):
            ys = []
            for h in range(G // 8):
                ys += _fft([load(f1, r0 + h * 8) for f1 in range(R1)], +1)
            return (jnp.concatenate([y[0] for y in ys], axis=0),
                    jnp.concatenate([y[1] for y in ys], axis=0))

        nyq = tile(lambda f1, r: tuple(pltpu.roll(zn[c, pl.ds(r, 8), :], 128 - f1, 1) if f1
                                       else zn[c, pl.ds(r, 8), :] for c in range(2)))[0]
        gs = []
        for j in range(4):
            yr, yi = tile(lambda f1, r: (zb[f1, pl.ds(r, 8), j * 128:(j + 1) * 128],
                                         zb[f1, pl.ds(R2 + r, 8), j * 128:(j + 1) * 128]))
            if j == 0:
                yi = jnp.where(lane0, nyq, yi)
            p = _dot_nt(jnp.concatenate([yr, yi], axis=1).astype(bf16), fd[j])
            gs.append((p[:, :128], p[:, 128:]))
        y = jnp.concatenate(_rfft8_adjoint(gs), axis=1)
        for t1 in range(R1):
            xb[g, t1] = jnp.concatenate(
                [y[(h * R1 + t1) * 8:(h * R1 + t1 + 1) * 8] for h in range(G // 8)], axis=0).astype(bf16)

    _loop(R2 // G, UB[3], inv)


def _attention_phase(xa, mem_ref, wqkv, pre, wo, outa, before_steps, store_rows):
    row = lax.broadcasted_iota(jnp.int32, (L, L), 0)
    col = lax.broadcasted_iota(jnp.int32, (L, L), 1)

    def step(s, mem, ahead):
        mask = (row < M) | (row >= col)
        rows = pl.ds(pl.multiple_of(s * SEG, SEG), SEG)
        h = jnp.concatenate([mem, xa[rows, :].astype(f32)], axis=0)
        if ahead:
            h = h[:L - 8]
        st = {}

        def project(hd, lo, hi):
            w = jnp.concatenate([wqkv[hd, j, lo // 2:hi // 2, :] for j in range(3)], axis=1)
            return _dot(h[:, lo:hi], pltpu.bitcast(w, bf16))

        split = D // 4
        for hd in range(3):
            st['early', hd] = project(hd, 0, split)

        def do_qkv(hd):
            qkv = st['early', hd] + project(hd, split, D) if ('early', hd) in st else project(hd, 0, D)
            if ahead:
                r8 = pl.ds(pl.multiple_of(s * 8, 8), 8)
                qkv = jnp.concatenate(
                    [qkv, jnp.concatenate([pre[hd, j, r8, :] for j in range(3)], axis=1)], axis=0)
            st['q', hd] = qkv[:, :128] * (DH ** -0.5)
            st['k', hd] = qkv[:, 128:256].astype(bf16)
            st['v', hd] = qkv[:, 256:].astype(bf16)

        def do_qk(hd):
            sc = jnp.where(mask, _dot_nt(st['q', hd], st['k', hd]), -1e9)
            e = jnp.exp(sc - jnp.max(sc, axis=1, keepdims=True))
            st['e', hd] = e
            den = jnp.sum(e, axis=1, keepdims=True)
            r = pl.reciprocal(den, approx=True)
            st['r', hd] = r * (2.0 - den * r)

        def do_pv(hd):
            st['o', hd] = _dot(st['e', hd], st['v', hd]) * st['r', hd]

        def do_wo(g, ng=4):
            o = jnp.concatenate([st['o', hd] for hd in range(g * ng, (g + 1) * ng)], axis=1)
            for n in range(8):
                r = _dot(o, pltpu.bitcast(wo[g * ng * 64:(g + 1) * ng * 64, n * 128:(n + 1) * 128], bf16))
                st['out', n] = st['out', n] + r if ('out', n) in st else r

        for t in range(H):
            do_qkv(t)
            if t >= 2: do_qk(t - 2)
            if t >= 4: do_pv(t - 4)
        do_wo(0); do_qk(H - 2); do_pv(H - 4)
        do_wo(1); do_qk(H - 1); do_pv(H - 3)
        do_wo(2); do_pv(H - 2)
        do_wo(3); do_pv(H - 1)
        do_wo(1, 16)
        out = jnp.concatenate([st['out', n] for n in range(8)], axis=1)
        outa[rows, :] = out[M:].astype(bf16)
        return out[:M].astype(bf16).astype(f32)

    def steps(ahead, i, mem):
        if ahead:
            before_steps(i)
        for u in range(UNROLL):
            mem = step(i * UNROLL + u, mem, ahead)
        store_rows(i)
        return mem

    mem = lax.fori_loop(0, PRE // UNROLL, functools.partial(steps, True), mem_ref[...].astype(f32))
    lax.fori_loop(PRE // UNROLL, NSEG // UNROLL, functools.partial(steps, False), mem)


def _kernel(xa_hbm, xa3_hbm, mem_hbm, wq_hbm, wk_hbm, wv_hbm, wo_hbm, xb_hbm, wr_hbm, wi_hbm, fd_hbm, fs_hbm,
            out_hbm, mem_ref, raw, wqkv, xq, xpre, pre, wo, xa, ya, xb, fd, fs, wraw, wnyq, wst, zb, yb, zn,
            sems, xsem, fsem, wsem, osem):
    def copy(src, dst, i, priority=0):
        c = pltpu.make_async_copy(src, dst, sems.at[i])
        c.start(priority=priority)
        return c

    def xb_copy(g):
        return pltpu.make_async_copy(xb_hbm.at[:, pl.ds(pl.multiple_of(g * G, G), G), :], xb.at[g], xsem.at[g])

    def yb_copy(g):
        return pltpu.make_async_copy(
            xb.at[g], out_hbm.at[:, pl.ds(pl.multiple_of(g * G, G), G), pl.ds(D, D)], osem.at[1])

    def raw_chunk(c):
        return raw.at[c, pl.ds(0, D * HG // 2), :]

    def w_copy(j, hg):
        src = (wq_hbm, wk_hbm, wv_hbm)[j].bitcast(u32).at[:, pl.ds(hg * (HG // 2), HG // 2), :]
        c = j * (H // HG) + hg
        return pltpu.make_async_copy(src, raw_chunk(c).reshape(D, HG // 2, DH), wsem.at[c])

    small = [copy(fd_hbm, fd, 0), copy(fs_hbm, fs, 4), copy(mem_hbm, mem_ref, 5)]
    small += [copy(w.at[pl.ds(D // 2, 1), :], wnyq.at[c], 1 + c) for c, w in enumerate((wr_hbm, wi_hbm))]
    xb_copy(0).start()
    for c in small:
        c.wait()
    for g in range(1, R2 // G):
        xb_copy(g).start()

    def filter_copies(g):
        return [pltpu.make_async_copy(
            w.at[pl.ds(0, D // 2), pl.ds(pl.multiple_of(t * 128, 128), 128)], wraw.at[c * R1 + t, pl.ds(0, D // 2), :], fsem.at[g])
            for t in (2 * g, 2 * g + 1) for c, w in enumerate((wr_hbm, wi_hbm))]

    def wait_rows(g):
        xb_copy(g).wait()

        @pl.when(g == 2)
        def _():
            for i in range(R1 // 2):
                for cp in filter_copies(i):
                    cp.start()
            x_ahead().start()

    def x_first():
        rows = pl.ds(0, XA0 * SEG)
        return pltpu.make_async_copy(xa_hbm.at[rows, :], xa.at[rows, :], sems.at[6])

    def x_ahead():
        return pltpu.make_async_copy(xa3_hbm.at[pl.ds(0, PRE), pl.ds(SEG - 8, 8), :], xq, sems.at[9])

    def wo_copy():
        return pltpu.make_async_copy(wo_hbm.bitcast(u32), wo, sems.at[7])

    def wait_filter(g):
        for cp in filter_copies(g):
            cp.wait()

        @pl.when(g == R1 // 2 - 2)
        def _():
            for j in range(3):
                for hg in range(H // HG):
                    w_copy(j, hg).start()
            wo_copy().start()
            x_first().start()

    def prepare_filter(g):
        pairs = wraw.bitcast(u32)
        for t in (2 * g, 2 * g + 1):
            dst = pl.ds(pl.multiple_of(t * 64, 64), 64)
            for j in range(NT):
                for c in range(2):
                    res = []
                    for k1 in _k1_pair(j):
                        w = pairs[c * R1 + t, pl.ds(k1 // 2, 64, stride=4), :]
                        res.append(pltpu.bitcast(w & u32(0xFFFF0000) if k1 % 2 else w << 16, f32))
                    if j == 0:
                        dc = lax.broadcasted_iota(jnp.int32, (8, 128), 0) == 0
                        res[:1] = [jnp.where(dc, 0.5 * res[0][:8], res[0][:8]), res[0][8:]]
                    tile = jnp.concatenate(res, axis=0)
                    tile = pltpu.bitcast(tile.T, u32)
                    wst[c, j, dst, :] = jnp.concatenate(
                        [(tile[r:r + 8] >> 16) | tile[r + 8:r + 16] for r in range(0, 128, 16)], axis=0)
                yield

    _spectral_phase(xb, fd, fs, wst, wnyq, zb, yb, zn, wait_rows, wait_filter, prepare_filter)

    x_ahead().wait()
    for s in range(PRE):
        xpre[s * 8:(s + 1) * 8, :] = xq[s].astype(f32)

    def relayout(c):
        j, h0 = c // (H // HG), (c % (H // HG)) * HG
        for i in range(HG // 2):
            w = raw[c, pl.ds(i, D, stride=HG // 2), :]
            for hd, bits in ((2 * i, w << 16), (2 * i + 1, w & u32(0xFFFF0000))):
                panel = pltpu.bitcast(bits, f32).astype(bf16)
                wqkv[h0 + hd, j] = pltpu.bitcast(panel, u32)
                pre[h0 + hd, j] = _dot(xpre[...], panel)

    _loop(3 * H // HG, UB[4], relayout,
          lambda c: pltpu.make_async_copy(raw_chunk(c), raw_chunk(c), wsem.at[c]).wait())
    wo_copy().wait()
    x_first().wait()
    rest = pl.ds(XA0 * SEG, S - XA0 * SEG)
    c_rest = copy(xa_hbm.at[rest, :], xa.at[rest, :], 8)
    for g in range(R2 // G):
        yb_copy(g).start()

    def before_steps(i):
        @pl.when(i == XA0 // UNROLL)
        def _():
            c_rest.wait()

    def out_copy(i):
        n = UNROLL * SEG
        dst = out_hbm.at[i // (R2 // n), pl.ds(pl.multiple_of((i % (R2 // n)) * n, n), n), pl.ds(0, D)]
        return pltpu.make_async_copy(ya.at[pl.ds(pl.multiple_of(i * n, n), n), :], dst, osem.at[0])

    _attention_phase(xa, mem_ref, wqkv, pre, wo, ya, before_steps, lambda i: out_copy(i).start())

    def drain(i, _):
        out_copy(i).wait()
        return 0

    lax.fori_loop(0, NSEG // UNROLL, drain, 0)
    for g in range(R2 // G):
        yb_copy(g).wait()


@jax.jit
def pallas_concat_heads__memory_aug_recurrent_mem_tr__spectral_gfnet__prompt_kernel(
    A_x, A_mem0, A_Wq, A_Wk, A_Wv, A_Wo, A_seg_len, B_x, B_w_r, B_w_i,
):
    del A_seg_len
    hbm = pl.BlockSpec(memory_space=pl.ANY)
    out = pl.pallas_call(
        _kernel,
        out_shape=jax.ShapeDtypeStruct((R1, R2, 2 * D), bf16),
        in_specs=[hbm] * 12,
        out_specs=hbm,
        scratch_shapes=[
            pltpu.VMEM((M, D), bf16),
            pltpu.VMEM((3 * H // HG, D * HG // 2 + 8, DH), u32),
            pltpu.VMEM((H, 3, D // 2, DH), u32),
            pltpu.VMEM((PRE, 8, D), bf16),
            pltpu.VMEM((PRE * 8, D), f32),
            pltpu.VMEM((H, 3, PRE * 8, DH), f32),
            pltpu.VMEM((H * DH // 2, D), u32),
            pltpu.VMEM((S, D), bf16),
            pltpu.VMEM((S, D), bf16),
            pltpu.VMEM((R2 // G, R1, G, D), bf16),
            pltpu.VMEM((4, 256, 256), bf16),
            pltpu.VMEM((2, 2 * R2 + R1, R2), f32),
            pltpu.VMEM((2 * R1, D // 2 + 16, 128), bf16),
            pltpu.VMEM((2, 1, S), bf16),
            pltpu.VMEM((2, NT, S // 2 + 8, 128), u32),
            pltpu.VMEM((R1, 2 * R2, NT * 128), f32),
            pltpu.VMEM((R1, 2 * R2, NT * 128), f32),
            pltpu.VMEM((2, R2, 128), f32),
            pltpu.SemaphoreType.DMA((10,)),
            pltpu.SemaphoreType.DMA((R2 // G,)),
            pltpu.SemaphoreType.DMA((R1 // 2,)),
            pltpu.SemaphoreType.DMA((3 * H // HG,)),
            pltpu.SemaphoreType.DMA((2,)),
        ],
        compiler_params=pltpu.CompilerParams(vmem_limit_bytes=120 * 2 ** 20),
    )(
        A_x.reshape(S, D), A_x.reshape(NSEG, SEG, D), A_mem0.reshape(M, D),
        A_Wq, A_Wk, A_Wv,
        A_Wo.reshape(H * DH, D),
        B_x.reshape(R1, R2, D), B_w_r.T, B_w_i.T,
        jnp.asarray(_FD, dtype=bf16), jnp.asarray(_FS),
    )
    return out.reshape(1, S, 2 * D)
```
